```python
import jax
import jax.numpy as jnp

def _softmax(x, axis=-1):
    return jax.nn.softmax(x, axis=axis)
def _gelu(x):
    return jax.nn.gelu(x, approximate=True)
def _silu(x):
    return jax.nn.silu(x)
def _sigmoid(x):
    return jax.nn.sigmoid(x)
def _layernorm(x, axis=-1, eps=1e-5):
    m = jnp.mean(x, axis=axis, keepdims=True)
    v = jnp.var(x, axis=axis, keepdims=True)
    return (x - m) / jnp.sqrt(v + eps)
def _scatter_add(tgt, idx, src, axis=0):
    return tgt.at[idx].add(src)
def _segment_sum(src, seg, n):
    return jax.ops.segment_sum(src, seg, n)
class _Rng:
    def __init__(self, key):
        self._k = key
    def _next(self):
        self._k, sub = jax.random.split(self._k)
        return sub
    def normal(self, shape):
        return jax.random.normal(self._next(), shape, dtype=jnp.bfloat16)
    def randint(self, lo, hi, shape):
        return jax.random.randint(self._next(), shape, lo, hi, dtype=jnp.int32)
    def uniform(self, shape, lo=0.0, hi=1.0):
        return jax.random.uniform(self._next(), shape, jnp.bfloat16, lo, hi)
    def permutation(self, n):
        return jax.random.permutation(self._next(), n)


kernel_name = 'interleave_layers__compressed_kv_cla__moe_arch_mod__decode'

def setup_inputs():
    _rng = _Rng(jax.random.key(int.from_bytes(__import__("os").urandom(4), "little")))
    _w = (lambda a: (lambda t: t.astype(jnp.bfloat16) if jnp.issubdtype(t.dtype, jnp.floating) else t)(jnp.asarray(a)))
    def _A_setup():
        B, H, Sq, Sk, D, M = 1, 32, 1, 4096, 128, 640
        Dc = 4 * D
        return {
            "x": _w((lambda *s: _rng.normal(s) * 0.05)(B, Sq, M)),
            "c_kv": _w((lambda *s: _rng.normal(s) * 0.05)(B, Sk, Dc)),
            "w_q": _w((lambda *s: _rng.normal(s) * 0.05)(M, H, D) * (M ** -0.5)),
            "w_uk": _w((lambda *s: _rng.normal(s) * 0.05)(Dc, H, D) * (Dc ** -0.5)),
            "w_uv": _w((lambda *s: _rng.normal(s) * 0.05)(Dc, H, D) * (Dc ** -0.5)),
            "w_o": _w((lambda *s: _rng.normal(s) * 0.05)(H, D, M) * ((H * D) ** -0.5)),
        }
    _A_in = _A_setup()

    def _B_setup():
        B, S, D, F, C = 1, 1, 640, 1728, 1
        return {
            "x": _w((lambda *s: _rng.normal(s) * 0.05)(B, S, D)),
            "w_r": _w((lambda *s: _rng.normal(s) * 0.05)(D)),
            "w_gate": _w((lambda *s: _rng.normal(s) * 0.05)(D, F)),
            "w_up": _w((lambda *s: _rng.normal(s) * 0.05)(D, F)),
            "w_down": _w((lambda *s: _rng.normal(s) * 0.05)(F, D)),
        }
    _B_in = _B_setup()

    return {
        "A_x": _A_in["x"],
        "A_c_kv": _A_in["c_kv"],
        "A_w_q": _A_in["w_q"],
        "A_w_uk": _A_in["w_uk"],
        "A_w_uv": _A_in["w_uv"],
        "A_w_o": _A_in["w_o"],
        "B_x": _B_in["x"],
        "B_w_r": _B_in["w_r"],
        "B_w_gate": _B_in["w_gate"],
        "B_w_up": _B_in["w_up"],
        "B_w_down": _B_in["w_down"],
    }

def reference(A_x, A_c_kv, A_w_q, A_w_uk, A_w_uv, A_w_o, B_x, B_w_r, B_w_gate, B_w_up, B_w_down):
    def _A_ref(x, c_kv, w_q, w_uk, w_uv, w_o):
        B, Sq, M = x.shape[0], x.shape[1], x.shape[2]
        Sk = c_kv.shape[1]
        H, D = w_q.shape[1], w_q.shape[2]
        q = jnp.einsum("bqm,mhd->bhqd", x, w_q)
        k = jnp.einsum("bkc,chd->bhkd", c_kv, w_uk)
        v = jnp.einsum("bkc,chd->bhkd", c_kv, w_uv)
        scores = jnp.einsum("bhqd,bhkd->bhqk", q, k) * (D ** -0.5)
        off = Sk - Sq
        qi = jnp.arange(Sq)[:, None]
        kj = jnp.arange(Sk)[None, :]
        cmask = kj <= (qi + off)
        scores = jnp.where(cmask[None, None], scores, -1e9)
        p = _softmax(scores, axis=-1)
        ctx = jnp.einsum("bhqk,bhkd->bhqd", p, v)
        return jnp.einsum("bhqd,hdm->bqm", ctx, w_o)

    def _B_ref(x, w_r, w_gate, w_up, w_down):
        B, S, D = x.shape
        C = 1
        r = x @ w_r
        idx = jnp.argsort(-r, axis=-1)[:, :C]
        idx_e = jnp.repeat(idx.reshape(B, C, 1), D, axis=2)
        x_sel = jnp.take_along_axis(x, idx_e, axis=1)
        g = _silu(x_sel @ w_gate)
        u = x_sel @ w_up
        y = (g * u) @ w_down
        r_sel = _sigmoid(jnp.take_along_axis(r, idx, axis=1))
        y = y * r_sel.reshape(B, C, 1)
        b_off = (jnp.arange(B) * S).reshape(B, 1)
        flat_idx = (idx + b_off).reshape(B * C)
        zero = (x * 0.0).reshape(B * S, D)
        upd = _scatter_add(zero, flat_idx, y.reshape(B * C, D), axis=0)
        return x + upd.reshape(B, S, D)

    x = A_x
    x = x + _A_ref(_layernorm(x, axis=-1), A_c_kv, A_w_q, A_w_uk, A_w_uv, A_w_o)
    x = x + _B_ref(_layernorm(x, axis=-1), B_w_r, B_w_gate, B_w_up, B_w_down)
    x = x + _A_ref(_layernorm(x, axis=-1), A_c_kv, A_w_q, A_w_uk, A_w_uv, A_w_o)
    x = x + _B_ref(_layernorm(x, axis=-1), B_w_r, B_w_gate, B_w_up, B_w_down)
    return x
```

```python
import jax
import jax.numpy as jnp
from jax import lax
import jax.experimental.pallas as pl
import jax.experimental.pallas.tpu as pltpu

bf16 = jnp.bfloat16
f32 = jnp.float32
u32 = jnp.uint32
i32 = jnp.int32

M = 640
H = 32
D = 128
SK = 4096
DC = 512
F = 1728
NJ = M // 128
NC = DC // 128
NK = SK // 128
NF = (F + 127) // 128
LOG2E = 1.4426950408889634
EPS = 1e-5

WD_CHUNKS = [(0, 384), (384, 384), (768, 384), (1152, 256), (1408, 128), (1536, 128), (1664, 64)]


def _dot(a, b):
    return jnp.dot(a, b, preferred_element_type=f32)


def _iota(shape, dim):
    return lax.broadcasted_iota(i32, shape, dim)


def _layernorm(x):
    m = jnp.mean(x, axis=-1, keepdims=True)
    xc = x - m
    v = jnp.mean(xc * xc, axis=-1, keepdims=True)
    return xc * lax.rsqrt(v + EPS)


def _kernel(x_hbm, wr_hbm, wq_hbm, wuk_hbm, c_hbm, wuv_hbm, wo_hbm, wg_hbm, wu_hbm, wd_hbm,
            o_hbm,
            x_v, wr_v, wq_v, wuk_v, c_v, wuv_v, wo_v, wg_v, wu_v, wd_v,
            ukT_v, cT_v, uv_v, gT_v, uT_v, s_v, o_v, sems):
    cps = {}

    def add(name, src, dst):
        cp = pltpu.make_async_copy(src, dst, sems.at[len(cps)])
        cp.start()
        cps[name] = cp

    add("wq", wq_hbm.bitcast(u32), wq_v)
    add("x", x_hbm, x_v)
    add("wr", wr_hbm, wr_v)
    add("wuk", wuk_hbm.bitcast(u32), wuk_v)
    add("c", c_hbm, c_v)
    add("wuv", wuv_hbm.bitcast(u32), wuv_v)
    add("wo", wo_hbm, wo_v)
    add("wg", wg_hbm, wg_v)
    add("wu", wu_hbm, wu_v)
    for i, (s, n) in enumerate(WD_CHUNKS):
        add(f"wd{i}", wd_hbm.at[pl.ds(s, n)], wd_v.at[pl.ds(s, n)])

    lane = _iota((8, 128), 1)
    sub = _iota((8, 128), 0)
    lo_m = jnp.uint32(0x0000FFFF)
    hi_m = jnp.uint32(0xFFFF0000)
    zero_u = jnp.zeros((8, 128), u32)
    mask16 = jnp.where(lane % 16 == 2 * sub, lo_m, zero_u) | jnp.where(lane % 16 == 2 * sub + 1, hi_m, zero_u)
    mask2 = jnp.where(lane % 2 == 0, jnp.full((8, 128), 0x0000FFFF, u32), jnp.full((8, 128), 0xFFFF0000, u32))

    def pack_u32(a):
        return pltpu.bitcast(a.astype(bf16), u32)

    def expand2(p, half):
        g = jnp.take_along_axis(p, 64 * half + lane // 2, axis=1)
        return pltpu.bitcast(g & mask2, bf16)

    def attn(x, first):
        xn = _layernorm(x)
        xb = xn.astype(bf16).astype(f32)
        xw = pltpu.bitcast(xb, u32)
        xw = xw | (xw >> 16)
        if first:
            cps["wq"].wait()
        qacc = [None, None]
        for u in range(M // 64):
            src = xw[:, (u // 2) * 128:(u // 2 + 1) * 128]
            xe = jnp.take_along_axis(src, 64 * (u % 2) + 8 * sub + lane // 16, axis=1)
            for s in range(8):
                t = 8 * u + s
                lhs = pltpu.bitcast(jnp.broadcast_to(xe[s:s + 1, :], (8, 128)) & mask16, bf16)
                for g in range(2):
                    w = wq_v[pl.ds(8 * t, 8), pl.ds(8 * g, 8), :].reshape(64, 128)
                    y = _dot(lhs, pltpu.bitcast(w, bf16))
                    qacc[g] = y if qacc[g] is None else qacc[g] + y
        if first:
            cps["wuk"].wait()
            for hp in range(16):
                for cb in range(NC):
                    rows = [wuk_v[pl.ds((cb * 128 + r * 8) * 16 + hp, 8, stride=16), :] for r in range(16)]
                    t = jnp.concatenate(rows, axis=0)
                    ukT_v[pl.ds((hp * NC + cb) * 128, 128), :] = t.T
        qlhs = []
        for g in range(2):
            p = pack_u32(qacc[g])
            qlhs.append(jnp.concatenate([expand2(p, 0), expand2(p, 1)], axis=1))
        qabs = [[[None, None] for _ in range(NC)] for _ in range(2)]
        for hp in range(16):
            g, r = hp // 8, hp % 8
            k = r // 4
            sel = (sub // 2) == (r % 4)
            for cb in range(NC):
                w = pltpu.bitcast(ukT_v[pl.ds((hp * NC + cb) * 128, 128), :], bf16)
                y = _dot(qlhs[g], w)[8 * k:8 * k + 8, :]
                old = qabs[g][cb][k]
                qabs[g][cb][k] = y if old is None else jnp.where(sel, y, old)
        scale = (D ** -0.5) * LOG2E
        qa = jnp.concatenate(
            [jnp.concatenate([jnp.concatenate(qabs[g][cb], axis=0) for cb in range(NC)], axis=1) for g in range(2)],
            axis=0)
        qa = (qa * scale).astype(bf16)
        if first:
            cps["c"].wait()
        mrun = None
        for kb in range(NK):
            if first:
                for cb in range(NC):
                    t = c_v[pl.ds(kb * 128, 128), pl.ds(cb * 128, 128)]
                    cT_v[kb, pl.ds(cb * 64, 64), :] = pltpu.bitcast(t.T, u32)
            s = _dot(qa, pltpu.bitcast(cT_v[kb], bf16))
            s_v[kb] = s
            mrun = s if mrun is None else jnp.maximum(mrun, s)
        mrow = jnp.max(mrun, axis=-1, keepdims=True)
        lsum = None
        cacc = [None] * NC
        for kb in range(NK):
            p = jnp.exp2(s_v[kb] - mrow)
            lsum = p if lsum is None else lsum + p
            pb = p.astype(bf16)
            for cb in range(NC):
                y = _dot(pb, c_v[pl.ds(kb * 128, 128), pl.ds(cb * 128, 128)])
                cacc[cb] = y if cacc[cb] is None else cacc[cb] + y
        linv = 1.0 / jnp.sum(lsum, axis=-1, keepdims=True)
        if first:
            cps["wuv"].wait()
            for hp in range(16):
                for r in range(DC // 8):
                    uv_v[pl.ds(hp * DC + r * 8, 8), :] = wuv_v[pl.ds(r * 8 * 16 + hp, 8, stride=16), :]
        clhs = []
        for g in range(2):
            parts = []
            for cb in range(NC):
                p = pack_u32(cacc[cb][16 * g:16 * g + 16, :] * linv[16 * g:16 * g + 16, :])
                parts += [expand2(p, 0), expand2(p, 1)]
            clhs.append(jnp.concatenate(parts, axis=1))
        ctx = [None] * 4
        for hp in range(16):
            g, r = hp // 8, hp % 8
            k = r // 4
            sel = (sub // 2) == (r % 4)
            w = pltpu.bitcast(uv_v[pl.ds(hp * DC, DC), :], bf16)
            y = _dot(clhs[g], w)[8 * k:8 * k + 8, :]
            old = ctx[2 * g + k]
            ctx[2 * g + k] = y if old is None else jnp.where(sel, y, old)
        if first:
            cps["wo"].wait()
        lhs = jnp.concatenate(
            [jnp.broadcast_to(ctx[h // 8][h % 8:h % 8 + 1, :], (8, 128)) for h in range(H)], axis=1).astype(bf16)
        return _dot(lhs, wo_v[...])

    def ffn(x, first):
        xn = _layernorm(x)
        xb = xn.astype(bf16)
        r = jnp.sum(xb.astype(f32) * wr, axis=-1, keepdims=True)
        rs = jax.nn.sigmoid(r)
        outs = []
        for name, raw, proc in (("wg", wg_v, gT_v), ("wu", wu_v, uT_v)):
            if first:
                cps[name].wait()
                for fb in range(NF):
                    n = min(128, F - fb * 128)
                    for j in range(NJ):
                        t = raw[pl.ds(fb * 128, n), pl.ds(j * 128, 128)]
                        if n < 128:
                            t = jnp.concatenate([t, jnp.zeros((128 - n, 128), bf16)], axis=0)
                        proc[fb, pl.ds(j * 64, 64), :] = pltpu.bitcast(t.T, u32)
            outs.append([_dot(xb, pltpu.bitcast(proc[fb], bf16)) for fb in range(NF)])
        hs = [(jax.nn.silu(outs[0][fb]) * outs[1][fb]).astype(bf16) for fb in range(NF)]
        y = None
        for i, (s0, n0) in enumerate(WD_CHUNKS):
            if first:
                cps[f"wd{i}"].wait()
            pos = s0
            while pos < s0 + n0:
                n = min(128, s0 + n0 - pos)
                fb = pos // 128
                yy = _dot(hs[fb][:, :n], wd_v[pl.ds(pos, n), :])
                y = yy if y is None else y + yy
                pos += n
        return xn + (xn * 0.0 + y * rs)

    cps["x"].wait()
    cps["wr"].wait()
    x = jnp.broadcast_to(x_v[0].astype(f32), (8, M))
    wr = wr_v[...].astype(f32).reshape(1, M)
    x = x + attn(x, True)
    x = x + ffn(x, True)
    x = x + attn(x, False)
    x = x + ffn(x, False)
    o_v[0] = x[0:1, :].astype(bf16)
    ocp = pltpu.make_async_copy(o_v, o_hbm, sems.at[len(cps)])
    ocp.start()
    ocp.wait()


@jax.jit
def pallas_interleave_layers__compressed_kv_cla__moe_arch_mod__decode_kernel(
    A_x, A_c_kv, A_w_q, A_w_uk, A_w_uv, A_w_o, B_x, B_w_r, B_w_gate, B_w_up, B_w_down,
):
    del B_x
    hbm = lambda a: pltpu.with_memory_space_constraint(a, pltpu.HBM)
    ins = [
        A_x, B_w_r, A_w_q,
        A_w_uk.reshape(DC * H, D),
        A_c_kv.reshape(SK, DC),
        A_w_uv.reshape(DC * H, D),
        A_w_o.reshape(H * D, M),
        B_w_gate.T, B_w_up.T, B_w_down,
    ]
    ins = [hbm(a) for a in ins]
    scratch = [
        pltpu.VMEM((1, 1, M), bf16),
        pltpu.VMEM((M,), bf16),
        pltpu.VMEM((M, H // 2, D), u32),
        pltpu.VMEM((DC * H // 2, D), u32),
        pltpu.VMEM((SK, DC), bf16),
        pltpu.VMEM((DC * H // 2, D), u32),
        pltpu.VMEM((H * D, M), bf16),
        pltpu.VMEM((F, M), bf16),
        pltpu.VMEM((F, M), bf16),
        pltpu.VMEM((F, M), bf16),
        pltpu.VMEM((16 * NC * 128, 128), u32),
        pltpu.VMEM((NK, DC // 2, 128), u32),
        pltpu.VMEM((16 * DC, 128), u32),
        pltpu.VMEM((NF, M // 2, 128), u32),
        pltpu.VMEM((NF, M // 2, 128), u32),
        pltpu.VMEM((NK, H, 128), f32),
        pltpu.VMEM((1, 1, M), bf16),
        pltpu.SemaphoreType.DMA((32,)),
    ]
    return pl.pallas_call(
        _kernel,
        in_specs=[pl.BlockSpec(memory_space=pl.ANY)] * len(ins),
        out_specs=pl.BlockSpec(memory_space=pl.ANY),
        out_shape=jax.ShapeDtypeStruct((1, 1, M), bf16),
        scratch_shapes=scratch,
        compiler_params=pltpu.CompilerParams(
            vmem_limit_bytes=100 * 1024 * 1024,
            disable_semaphore_checks=True,
            disable_bounds_checks=True,
        ),
    )(*ins)
```

```python
import os
import jax
import jax.numpy as jnp
from jax import lax
import jax.experimental.pallas as pl
import jax.experimental.pallas.tpu as pltpu

bf16 = jnp.bfloat16
f32 = jnp.float32
u32 = jnp.uint32
i32 = jnp.int32

M = 640
H = 32
D = 128
SK = 4096
DC = 512
F = 1728
NJ = M // 128
NC = DC // 128
NK = SK // 128
NF = (F + 127) // 128
LOG2E = 1.4426950408889634
EPS = 1e-5

REGIONS = True
REGIONS1 = True
NODMA = False
STOP1 = int(os.environ.get('STOP1', '99'))
STOP = int(os.environ.get('STOP', '99'))

Q_MXU = 4
Q_GROUPS = [4] * 7
O_VPU = 23
F_GROUPS = [2, 2, 2, 2]
F_VPU = sum(F_GROUPS)
Q_VPU = H - Q_MXU
assert sum(Q_GROUPS) == Q_VPU and Q_MXU % 2 == 0

WO_CHUNKS = 4
WU_CHUNKS = [(0, 512), (4, 512), (8, 384), (11, 320)]
WD_CHUNKS = [(0, 384), (384, 384), (768, 384), (1152, 256), (1408, 128), (1536, 128), (1664, 64)]


def _dot(a, b):
    return jnp.dot(a, b, preferred_element_type=f32)


def _iota(shape, dim):
    return lax.broadcasted_iota(i32, shape, dim)


def _layernorm(x):
    m = jnp.mean(x, axis=-1, keepdims=True)
    xc = x - m
    v = jnp.mean(xc * xc, axis=-1, keepdims=True)
    return xc * lax.rsqrt(v + EPS)


def _as_u32(a):
    return pltpu.bitcast(a, u32)


def _as_bf16(a):
    return pltpu.bitcast(a, bf16)


def _lo(w):
    return pltpu.bitcast(w << 16, f32)


def _hi(w):
    return pltpu.bitcast(w & jnp.uint32(0xFFFF0000), f32)


def _widen(v):
    v = v[0:8, :]
    return jnp.concatenate([v] * 5, axis=1)


def _rowsum(acc):
    return jnp.broadcast_to(jnp.sum(acc, axis=0, keepdims=True), (8, 128))


def _kernel(x_hbm, wr_hbm, wq_hbm, wuk_hbm, c_hbm, wuv_hbm, wo_hbm, wg_hbm, wu_hbm, wd_hbm,
            o_hbm,
            x_v, wr_v, wq_v, wuk_v, wuv_v, wo_v, wg_v, wu_v, wd_v,
            wqb, wqf, ukb, cT, c2, uvb, wob, wof, gub, guf, wdb, xt0, xt1, xt2, xt3, xt4, s_v, o_v, sems, zsem):
    cps = {}
    names = []
    families = {}

    class _No:
        def wait(self): pass
    def add(name, src, dst):
        if NODMA and name not in ("x", "wr"):
            cps[name] = _No(); return
        cp = pltpu.make_async_copy(src, dst, sems.at[len(cps)])
        cp.start()
        cps[name] = cp
        names.append(name)

    def add_pairs(name, src, dst):
        s32 = src.bitcast(u32)
        families[name + "0"] = (s32, dst)
        for hp in range(H // 2):
            add(f"{name}{hp}", s32.at[:, hp, :], dst.at[hp])

    add("x", x_hbm, x_v)
    add("wr", wr_hbm, wr_v)
    add_pairs("wq", wq_hbm, wq_v)
    add_pairs("wuk", wuk_hbm, wuk_v)
    c32 = c_hbm.bitcast(u32)
    for cb in range(NC):
        add(f"c{cb}", c32.at[:, pl.ds(cb * 128, 128)], c2.at[cb])
    add_pairs("wuv", wuv_hbm, wuv_v)
    add("wg", wg_hbm, wg_v)
    hpc = H // WO_CHUNKS
    for i in range(WO_CHUNKS):
        add(f"wo{i}", wo_hbm.at[pl.ds(i * hpc * D, hpc * D)], wo_v.at[pl.ds(i * hpc * D, hpc * D)])
    for i, (s, n) in enumerate(WU_CHUNKS):
        add(f"wu{i}", wu_hbm.at[pl.ds(128 * s, n)], wu_v.at[pl.ds(128 * s, n)])
    for i, (s, n) in enumerate(WD_CHUNKS):
        add(f"wd{i}", wd_hbm.at[pl.ds(s, n)], wd_v.at[pl.ds(s, n)])

    def cps_wait_dyn(first_name, hp):
        if NODMA:
            return
        src, dst = families[first_name]
        pltpu.make_async_copy(src.at[:, hp, :], dst.at[hp], sems.at[names.index(first_name) + hp]).wait()

    sub = _iota((8, 128), 0)
    xts = [xt0, xt1, xt2, xt3, xt4]
    zs = [pl.semaphore_read(zsem.at[n_]) for n_ in range(32)]
    z0 = zs[0]
    zvec = jnp.zeros((8, 128), u32) + zs[-1].astype(u32)
    zi = iter(zs[1:-1])

    def repack(src, hp, dst, rows):
        for i in range(rows // 16):
            v = src[hp, pl.ds(16 * i, 16), :]
            dst[2 * hp, pl.ds(8 * i, 8), :] = _as_u32(_lo(v).astype(bf16))
            dst[2 * hp + 1, pl.ds(8 * i, 8), :] = _as_u32(_hi(v).astype(bf16))

    def prep_wq():
        for hp in range(Q_MXU // 2):
            cps[f"wq{hp}"].wait()
            repack(wq_v, hp, wqb, M)

        def vpu_pair(k, carry):
            hp = k + Q_MXU // 2
            cps_wait_dyn("wq0", hp)
            v = wq_v[hp]
            wqf[2 * k] = _lo(v)
            wqf[2 * k + 1] = _hi(v)
            return carry
        lax.fori_loop(0, Q_VPU // 2, vpu_pair, 0)

    def prep_wuk():
        def pair(hp, carry):
            cps_wait_dyn("wuk0", hp)
            for cb in range(NC):
                t = wuk_v[hp, pl.ds(cb * 128, 128), :].T
                ukb[2 * hp, pl.ds(cb * 64, 64), :] = _as_u32(_lo(t).astype(bf16))
                ukb[2 * hp + 1, pl.ds(cb * 64, 64), :] = _as_u32(_hi(t).astype(bf16))
            return carry
        lax.fori_loop(0, 16, pair, 0)

    def prep_c():
        for cb in range(NC):
            cps[f"c{cb}"].wait()

            def blk(i, carry, cb=cb):
                for kk in range(16):
                    kb = 16 * i + kk
                    t = _as_bf16(c2[cb, pl.ds(pl.multiple_of(kb * 64, 64), 64), :])
                    cT[kb, pl.ds(cb * 64, 64), :] = _as_u32(t.T)
                return carry
            lax.fori_loop(0, NK // 16, blk, 0)

    def prep_wuv():
        def pair(hp, carry):
            cps_wait_dyn("wuv0", hp)
            repack(wuv_v, hp, uvb, DC)
            return carry
        lax.fori_loop(0, 16, pair, 0)

    def prep_gu(mat, raw, fb0, fb1):
        def vpu_blk(fb, carry):
            for j in range(NJ):
                t = raw[pl.ds(pl.multiple_of(fb * 128, 128), 128), pl.ds(j * 128, 128)].T
                guf[2 * fb + mat, pl.ds(j * 128, 128), :] = t.astype(f32)
            return carry
        if fb0 < F_VPU:
            lax.fori_loop(fb0, min(fb1, F_VPU), vpu_blk, 0)

        def mxu_blk(fb, carry):
            for j in range(NJ):
                t = raw[pl.ds(pl.multiple_of(fb * 128, 128), 128), pl.ds(j * 128, 128)].T
                gub[2 * (fb - F_VPU) + mat, pl.ds(j * 64, 64), :] = _as_u32(t)
            return carry
        lo, hi = max(fb0, F_VPU), min(fb1, NF - 1)
        if lo < hi:
            lax.fori_loop(lo, hi, mxu_blk, 0)
        if fb1 == NF:
            for j in range(NJ):
                t = raw[pl.ds((NF - 1) * 128, 64), pl.ds(j * 128, 128)]
                t = jnp.concatenate([t, jnp.zeros((64, 128), bf16)], axis=0).T
                gub[2 * (NF - 1 - F_VPU) + mat, pl.ds(j * 64, 64), :] = _as_u32(t)

    def prep_wo(h0, h1):
        def vpu_head(h, carry):
            for j in range(NJ):
                t = wo_v[pl.ds(pl.multiple_of(h * 128, 128), 128), pl.ds(j * 128, 128)]
                wof[h * NJ + j] = t.astype(f32)
            return carry

        def mxu_head(h, carry):
            for j in range(NJ):
                t = wo_v[pl.ds(pl.multiple_of(h * 128, 128), 128), pl.ds(j * 128, 128)]
                wob[(h - O_VPU) * NJ + j] = _as_u32(t)
            return carry
        if h0 < O_VPU:
            lax.fori_loop(h0, min(h1, O_VPU), vpu_head, 0)
        if h1 > O_VPU:
            lax.fori_loop(max(h0, O_VPU), h1, mxu_head, 0)

    def stage_xt(xb):
        for kb in range(NJ):
            t = jnp.broadcast_to(xb[0:1, kb * 128:(kb + 1) * 128], (128, 128)).T
            xts[kb][pl.ds(0, 128), :] = t.astype(f32)

    def vpu_cols(wref, idxs, static, prev):
        accs = [None] * len(idxs)
        if not static:
            zf = next(zi)
            for kb in range(NJ):
                xts[kb][pl.ds(zf + 128, 8), :] = pltpu.bitcast(zvec, f32)
        for i in range(M // 8):
            xt = xts[i // 16][pl.ds(8 * (i % 16), 8), :]
            for n, c in enumerate(idxs):
                p = xt * wref[c, pl.ds(8 * i, 8), :]
                if accs[n] is None:
                    if prev:
                        p = p + pltpu.bitcast(_as_u32(prev[n % len(prev)]) & zvec, f32)
                    accs[n] = p
                else:
                    accs[n] = accs[n] + p
        prev[:] = accs
        return [_rowsum(a) for a in accs]

    def region(fn, first, zero):
        if (first and not REGIONS1) or not REGIONS:
            return fn()
        return lax.cond(zs[0] == 0, fn, lambda: zero)

    def phase_a(xb, first):
        stage_xt(xb)
        qabs = [[None] * NC for _ in range(4)]

        def s2(h, qh):
            qb = qh.astype(bf16)
            for cb in range(NC):
                y = _dot(qb, _as_bf16(ukb[h, pl.ds(cb * 64, 64), :]))
                old = qabs[h // 8][cb]
                qabs[h // 8][cb] = y if old is None else jnp.where(sub == h % 8, y, old)

        for h in range(Q_MXU):
            s2(h, _dot(xb, _as_bf16(wqb[h])))
        h0 = 0
        prev = []
        for gsz in Q_GROUPS:
            qs = vpu_cols(wqf, list(range(h0, h0 + gsz)), h0 == 0, prev)
            for n in range(gsz):
                s2(Q_MXU + h0 + n, qs[n])
            h0 += gsz
        scale = (D ** -0.5) * LOG2E
        qa = jnp.concatenate([jnp.concatenate(qabs[g], axis=1) for g in range(4)], axis=0)
        return (qa * scale).astype(bf16)

    def phase_b(qa):
        mrun = None
        for kb in range(NK):
            s = _dot(qa, _as_bf16(cT[kb]))
            s_v[kb] = s
            mrun = s if mrun is None else jnp.maximum(mrun, s)
        mrow = jnp.max(mrun, axis=-1, keepdims=True)
        lsum = None
        cacc = [None] * NC
        for kb in range(NK):
            p = jnp.exp2(s_v[kb] - mrow)
            lsum = p if lsum is None else lsum + p
            pb = p.astype(bf16)
            for cb in range(NC):
                y = _dot(pb, _as_bf16(c2[cb, pl.ds(kb * 64, 64), :]))
                cacc[cb] = y if cacc[cb] is None else cacc[cb] + y
        linv = 1.0 / jnp.sum(lsum, axis=-1, keepdims=True)
        return jnp.concatenate([(cacc[cb] * linv).astype(bf16) for cb in range(NC)], axis=1)

    def phase_c(cx):
        vacc = [None] * NJ
        macc = [None] * NJ
        ys = {}
        la = 4
        for i in range(H + la):
            if i < H:
                g = i // 8
                ys[i] = _dot(cx[8 * g:8 * g + 8, :], _as_bf16(uvb[i]))
            h = i - la
            if h < 0:
                continue
            yb = ys[h][h % 8:h % 8 + 1, :].astype(bf16)
            if h < O_VPU:
                xt = jnp.broadcast_to(yb, (128, 128)).T.astype(f32)
                for ii in range(D // 8):
                    for j in range(NJ):
                        p = xt[8 * ii:8 * ii + 8, :] * wof[h * NJ + j, pl.ds(8 * ii, 8), :]
                        vacc[j] = p if vacc[j] is None else vacc[j] + p
            else:
                lhs = jnp.broadcast_to(yb, (8, 128))
                for j in range(NJ):
                    yy = _dot(lhs, _as_bf16(wob[(h - O_VPU) * NJ + j]))
                    macc[j] = yy if macc[j] is None else macc[j] + yy
        return jnp.concatenate([_rowsum(vacc[j]) + macc[j] for j in range(NJ)], axis=1)

    def phase_d(xb, first):
        stage_xt(xb)
        yacc = [None] * NJ
        waited = set()

        def s9(fb, hb):
            if first:
                for i, (s0, n0) in enumerate(WD_CHUNKS):
                    if s0 < (fb + 1) * 128 and s0 + n0 > fb * 128 and i not in waited:
                        cps[f"wd{i}"].wait()
                        waited.add(i)
            for j in range(NJ):
                if first:
                    n = min(128, F - fb * 128)
                    t = wd_v[pl.ds(fb * 128, n), pl.ds(j * 128, 128)]
                    if n < 128:
                        t = jnp.concatenate([t, jnp.zeros((128 - n, 128), bf16)], axis=0)
                    wdb[z0 + fb * NJ + j] = _as_u32(t)
                else:
                    t = _as_bf16(wdb[fb * NJ + j])
                yy = _dot(hb, t)
                yacc[j] = yy if yacc[j] is None else yacc[j] + yy

        hs = {}
        for i in range(NF - F_VPU):
            g = _dot(xb, _as_bf16(gub[2 * i]))
            u = _dot(xb, _as_bf16(gub[2 * i + 1]))
            hs[F_VPU + i] = (jax.nn.silu(g) * u).astype(bf16)
        if not first:
            for fb in range(F_VPU, NF):
                s9(fb, hs[fb])
        f0 = 0
        prev = []
        for gsz in F_GROUPS:
            ys = vpu_cols(guf, list(range(2 * f0, 2 * (f0 + gsz))), f0 == 0, prev)
            for n in range(gsz):
                hs[f0 + n] = (jax.nn.silu(ys[2 * n]) * ys[2 * n + 1]).astype(bf16)
                if not first:
                    s9(f0 + n, hs[f0 + n])
            f0 += gsz
        if first:
            for fb in range(NF):
                s9(fb, hs[fb])
        return jnp.concatenate(yacc, axis=1)

    def attn(x, first):
        xb = _layernorm(x).astype(bf16)
        if first:
            prep_wq()
            prep_wuk()
        if first and STOP1 == 1: return _widen(ukb[3, pl.ds(0, 8), :].astype(f32) + wqf[3, pl.ds(0, 8), :])
        qa = region(lambda: phase_a(xb, first), first, jnp.zeros((H, DC), bf16))
        if first and STOP1 == 2: return _widen(sum((qa[8*i:8*i+8, 128*j:128*j+128].astype(f32) for i in range(4) for j in range(4))))
        if not first and STOP == 2: return _widen(sum((qa[8*i:8*i+8, 128*j:128*j+128].astype(f32) for i in range(4) for j in range(4))))
        if first:
            prep_c()
        if first and STOP1 == 3: return _widen(cT[3, pl.ds(0, 8), :].astype(f32) + qa[0:8, 0:128])
        cx = region(lambda: phase_b(qa), first, jnp.zeros((H, DC), bf16))
        if first and STOP1 == 4: return _widen(cx[0:8, 0:128].astype(f32))
        if not first and STOP == 5: return _widen(sum((cx[8*i:8*i+8, 128*j:128*j+128].astype(f32) for i in range(4) for j in range(4))))
        if first:
            prep_wuv()
            if STOP1 == 5: return _widen(cx[0:8, 0:128].astype(f32) + uvb[3, pl.ds(0, 8), :].astype(f32))
            cps["wg"].wait()
            prep_gu(0, wg_v, 0, NF)
            if STOP1 == 6: return _widen(cx[0:8, 0:128].astype(f32) + uvb[3, pl.ds(0, 8), :].astype(f32) + guf[1, pl.ds(0, 8), :])
            for i in range(WO_CHUNKS):
                cps[f"wo{i}"].wait()
                prep_wo(i * hpc, (i + 1) * hpc)
        if first and STOP1 == 7: return _widen(cx[0:8, 0:128].astype(f32) + uvb[3, pl.ds(0, 8), :].astype(f32) + guf[1, pl.ds(0, 8), :] + wof[1, pl.ds(0, 8), :])
        return region(lambda: phase_c(cx), first, jnp.zeros((8, M), f32))

    def ffn(x, first):
        xn = _layernorm(x)
        xb = xn.astype(bf16)
        r = jnp.sum(xb.astype(f32) * wr, axis=-1, keepdims=True)
        rs = jax.nn.sigmoid(r)
        if first:
            for i, (s0, n0) in enumerate(WU_CHUNKS):
                cps[f"wu{i}"].wait()
                prep_gu(1, wu_v, s0, s0 + (n0 + 127) // 128)
        y = region(lambda: phase_d(xb, first), first, jnp.zeros((8, M), f32))
        return xn + (xn * 0.0 + y * rs)

    cps["x"].wait()
    cps["wr"].wait()
    x = jnp.broadcast_to(x_v[0].astype(f32), (8, M))
    wr = wr_v[...].astype(f32).reshape(1, M)
    x = x + attn(x, True)
    if STOP1 > 8: x = x + ffn(x, True)
    if STOP > 0: x = x + attn(x, False)
    if STOP > 7: x = x + ffn(x, False)
    o_v[0] = x[0:1, :].astype(bf16)
    ocp = pltpu.make_async_copy(o_v, o_hbm, sems.at[len(cps)])
    ocp.start()
    ocp.wait()


@jax.jit
def pallas_interleave_layers__compressed_kv_cla__moe_arch_mod__decode_kernel(
    A_x, A_c_kv, A_w_q, A_w_uk, A_w_uv, A_w_o, B_x, B_w_r, B_w_gate, B_w_up, B_w_down,
):
    del B_x
    hbm = lambda a: pltpu.with_memory_space_constraint(a, pltpu.HBM)
    ins = [
        A_x, B_w_r,
        A_w_q,
        A_w_uk,
        A_c_kv.reshape(SK, DC),
        A_w_uv,
        A_w_o.reshape(H * D, M),
        B_w_gate.T, B_w_up.T, B_w_down,
    ]
    ins = [hbm(a) for a in ins]
    scratch = [
        pltpu.VMEM((1, 1, M), bf16),
        pltpu.VMEM((M,), bf16),
        pltpu.VMEM((H // 2, M, D), u32),
        pltpu.VMEM((H // 2, DC, D), u32),
        pltpu.VMEM((H // 2, DC, D), u32),
        pltpu.VMEM((H * D, M), bf16),
        pltpu.VMEM((F, M), bf16),
        pltpu.VMEM((F, M), bf16),
        pltpu.VMEM((F, M), bf16),
        pltpu.VMEM((Q_MXU, M // 2, 128), u32),
        pltpu.VMEM((Q_VPU, M, 128), f32),
        pltpu.VMEM((H, NC * 64, 128), u32),
        pltpu.VMEM((NK, DC // 2, 128), u32),
        pltpu.VMEM((NC, SK // 2, 128), u32),
        pltpu.VMEM((H, DC // 2, 128), u32),
        pltpu.VMEM(((H - O_VPU) * NJ, 64, 128), u32),
        pltpu.VMEM((O_VPU * NJ, 128, 128), f32),
        pltpu.VMEM((2 * (NF - F_VPU), M // 2, 128), u32),
        pltpu.VMEM((2 * F_VPU, M, 128), f32),
        pltpu.VMEM((NF * NJ, 64, 128), u32),
        pltpu.VMEM((160, 128), f32),
        pltpu.VMEM((160, 128), f32),
        pltpu.VMEM((160, 128), f32),
        pltpu.VMEM((160, 128), f32),
        pltpu.VMEM((160, 128), f32),
        pltpu.VMEM((NK, H, 128), f32),
        pltpu.VMEM((1, 1, M), bf16),
        pltpu.SemaphoreType.DMA((80,)),
        pltpu.SemaphoreType.REGULAR((32,)),
    ]
    return pl.pallas_call(
        _kernel,
        in_specs=[pl.BlockSpec(memory_space=pl.ANY)] * len(ins),
        out_specs=pl.BlockSpec(memory_space=pl.ANY),
        out_shape=jax.ShapeDtypeStruct((1, 1, M), bf16),
        scratch_shapes=scratch,
        compiler_params=pltpu.CompilerParams(
            vmem_limit_bytes=120 * 1024 * 1024,
            disable_semaphore_checks=True,
            disable_bounds_checks=True,
            flags={"XLA_TPU_FORCE_LP_LLO_SCHEDULER": True},
        ),
    )(*ins)
```

```python
import os
import jax
import jax.numpy as jnp
from jax import lax
import jax.experimental.pallas as pl
import jax.experimental.pallas.tpu as pltpu

bf16 = jnp.bfloat16
f32 = jnp.float32
u32 = jnp.uint32
i32 = jnp.int32

M = 640
H = 32
D = 128
SK = 4096
DC = 512
F = 1728
NJ = M // 128
NC = DC // 128
NK = SK // 128
NF = (F + 127) // 128
LOG2E = 1.4426950408889634
EPS = 1e-5

REGIONS = False
REGIONS1 = True
NODMA = False
STOP1 = int(os.environ.get('STOP1', '99'))
STOP = int(os.environ.get('STOP', '99'))

Q_MXU = 8
Q_GROUPS = [5, 5, 4, 4, 4, 2]
O_VPU = 23
F_GROUPS = [2, 2, 2, 2]
F_VPU = sum(F_GROUPS)
Q_VPU = H - Q_MXU
assert sum(Q_GROUPS) == Q_VPU and Q_MXU % 2 == 0

WO_CHUNKS = 4
WU_CHUNKS = [(0, 512), (4, 512), (8, 384), (11, 320)]
WD_CHUNKS = [(0, 384), (384, 384), (768, 384), (1152, 256), (1408, 128), (1536, 128), (1664, 64)]


def _dot(a, b):
    return jnp.dot(a, b, preferred_element_type=f32)


def _iota(shape, dim):
    return lax.broadcasted_iota(i32, shape, dim)


def _ln_parts(x):
    m = jnp.sum(x, axis=-1, keepdims=True) * (1.0 / M)
    m2 = jnp.sum(x * x, axis=-1, keepdims=True) * (1.0 / M)
    v = jnp.maximum(m2 - m * m, 0.0)
    return x - m, lax.rsqrt(v + EPS)


def _as_u32(a):
    return pltpu.bitcast(a, u32)


def _as_bf16(a):
    return pltpu.bitcast(a, bf16)


def _lo(w):
    return pltpu.bitcast(w << 16, f32)


def _hi(w):
    return pltpu.bitcast(w & jnp.uint32(0xFFFF0000), f32)


def _widen(v):
    v = v[0:8, :]
    return jnp.concatenate([v] * 5, axis=1)


def _rowsum(acc):
    return jnp.broadcast_to(jnp.sum(acc, axis=0, keepdims=True), (8, 128))


def _kernel(x_hbm, wr_hbm, wq_hbm, wuk_hbm, c_hbm, wuv_hbm, wo_hbm, wg_hbm, wu_hbm, wd_hbm,
            o_hbm,
            x_v, wr_v, wq_v, wuk_v, wuv_v, wo_v, wg_v, wu_v, wd_v,
            wqb, wqf, ukb, cT, c2, uvb, wob, wof, gub, guf, wdb, xt0, xt1, xt2, xt3, xt4, s_v, o_v, sems, zsem):
    cps = {}
    names = []
    families = {}

    class _No:
        def wait(self): pass
    def add(name, src, dst):
        if NODMA and name not in ("x", "wr"):
            cps[name] = _No(); return
        cp = pltpu.make_async_copy(src, dst, sems.at[len(cps)])
        cp.start()
        cps[name] = cp
        names.append(name)

    def add_pairs(name, src, dst):
        s32 = src.bitcast(u32)
        families[name + "0"] = (s32, dst)
        for hp in range(H // 2):
            add(f"{name}{hp}", s32.at[:, hp, :], dst.at[hp])

    add("x", x_hbm, x_v)
    add("wr", wr_hbm, wr_v)
    add_pairs("wq", wq_hbm, wq_v)
    add_pairs("wuk", wuk_hbm, wuk_v)
    c32 = c_hbm.bitcast(u32)
    for cb in range(NC):
        add(f"c{cb}", c32.at[:, pl.ds(cb * 128, 128)], c2.at[cb])
    add_pairs("wuv", wuv_hbm, wuv_v)
    add("wg", wg_hbm, wg_v)
    hpc = H // WO_CHUNKS
    for i in range(WO_CHUNKS):
        add(f"wo{i}", wo_hbm.at[pl.ds(i * hpc * D, hpc * D)], wo_v.at[pl.ds(i * hpc * D, hpc * D)])
    for i, (s, n) in enumerate(WU_CHUNKS):
        add(f"wu{i}", wu_hbm.at[pl.ds(128 * s, n)], wu_v.at[pl.ds(128 * s, n)])
    for i, (s, n) in enumerate(WD_CHUNKS):
        add(f"wd{i}", wd_hbm.at[pl.ds(s, n)], wd_v.at[pl.ds(s, n)])

    def cps_wait_dyn(first_name, hp):
        if NODMA:
            return
        src, dst = families[first_name]
        pltpu.make_async_copy(src.at[:, hp, :], dst.at[hp], sems.at[names.index(first_name) + hp]).wait()

    sub = _iota((8, 128), 0)
    xts = [xt0, xt1, xt2, xt3, xt4]
    zs = [pl.semaphore_read(zsem.at[n_]) for n_ in range(32)]
    z0 = zs[0]
    zvec = jnp.zeros((8, 128), u32) + zs[-1].astype(u32)
    zmask = zvec != 0
    zi = iter(zs[1:-1])

    def repack(src, hp, dst, rows):
        for i in range(rows // 16):
            v = src[hp, pl.ds(16 * i, 16), :]
            dst[2 * hp, pl.ds(8 * i, 8), :] = _as_u32(_lo(v).astype(bf16))
            dst[2 * hp + 1, pl.ds(8 * i, 8), :] = _as_u32(_hi(v).astype(bf16))

    def prep_wq():
        for hp in range(Q_MXU // 2):
            cps[f"wq{hp}"].wait()
            repack(wq_v, hp, wqb, M)

        def vpu_pair(k, carry):
            hp = k + Q_MXU // 2
            cps_wait_dyn("wq0", hp)
            v = wq_v[hp]
            wqf[2 * k] = _lo(v)
            wqf[2 * k + 1] = _hi(v)
            return carry
        lax.fori_loop(0, Q_VPU // 2, vpu_pair, 0)

    def prep_wuk():
        def pair(hp, carry):
            cps_wait_dyn("wuk0", hp)
            for cb in range(NC):
                t = wuk_v[hp, pl.ds(cb * 128, 128), :].T
                ukb[2 * hp, pl.ds(cb * 64, 64), :] = _as_u32(_lo(t).astype(bf16))
                ukb[2 * hp + 1, pl.ds(cb * 64, 64), :] = _as_u32(_hi(t).astype(bf16))
            return carry
        lax.fori_loop(0, 16, pair, 0)

    def prep_c():
        for cb in range(NC):
            cps[f"c{cb}"].wait()

            def blk(i, carry, cb=cb):
                for kk in range(16):
                    kb = 16 * i + kk
                    t = _as_bf16(c2[cb, pl.ds(pl.multiple_of(kb * 64, 64), 64), :])
                    cT[kb, pl.ds(cb * 64, 64), :] = _as_u32(t.T)
                return carry
            lax.fori_loop(0, NK // 16, blk, 0)

    def prep_wuv():
        def pair(hp, carry):
            cps_wait_dyn("wuv0", hp)
            repack(wuv_v, hp, uvb, DC)
            return carry
        lax.fori_loop(0, 16, pair, 0)

    def prep_gu(mat, raw, fb0, fb1):
        def vpu_blk(fb, carry):
            for j in range(NJ):
                t = raw[pl.ds(pl.multiple_of(fb * 128, 128), 128), pl.ds(j * 128, 128)].T
                guf[2 * fb + mat, pl.ds(j * 128, 128), :] = t.astype(f32)
            return carry
        if fb0 < F_VPU:
            lax.fori_loop(fb0, min(fb1, F_VPU), vpu_blk, 0)

        def mxu_blk(fb, carry):
            for j in range(NJ):
                t = raw[pl.ds(pl.multiple_of(fb * 128, 128), 128), pl.ds(j * 128, 128)].T
                gub[2 * (fb - F_VPU) + mat, pl.ds(j * 64, 64), :] = _as_u32(t)
            return carry
        lo, hi = max(fb0, F_VPU), min(fb1, NF - 1)
        if lo < hi:
            lax.fori_loop(lo, hi, mxu_blk, 0)
        if fb1 == NF:
            for j in range(NJ):
                t = raw[pl.ds((NF - 1) * 128, 64), pl.ds(j * 128, 128)]
                t = jnp.concatenate([t, jnp.zeros((64, 128), bf16)], axis=0).T
                gub[2 * (NF - 1 - F_VPU) + mat, pl.ds(j * 64, 64), :] = _as_u32(t)

    def prep_wo(h0, h1):
        def vpu_head(h, carry):
            for j in range(NJ):
                t = wo_v[pl.ds(pl.multiple_of(h * 128, 128), 128), pl.ds(j * 128, 128)]
                wof[h * NJ + j] = t.astype(f32)
            return carry

        def mxu_head(h, carry):
            for j in range(NJ):
                t = wo_v[pl.ds(pl.multiple_of(h * 128, 128), 128), pl.ds(j * 128, 128)]
                wob[(h - O_VPU) * NJ + j] = _as_u32(t)
            return carry
        if h0 < O_VPU:
            lax.fori_loop(h0, min(h1, O_VPU), vpu_head, 0)
        if h1 > O_VPU:
            lax.fori_loop(max(h0, O_VPU), h1, mxu_head, 0)

    def stage_xt(xb):
        for kb in range(NJ):
            t = jnp.broadcast_to(xb[0:1, kb * 128:(kb + 1) * 128], (128, 128)).T
            xts[kb][pl.ds(0, 128), :] = t.astype(f32)

    def vpu_cols(wref, idxs, static, prev):
        accs = [None] * len(idxs)
        if not static:
            zf = next(zi)
            for kb in range(NJ):
                xts[kb][pl.ds(zf + 128, 8), :] = pltpu.bitcast(zvec, f32)
        for i in range(M // 8):
            xt = xts[i // 16][pl.ds(8 * (i % 16), 8), :]
            for n, c in enumerate(idxs):
                p = xt * wref[c, pl.ds(8 * i, 8), :]
                if accs[n] is None:
                    if prev:
                        p = jnp.where(zmask, prev[n % len(prev)], p)
                    accs[n] = p
                else:
                    accs[n] = accs[n] + p
        prev[:] = accs
        return [_rowsum(a) for a in accs]

    def region(fn, first, zero):
        if (first and not REGIONS1) or not REGIONS:
            return fn()
        return lax.cond(zs[0] == 0, fn, lambda: zero)

    def phase_a(xb, rstd, first):
        stage_xt(xb)
        qabs = [[None] * NC for _ in range(4)]

        def s2(h, qh):
            qb = qh.astype(bf16)
            for cb in range(NC):
                y = _dot(qb, _as_bf16(ukb[h, pl.ds(cb * 64, 64), :]))
                old = qabs[h // 8][cb]
                qabs[h // 8][cb] = y if old is None else jnp.where(sub == h % 8, y, old)

        qm = [_dot(xb, _as_bf16(wqb[h])) for h in range(Q_MXU)]
        for h in range(Q_MXU):
            s2(h, qm[h])
        h0 = 0
        prev = []
        for gsz in Q_GROUPS:
            qs = vpu_cols(wqf, list(range(h0, h0 + gsz)), h0 == 0, prev)
            for n in range(gsz):
                s2(Q_MXU + h0 + n, qs[n])
            h0 += gsz
        scale = rstd[0:1, 0:1] * ((D ** -0.5) * LOG2E)
        qa = jnp.concatenate([jnp.concatenate(qabs[g], axis=1) for g in range(4)], axis=0)
        return (qa * scale).astype(bf16)

    def phase_b(qa):
        def s3(k0, k1):
            mrun = None
            for kb in range(k0, k1):
                s = _dot(qa, _as_bf16(cT[kb]))
                s_v[kb] = s
                mrun = s if mrun is None else jnp.maximum(mrun, s)
            return jnp.max(mrun, axis=-1, keepdims=True)

        def s5(k0, k1, mrow):
            lsum = None
            cacc = [None] * NC
            for kb in range(k0, k1):
                p = jnp.exp2(s_v[kb] - mrow)
                lsum = p if lsum is None else lsum + p
                pb = p.astype(bf16)
                for cb in range(NC):
                    y = _dot(pb, _as_bf16(c2[cb, pl.ds(kb * 64, 64), :]))
                    cacc[cb] = y if cacc[cb] is None else cacc[cb] + y
            return jnp.sum(lsum, axis=-1, keepdims=True), cacc

        hk = NK // 2
        ma = s3(0, hk)
        mb = s3(hk, NK)
        la, ca = s5(0, hk, ma)
        lb, cb_ = s5(hk, NK, mb)
        m = jnp.maximum(ma, mb)
        fa = jnp.exp2(ma - m)
        fb = jnp.exp2(mb - m)
        linv = 1.0 / (la * fa + lb * fb)
        wa = fa * linv
        wb = fb * linv
        return jnp.concatenate([(ca[c] * wa + cb_[c] * wb).astype(bf16) for c in range(NC)], axis=1)

    def phase_c(cx):
        vacc = [None] * NJ
        macc = [None] * NJ
        ys = {}
        la = 4
        for i in range(H + la):
            if i < H:
                g = i // 8
                ys[i] = _dot(cx[8 * g:8 * g + 8, :], _as_bf16(uvb[i]))
            h = i - la
            if 0 <= h < O_VPU:
                yb = ys[h][h % 8:h % 8 + 1, :].astype(bf16)
                xt = jnp.broadcast_to(yb, (128, 128)).T.astype(f32)
                for ii in range(D // 8):
                    for j in range(NJ):
                        p = xt[8 * ii:8 * ii + 8, :] * wof[h * NJ + j, pl.ds(8 * ii, 8), :]
                        vacc[j] = p if vacc[j] is None else vacc[j] + p
        for h in range(O_VPU, H):
            lhs = jnp.broadcast_to(ys[h][h % 8:h % 8 + 1, :].astype(bf16), (8, 128))
            for j in range(NJ):
                yy = _dot(lhs, _as_bf16(wob[(h - O_VPU) * NJ + j]))
                macc[j] = yy if macc[j] is None else macc[j] + yy
        return jnp.concatenate([_rowsum(vacc[j]) + macc[j] for j in range(NJ)], axis=1)

    def phase_d(xb, rstd, first):
        stage_xt(xb)
        yacc = [None] * NJ
        waited = set()

        def s9(fb, hb):
            if first:
                for i, (s0, n0) in enumerate(WD_CHUNKS):
                    if s0 < (fb + 1) * 128 and s0 + n0 > fb * 128 and i not in waited:
                        cps[f"wd{i}"].wait()
                        waited.add(i)
            for j in range(NJ):
                if first:
                    n = min(128, F - fb * 128)
                    t = wd_v[pl.ds(fb * 128, n), pl.ds(j * 128, 128)]
                    if n < 128:
                        t = jnp.concatenate([t, jnp.zeros((128 - n, 128), bf16)], axis=0)
                    wdb[z0 + fb * NJ + j] = _as_u32(t)
                else:
                    t = _as_bf16(wdb[fb * NJ + j])
                yy = _dot(hb, t)
                yacc[j] = yy if yacc[j] is None else yacc[j] + yy

        hs = {}
        for i in range(NF - F_VPU):
            g = _dot(xb, _as_bf16(gub[2 * i]))
            u = _dot(xb, _as_bf16(gub[2 * i + 1]))
            hs[F_VPU + i] = (jax.nn.silu(g * rstd) * (u * rstd)).astype(bf16)
        if not first:
            for fb in range(F_VPU, NF):
                s9(fb, hs[fb])
        f0 = 0
        prev = []
        for gsz in F_GROUPS:
            ys = vpu_cols(guf, list(range(2 * f0, 2 * (f0 + gsz))), f0 == 0, prev)
            for n in range(gsz):
                hs[f0 + n] = (jax.nn.silu(ys[2 * n] * rstd) * (ys[2 * n + 1] * rstd)).astype(bf16)
                if not first:
                    s9(f0 + n, hs[f0 + n])
            f0 += gsz
        if first:
            for fb in range(NF):
                s9(fb, hs[fb])
        return jnp.concatenate(yacc, axis=1)

    def attn(x, first):
        xc, rstd = _ln_parts(x)
        xb = xc.astype(bf16)
        if first:
            prep_wq()
            prep_wuk()
        if first and STOP1 == 1: return _widen(ukb[3, pl.ds(0, 8), :].astype(f32) + wqf[3, pl.ds(0, 8), :])
        qa = region(lambda: phase_a(xb, rstd, first), first, jnp.zeros((H, DC), bf16))
        if first and STOP1 == 2: return _widen(sum((qa[8*i:8*i+8, 128*j:128*j+128].astype(f32) for i in range(4) for j in range(4))))
        if not first and STOP == 2: return _widen(sum((qa[8*i:8*i+8, 128*j:128*j+128].astype(f32) for i in range(4) for j in range(4))))
        if first:
            prep_c()
        if first and STOP1 == 3: return _widen(cT[3, pl.ds(0, 8), :].astype(f32) + qa[0:8, 0:128])
        cx = region(lambda: phase_b(qa), first, jnp.zeros((H, DC), bf16))
        if first and STOP1 == 4: return _widen(cx[0:8, 0:128].astype(f32))
        if not first and STOP == 5: return _widen(sum((cx[8*i:8*i+8, 128*j:128*j+128].astype(f32) for i in range(4) for j in range(4))))
        if first:
            prep_wuv()
            if STOP1 == 5: return _widen(cx[0:8, 0:128].astype(f32) + uvb[3, pl.ds(0, 8), :].astype(f32))
            cps["wg"].wait()
            prep_gu(0, wg_v, 0, NF)
            if STOP1 == 6: return _widen(cx[0:8, 0:128].astype(f32) + uvb[3, pl.ds(0, 8), :].astype(f32) + guf[1, pl.ds(0, 8), :])
            for i in range(WO_CHUNKS):
                cps[f"wo{i}"].wait()
                prep_wo(i * hpc, (i + 1) * hpc)
        if first and STOP1 == 7: return _widen(cx[0:8, 0:128].astype(f32) + uvb[3, pl.ds(0, 8), :].astype(f32) + guf[1, pl.ds(0, 8), :] + wof[1, pl.ds(0, 8), :])
        return region(lambda: phase_c(cx), first, jnp.zeros((8, M), f32))

    def ffn(x, first):
        xc, rstd = _ln_parts(x)
        xn = xc * rstd
        xb = xc.astype(bf16)
        r = jnp.sum(xn.astype(bf16).astype(f32) * wr, axis=-1, keepdims=True)
        rs = jax.nn.sigmoid(r)
        if first:
            for i, (s0, n0) in enumerate(WU_CHUNKS):
                cps[f"wu{i}"].wait()
                prep_gu(1, wu_v, s0, s0 + (n0 + 127) // 128)
        y = region(lambda: phase_d(xb, rstd, first), first, jnp.zeros((8, M), f32))
        return xn + (xn * 0.0 + y * rs)

    cps["x"].wait()
    cps["wr"].wait()
    x = jnp.broadcast_to(x_v[0].astype(f32), (8, M))
    wr = wr_v[...].astype(f32).reshape(1, M)
    x = x + attn(x, True)
    if STOP1 > 8: x = x + ffn(x, True)
    if STOP > 0: x = x + attn(x, False)
    if STOP > 7: x = x + ffn(x, False)
    o_v[0] = x[0:1, :].astype(bf16)
    ocp = pltpu.make_async_copy(o_v, o_hbm, sems.at[len(cps)])
    ocp.start()
    ocp.wait()


@jax.jit
def pallas_interleave_layers__compressed_kv_cla__moe_arch_mod__decode_kernel(
    A_x, A_c_kv, A_w_q, A_w_uk, A_w_uv, A_w_o, B_x, B_w_r, B_w_gate, B_w_up, B_w_down,
):
    del B_x
    hbm = lambda a: pltpu.with_memory_space_constraint(a, pltpu.HBM)
    ins = [
        A_x, B_w_r,
        A_w_q,
        A_w_uk,
        A_c_kv.reshape(SK, DC),
        A_w_uv,
        A_w_o.reshape(H * D, M),
        B_w_gate.T, B_w_up.T, B_w_down,
    ]
    ins = [hbm(a) for a in ins]
    scratch = [
        pltpu.VMEM((1, 1, M), bf16),
        pltpu.VMEM((M,), bf16),
        pltpu.VMEM((H // 2, M, D), u32),
        pltpu.VMEM((H // 2, DC, D), u32),
        pltpu.VMEM((H // 2, DC, D), u32),
        pltpu.VMEM((H * D, M), bf16),
        pltpu.VMEM((F, M), bf16),
        pltpu.VMEM((F, M), bf16),
        pltpu.VMEM((F, M), bf16),
        pltpu.VMEM((Q_MXU, M // 2, 128), u32),
        pltpu.VMEM((Q_VPU, M, 128), f32),
        pltpu.VMEM((H, NC * 64, 128), u32),
        pltpu.VMEM((NK, DC // 2, 128), u32),
        pltpu.VMEM((NC, SK // 2, 128), u32),
        pltpu.VMEM((H, DC // 2, 128), u32),
        pltpu.VMEM(((H - O_VPU) * NJ, 64, 128), u32),
        pltpu.VMEM((O_VPU * NJ, 128, 128), f32),
        pltpu.VMEM((2 * (NF - F_VPU), M // 2, 128), u32),
        pltpu.VMEM((2 * F_VPU, M, 128), f32),
        pltpu.VMEM((NF * NJ, 64, 128), u32),
        pltpu.VMEM((160, 128), f32),
        pltpu.VMEM((160, 128), f32),
        pltpu.VMEM((160, 128), f32),
        pltpu.VMEM((160, 128), f32),
        pltpu.VMEM((160, 128), f32),
        pltpu.VMEM((NK, H, 128), f32),
        pltpu.VMEM((1, 1, M), bf16),
        pltpu.SemaphoreType.DMA((80,)),
        pltpu.SemaphoreType.REGULAR((32,)),
    ]
    return pl.pallas_call(
        _kernel,
        in_specs=[pl.BlockSpec(memory_space=pl.ANY)] * len(ins),
        out_specs=pl.BlockSpec(memory_space=pl.ANY),
        out_shape=jax.ShapeDtypeStruct((1, 1, M), bf16),
        scratch_shapes=scratch,
        compiler_params=pltpu.CompilerParams(
            vmem_limit_bytes=120 * 1024 * 1024,
            disable_semaphore_checks=True,
            disable_bounds_checks=True,
            flags={"XLA_TPU_FORCE_LP_LLO_SCHEDULER": True},
        ),
    )(*ins)
```

```python
import jax
import jax.numpy as jnp
from jax import lax
import jax.experimental.pallas as pl
import jax.experimental.pallas.tpu as pltpu

bf16 = jnp.bfloat16
f32 = jnp.float32
u32 = jnp.uint32
i32 = jnp.int32

M = 640
H = 32
D = 128
SK = 4096
DC = 512
F = 1728
NJ = M // 128
NC = DC // 128
NK = SK // 128
NF = (F + 127) // 128
LOG2E = 1.4426950408889634
EPS = 1e-5

REG1 = 'ABCD'
REG2 = 'C'

Q_MXU = 8
Q_GROUPS = [4, 4, 4, 4, 4, 4]
O_VPU = 24
F_GROUPS = [2, 2, 2, 2]
F_VPU = sum(F_GROUPS)
Q_VPU = H - Q_MXU
assert sum(Q_GROUPS) == Q_VPU and Q_MXU % 2 == 0 and F_VPU % 2 == 0

WO_CHUNKS = 4
WU_CHUNKS = [(0, 512), (4, 512), (8, 384), (11, 320)]
WD_CHUNKS = [(0, 384), (384, 384), (768, 384), (1152, 256), (1408, 128), (1536, 128), (1664, 64)]
NZ = 32


def _dot(a, b):
    return jnp.dot(a, b, preferred_element_type=f32)


def _u32(a):
    return pltpu.bitcast(a, u32)


def _bf16(a):
    return pltpu.bitcast(a, bf16)


def _lo(w):
    return pltpu.bitcast(w << 16, f32)


def _hi(w):
    return pltpu.bitcast(w & jnp.uint32(0xFFFF0000), f32)


def _rowsum(acc):
    return jnp.broadcast_to(jnp.sum(acc, axis=0, keepdims=True), (8, 128))


def _ln_parts(x):
    m = jnp.sum(x, axis=-1, keepdims=True) * (1.0 / M)
    m2 = jnp.sum(x * x, axis=-1, keepdims=True) * (1.0 / M)
    v = jnp.maximum(m2 - m * m, 0.0)
    return x - m, lax.rsqrt(v + EPS), m


def _xpose_bcast(row):
    r16 = jnp.broadcast_to(row, (16, 128)).astype(bf16)
    return jnp.concatenate([r16] * 8, axis=0).T.astype(f32)


def _kernel(x_hbm, wr_hbm, wq_hbm, wuk_hbm, c_hbm, wuv_hbm, wo_hbm, wg_hbm, wu_hbm, wd_hbm,
            o_hbm,
            x_v, wr_v, wq_v, wuk_v, wuv_v, wo_v, wg_v, wu_v, wd_v,
            wqb, wqf, ukb, cT, c2, uvb, wob, wof, gub, guf, wdb, xt0, xt1, xt2, xt3, xt4, s_v, o_v, sems, zsem):
    cps = {}
    names = []
    families = {}

    def add(name, src, dst):
        cp = pltpu.make_async_copy(src, dst, sems.at[len(names)])
        cp.start()
        cps[name] = cp
        names.append(name)

    def add_pairs(name, src, dst):
        s32 = src.bitcast(u32)
        families[name] = (s32, dst, len(names))
        for hp in range(H // 2):
            add(f"{name}{hp}", s32.at[:, hp, :], dst.at[hp])

    def wait_pair(name, hp):
        src, dst, base = families[name]
        pltpu.make_async_copy(src.at[:, hp, :], dst.at[hp], sems.at[base + hp]).wait()

    add("x", x_hbm, x_v)
    add("wr", wr_hbm, wr_v)
    add_pairs("wq", wq_hbm, wq_v)
    add_pairs("wuk", wuk_hbm, wuk_v)
    c32 = c_hbm.bitcast(u32)
    for cb in range(NC):
        add(f"c{cb}", c32.at[:, pl.ds(cb * 128, 128)], c2.at[cb])
    add_pairs("wuv", wuv_hbm, wuv_v)
    add("wg", wg_hbm, wg_v)
    hpc = H // WO_CHUNKS
    for i in range(WO_CHUNKS):
        add(f"wo{i}", wo_hbm.at[pl.ds(i * hpc * D, hpc * D)], wo_v.at[pl.ds(i * hpc * D, hpc * D)])
    for i, (s, n) in enumerate(WU_CHUNKS):
        add(f"wu{i}", wu_hbm.at[pl.ds(128 * s, n)], wu_v.at[pl.ds(128 * s, n)])
    for i, (s, n) in enumerate(WD_CHUNKS):
        add(f"wd{i}", wd_hbm.at[pl.ds(s, n)], wd_v.at[pl.ds(s, n)])

    sub = lax.broadcasted_iota(i32, (8, 128), 0)
    xts = [xt0, xt1, xt2, xt3, xt4]
    zs = [pl.semaphore_read(zsem.at[n]) for n in range(NZ)]
    z0 = zs[0]
    zvec = jnp.zeros((8, 128), u32) + zs[-1].astype(u32)
    zmask = zvec != 0
    zi = iter(zs[1:-1])

    def repack(src, hp, dst, rows):
        for i in range(rows // 16):
            v = src[hp, pl.ds(16 * i, 16), :]
            dst[2 * hp, pl.ds(8 * i, 8), :] = _u32(_lo(v).astype(bf16))
            dst[2 * hp + 1, pl.ds(8 * i, 8), :] = _u32(_hi(v).astype(bf16))

    def prep_wq():
        for hp in range(Q_MXU // 2):
            cps[f"wq{hp}"].wait()
            repack(wq_v, hp, wqb, M)

        def vpu_pair(k, carry):
            hp = k + Q_MXU // 2
            wait_pair("wq", hp)
            v = wq_v[hp]
            wqf[2 * k] = _lo(v)
            wqf[2 * k + 1] = _hi(v)
            return carry
        lax.fori_loop(0, Q_VPU // 2, vpu_pair, 0)

    def prep_wuk():
        def pair(hp, carry):
            wait_pair("wuk", hp)
            for cb in range(NC):
                t = wuk_v[hp, pl.ds(cb * 128, 128), :].T
                ukb[2 * hp, pl.ds(cb * 64, 64), :] = _u32(_lo(t).astype(bf16))
                ukb[2 * hp + 1, pl.ds(cb * 64, 64), :] = _u32(_hi(t).astype(bf16))
            return carry
        lax.fori_loop(0, H // 2, pair, 0)

    def prep_c():
        for cb in range(NC):
            cps[f"c{cb}"].wait()

            def blk(i, carry, cb=cb):
                for kk in range(16):
                    kb = 16 * i + kk
                    t = _bf16(c2[cb, pl.ds(pl.multiple_of(kb * 64, 64), 64), :])
                    cT[kb, pl.ds(cb * 64, 64), :] = _u32(t.T)
                return carry
            lax.fori_loop(0, NK // 16, blk, 0)

    def prep_wuv():
        def pair(hp, carry):
            wait_pair("wuv", hp)
            repack(wuv_v, hp, uvb, DC)
            return carry
        lax.fori_loop(0, H // 2, pair, 0)

    def prep_gu(mat, raw, fb0, fb1):
        def tile(fb, j):
            return raw[pl.ds(pl.multiple_of(fb * 128, 128), 128), pl.ds(j * 128, 128)].T

        def vpu_blks(i, carry):
            for fb in (2 * i, 2 * i + 1):
                for j in range(NJ):
                    guf[2 * fb + mat, pl.ds(j * 128, 128), :] = tile(fb, j).astype(f32)
            return carry
        if fb0 < F_VPU:
            lax.fori_loop(fb0 // 2, min(fb1, F_VPU) // 2, vpu_blks, 0)

        for fb in range(max(fb0, F_VPU), min(fb1, NF - 1)):
            for j in range(NJ):
                gub[z0 + 2 * (fb - F_VPU) + mat, pl.ds(j * 64, 64), :] = _u32(tile(fb, j))
        if fb1 == NF:
            for j in range(NJ):
                t = raw[pl.ds((NF - 1) * 128, 64), pl.ds(j * 128, 128)]
                t = jnp.concatenate([t, jnp.zeros((64, 128), bf16)], axis=0).T
                gub[z0 + 2 * (NF - 1 - F_VPU) + mat, pl.ds(j * 64, 64), :] = _u32(t)

    def prep_wo(h0, h1):
        def vpu_head(h, carry):
            for j in range(NJ):
                t = wo_v[pl.ds(pl.multiple_of(h * 128, 128), 128), pl.ds(j * 128, 128)]
                wof[h * NJ + j] = t.astype(f32)
            return carry

        def mxu_head(h, carry):
            for j in range(NJ):
                t = wo_v[pl.ds(pl.multiple_of(h * 128, 128), 128), pl.ds(j * 128, 128)]
                wob[(h - O_VPU) * NJ + j] = _u32(t)
            return carry
        if h0 < O_VPU:
            lax.fori_loop(h0, min(h1, O_VPU), vpu_head, 0)
        if h1 > O_VPU:
            lax.fori_loop(max(h0, O_VPU), h1, mxu_head, 0)

    def stage_xt(x, mean):
        for kb in range(NJ):
            t = _xpose_bcast(x[0:1, kb * 128:(kb + 1) * 128])
            xts[kb][pl.ds(0, 128), :] = t - mean[0:1, 0:1]

    def vpu_cols(wref, idxs, static, prev):
        accs = [None] * len(idxs)
        if not static:
            zf = next(zi)
            for kb in range(NJ):
                xts[kb][pl.ds(zf + 128, 8), :] = pltpu.bitcast(zvec, f32)
        for i in range(M // 8):
            xt = xts[i // 16][pl.ds(8 * (i % 16), 8), :]
            for n, c in enumerate(idxs):
                p = xt * wref[c, pl.ds(8 * i, 8), :]
                if accs[n] is None:
                    if prev:
                        p = jnp.where(zmask, prev[n % len(prev)], p)
                    accs[n] = p
                else:
                    accs[n] = accs[n] + p
        prev[:] = accs
        return [_rowsum(a) for a in accs]

    def region(fn, first, zero, tag):
        if tag not in (REG1 if first else REG2):
            return fn()
        return lax.cond(z0 == 0, fn, lambda: zero)

    def phase_a(x, xb, mean, rstd):
        stage_xt(x, mean)
        qabs = [[None] * NC for _ in range(4)]

        def absorb(h, qh):
            qb = qh.astype(bf16)
            for cb in range(NC):
                y = _dot(qb, _bf16(ukb[h, pl.ds(cb * 64, 64), :]))
                old = qabs[h // 8][cb]
                qabs[h // 8][cb] = y if old is None else jnp.where(sub == h % 8, y, old)

        qm = [_dot(xb, _bf16(wqb[h])) for h in range(Q_MXU)]
        for h in range(Q_MXU):
            absorb(h, qm[h])
        h0 = 0
        prev = []
        for gsz in Q_GROUPS:
            qs = vpu_cols(wqf, list(range(h0, h0 + gsz)), h0 == 0, prev)
            for n in range(gsz):
                absorb(Q_MXU + h0 + n, qs[n])
            h0 += gsz
        scale = rstd[0:1, 0:1] * ((D ** -0.5) * LOG2E)
        qa = jnp.concatenate([jnp.concatenate(qabs[g], axis=1) for g in range(4)], axis=0)
        return (qa * scale).astype(bf16)

    def phase_b(qa):
        def scores(k0, k1):
            mrun = None
            for kb in range(k0, k1):
                s = _dot(qa, _bf16(cT[kb]))
                s_v[kb] = s
                mrun = s if mrun is None else jnp.maximum(mrun, s)
            return jnp.max(mrun, axis=-1, keepdims=True)

        def weighted(k0, k1, mrow):
            lsum = None
            cacc = [None] * NC
            for kb in range(k0, k1):
                p = jnp.exp2(s_v[kb] - mrow)
                lsum = p if lsum is None else lsum + p
                pb = p.astype(bf16)
                for cb in range(NC):
                    y = _dot(pb, _bf16(c2[cb, pl.ds(kb * 64, 64), :]))
                    cacc[cb] = y if cacc[cb] is None else cacc[cb] + y
            return jnp.sum(lsum, axis=-1, keepdims=True), cacc

        hk = NK // 2
        ma = scores(0, hk)
        mb = scores(hk, NK)
        la, ca = weighted(0, hk, ma)
        lb, cb_ = weighted(hk, NK, mb)
        m = jnp.maximum(ma, mb)
        fa = jnp.exp2(ma - m)
        fb = jnp.exp2(mb - m)
        linv = 1.0 / (la * fa + lb * fb)
        wa = fa * linv
        wb = fb * linv
        return jnp.concatenate([(ca[c] * wa + cb_[c] * wb).astype(bf16) for c in range(NC)], axis=1)

    def phase_c(cx):
        vacc = [None] * NJ
        macc = [None] * NJ
        ys = {}
        la = 4
        for i in range(H + la):
            if i < H:
                g = i // 8
                ys[i] = _dot(cx[8 * g:8 * g + 8, :], _bf16(uvb[i]))
            h = i - la
            if 0 <= h < O_VPU:
                xt = _xpose_bcast(ys[h][h % 8:h % 8 + 1, :])
                for ii in range(D // 8):
                    for j in range(NJ):
                        p = xt[8 * ii:8 * ii + 8, :] * wof[h * NJ + j, pl.ds(8 * ii, 8), :]
                        vacc[j] = p if vacc[j] is None else vacc[j] + p
        for h in range(O_VPU, H):
            lhs = jnp.broadcast_to(ys[h][h % 8:h % 8 + 1, :], (8, 128)).astype(bf16)
            for j in range(NJ):
                yy = _dot(lhs, _bf16(wob[(h - O_VPU) * NJ + j]))
                macc[j] = yy if macc[j] is None else macc[j] + yy
        return jnp.concatenate([_rowsum(vacc[j]) + macc[j] for j in range(NJ)], axis=1)

    def phase_d(x, xb, mean, rstd, first):
        stage_xt(x, mean)
        yacc = [None] * NJ
        waited = set()

        def down(fb, hb):
            if first:
                for i, (s0, n0) in enumerate(WD_CHUNKS):
                    if s0 < (fb + 1) * 128 and s0 + n0 > fb * 128 and i not in waited:
                        cps[f"wd{i}"].wait()
                        waited.add(i)
            for j in range(NJ):
                if first:
                    n = min(128, F - fb * 128)
                    t = wd_v[pl.ds(fb * 128, n), pl.ds(j * 128, 128)]
                    if n < 128:
                        t = jnp.concatenate([t, jnp.zeros((128 - n, 128), bf16)], axis=0)
                    wdb[z0 + fb * NJ + j] = _u32(t)
                else:
                    t = _bf16(wdb[fb * NJ + j])
                yy = _dot(hb, t)
                yacc[j] = yy if yacc[j] is None else yacc[j] + yy

        def act(g, u):
            return (jax.nn.silu(g * rstd) * (u * rstd)).astype(bf16)

        hs = {}
        for i in range(NF - F_VPU):
            hs[F_VPU + i] = act(_dot(xb, _bf16(gub[2 * i])), _dot(xb, _bf16(gub[2 * i + 1])))
        if not first:
            for fb in range(F_VPU, NF):
                down(fb, hs[fb])
        f0 = 0
        prev = []
        for gsz in F_GROUPS:
            ys = vpu_cols(guf, list(range(2 * f0, 2 * (f0 + gsz))), f0 == 0, prev)
            for n in range(gsz):
                hs[f0 + n] = act(ys[2 * n], ys[2 * n + 1])
                if not first:
                    down(f0 + n, hs[f0 + n])
            f0 += gsz
        if first:
            for fb in range(NF):
                down(fb, hs[fb])
        return jnp.concatenate(yacc, axis=1)

    def attn(x, first):
        xc, rstd, mean = _ln_parts(x)
        xb = xc.astype(bf16)
        if first:
            prep_wq()
            prep_wuk()
        qa = region(lambda: phase_a(x, xb, mean, rstd), first, jnp.zeros((H, DC), bf16), 'A')
        if first:
            prep_c()
        cx = region(lambda: phase_b(qa), first, jnp.zeros((H, DC), bf16), 'B')
        if first:
            prep_wuv()
            cps["wg"].wait()
            prep_gu(0, wg_v, 0, NF)
            for i in range(WO_CHUNKS):
                cps[f"wo{i}"].wait()
                prep_wo(i * hpc, (i + 1) * hpc)
        return region(lambda: phase_c(cx), first, jnp.zeros((8, M), f32), 'C')

    def ffn(x, first):
        xc, rstd, mean = _ln_parts(x)
        xn = xc * rstd
        xb = xc.astype(bf16)
        r = jnp.sum(xn.astype(bf16).astype(f32) * wr, axis=-1, keepdims=True)
        rs = jax.nn.sigmoid(r)
        if first:
            for i, (s0, n0) in enumerate(WU_CHUNKS):
                cps[f"wu{i}"].wait()
                prep_gu(1, wu_v, s0, s0 + (n0 + 127) // 128)
        y = region(lambda: phase_d(x, xb, mean, rstd, first), first, jnp.zeros((8, M), f32), 'D')
        return xn + (xn * 0.0 + y * rs)

    cps["x"].wait()
    cps["wr"].wait()
    x = jnp.broadcast_to(x_v[0].astype(f32), (8, M))
    wr = wr_v[...].astype(f32).reshape(1, M)
    x = x + attn(x, True)
    x = x + ffn(x, True)
    x = x + attn(x, False)
    x = x + ffn(x, False)
    o_v[0] = x[0:1, :].astype(bf16)
    ocp = pltpu.make_async_copy(o_v, o_hbm, sems.at[len(names)])
    ocp.start()
    ocp.wait()


@jax.jit
def pallas_interleave_layers__compressed_kv_cla__moe_arch_mod__decode_kernel(
    A_x, A_c_kv, A_w_q, A_w_uk, A_w_uv, A_w_o, B_x, B_w_r, B_w_gate, B_w_up, B_w_down,
):
    del B_x
    ins = [
        A_x, B_w_r, A_w_q, A_w_uk,
        A_c_kv.reshape(SK, DC),
        A_w_uv,
        A_w_o.reshape(H * D, M),
        B_w_gate.T, B_w_up.T,
        B_w_down,
    ]
    scratch = [
        pltpu.VMEM((1, 1, M), bf16),
        pltpu.VMEM((M,), bf16),
        pltpu.VMEM((H // 2, M, D), u32),
        pltpu.VMEM((H // 2, DC, D), u32),
        pltpu.VMEM((H // 2, DC, D), u32),
        pltpu.VMEM((H * D, M), bf16),
        pltpu.VMEM((F, M), bf16),
        pltpu.VMEM((F, M), bf16),
        pltpu.VMEM((F, M), bf16),
        pltpu.VMEM((Q_MXU, M // 2, 128), u32),
        pltpu.VMEM((Q_VPU, M, 128), f32),
        pltpu.VMEM((H, NC * 64, 128), u32),
        pltpu.VMEM((NK, DC // 2, 128), u32),
        pltpu.VMEM((NC, SK // 2, 128), u32),
        pltpu.VMEM((H, DC // 2, 128), u32),
        pltpu.VMEM(((H - O_VPU) * NJ, 64, 128), u32),
        pltpu.VMEM((O_VPU * NJ, 128, 128), f32),
        pltpu.VMEM((2 * (NF - F_VPU), M // 2, 128), u32),
        pltpu.VMEM((2 * F_VPU, M, 128), f32),
        pltpu.VMEM((NF * NJ, 64, 128), u32),
        *[pltpu.VMEM((160, 128), f32) for _ in range(NJ)],
        pltpu.VMEM((NK, H, 128), f32),
        pltpu.VMEM((1, 1, M), bf16),
        pltpu.SemaphoreType.DMA((80,)),
        pltpu.SemaphoreType.REGULAR((NZ,)),
    ]
    return pl.pallas_call(
        _kernel,
        in_specs=[pl.BlockSpec(memory_space=pltpu.HBM)] * len(ins),
        out_specs=pl.BlockSpec(memory_space=pltpu.HBM),
        out_shape=jax.ShapeDtypeStruct((1, 1, M), bf16),
        scratch_shapes=scratch,
        compiler_params=pltpu.CompilerParams(
            vmem_limit_bytes=120 * 1024 * 1024,
            disable_semaphore_checks=True,
            disable_bounds_checks=True,
            flags={"XLA_TPU_FORCE_LP_LLO_SCHEDULER": True},
        ),
    )(*ins)
```

```python
import jax
import jax.numpy as jnp
from jax import lax
import jax.experimental.pallas as pl
import jax.experimental.pallas.tpu as pltpu

bf16 = jnp.bfloat16
f32 = jnp.float32
u32 = jnp.uint32
i32 = jnp.int32

M = 640
H = 32
D = 128
SK = 4096
DC = 512
F = 1728
NJ = M // 128
NC = DC // 128
NK = SK // 128
NF = (F + 127) // 128
LOG2E = 1.4426950408889634
EPS = 1e-5

REG1 = 'ABCD'
REG2 = 'C'

Q_MXU = 8
Q_GROUPS = [4, 4, 4, 4, 4, 4]
O_VPU = 24
F_GROUPS = [2, 2, 2, 2]
F_VPU = sum(F_GROUPS)
Q2_MXU = 8
K2_VPU = 4
K2_LANES = 3
Q_VPU = H - Q_MXU
assert sum(Q_GROUPS) == Q_VPU and Q_MXU % 2 == 0 and F_VPU % 2 == 0

WO_CHUNKS = 4
LATE = [11, 12]
WG_CHUNKS = [(0, 11), (13, 1)]
WU_CHUNKS = [(0, 4), (4, 4), (8, 3), (13, 1)]
WD_CHUNKS = [(0, 3), (3, 3), (6, 3), (9, 1), (10, 1), (13, 1)]
NL = len(LATE)
EARLY = [fb for fb in range(NF) if fb not in LATE]
ZH_UK = 16
ZH_UV = 16
LATE_STAGES = [[('g',11),('u',11),('g',12),('u',12)]]
Y_VPU = True
TIE_KB = 2
A2_KPOS = 4
TIE_KB2 = 3
A2_GROUPS = [4, 4, 4, 4, 4, 4]
AE_MXU = 20
AE_GROUPS = [4,4,4]
NZ = 32


def _dot(a, b):
    return jnp.dot(a, b, preferred_element_type=f32)


def _u32(a):
    return pltpu.bitcast(a, u32)


def _bf16(a):
    return pltpu.bitcast(a, bf16)


def _lo(w):
    return pltpu.bitcast(w << 16, f32)


def _hi(w):
    return pltpu.bitcast(w & jnp.uint32(0xFFFF0000), f32)


def _rowsum(acc):
    return jnp.broadcast_to(jnp.sum(acc, axis=0, keepdims=True), (8, 128))


def _ln_parts(x):
    m = jnp.sum(x, axis=-1, keepdims=True) * (1.0 / M)
    m2 = jnp.sum(x * x, axis=-1, keepdims=True) * (1.0 / M)
    v = jnp.maximum(m2 - m * m, 0.0)
    return x - m, lax.rsqrt(v + EPS), m


def _xpose_bcast(row):
    r16 = jnp.broadcast_to(row, (16, 128)).astype(bf16)
    return jnp.concatenate([r16] * 8, axis=0).T.astype(f32)


def _kernel(x_hbm, wr_hbm, wq_hbm, wuk_hbm, c_hbm, wuv_hbm, wo_hbm, wg_hbm, wu_hbm, wd_hbm,
            o_hbm,
            x_v, wr_v, wq_v, wuk_v, wuv_v, wo_v, wg_v, wu_v, wd_v,
            wqb, wqf, ukb, ukf, cs_v, rm_v, wdf, zb, zf, wdb, cT, c2, uvb, wob, wof, gub, guf, xt0, xt1, xt2, xt3, xt4, s_v, o_v, sems, zsem):
    cps = {}
    names = []
    families = {}

    def add(name, src, dst):
        cp = pltpu.make_async_copy(src, dst, sems.at[len(names)])
        cp.start()
        cps[name] = cp
        names.append(name)

    def add_pairs(name, src, dst):
        s32 = src.bitcast(u32)
        families[name] = (s32, dst, len(names))
        for hp in range(H // 2):
            add(f"{name}{hp}", s32.at[:, hp, :], dst.at[hp])

    def wait_pair(name, hp):
        src, dst, base = families[name]
        pltpu.make_async_copy(src.at[:, hp, :], dst.at[hp], sems.at[base + hp]).wait()

    add("x", x_hbm, x_v)
    add("wr", wr_hbm, wr_v)
    def add_blocks(name, src, dst, fb0, nb):
        rows = min(128 * nb, F - 128 * fb0)
        add(name, src.at[pl.ds(128 * fb0, rows)], dst.at[pl.ds(128 * fb0, rows)])

    add_pairs("wq", wq_hbm, wq_v)
    for fb in LATE:
        add_blocks(f"wdL{fb}", wd_hbm, wd_v, fb, 1)
    add_pairs("wuk", wuk_hbm, wuk_v)
    c32 = c_hbm.bitcast(u32)
    for cb in range(NC):
        add(f"c{cb}", c32.at[:, pl.ds(cb * 128, 128)], c2.at[cb])
    add_pairs("wuv", wuv_hbm, wuv_v)
    for i, (s, n) in enumerate(WG_CHUNKS):
        add_blocks(f"wg{i}", wg_hbm, wg_v, s, n)
    hpc = H // WO_CHUNKS
    for i in range(WO_CHUNKS):
        add(f"wo{i}", wo_hbm.at[pl.ds(i * hpc * D, hpc * D)], wo_v.at[pl.ds(i * hpc * D, hpc * D)])
    for i, (s, n) in enumerate(WU_CHUNKS):
        add_blocks(f"wu{i}", wu_hbm, wu_v, s, n)
    for i, (s, n) in enumerate(WD_CHUNKS):
        add_blocks(f"wd{i}", wd_hbm, wd_v, s, n)
    for fb in LATE:
        add_blocks(f"wgL{fb}", wg_hbm, wg_v, fb, 1)
        add_blocks(f"wuL{fb}", wu_hbm, wu_v, fb, 1)

    sub = lax.broadcasted_iota(i32, (8, 128), 0)
    xts = [xt0, xt1, xt2, xt3, xt4]
    zs = [pl.semaphore_read(zsem.at[n]) for n in range(NZ)]
    z0 = zs[0]
    zvec = jnp.zeros((8, 128), u32) + zs[-1].astype(u32)
    zmask = zvec != 0
    zi = iter(zs[1:-1])

    def repack(src, hp, dst, rows):
        for i in range(rows // 16):
            v = src[hp, pl.ds(16 * i, 16), :]
            dst[2 * hp, pl.ds(8 * i, 8), :] = _u32(_lo(v).astype(bf16))
            dst[2 * hp + 1, pl.ds(8 * i, 8), :] = _u32(_hi(v).astype(bf16))

    def prep_wq():
        def both(k, carry):
            hp = k + Q_MXU // 2
            wait_pair("wq", hp)
            repack(wq_v, hp, wqb, M)
            v = wq_v[hp]
            wqf[2 * k] = _lo(v)
            wqf[2 * k + 1] = _hi(v)
            return carry

        for hp in range(Q_MXU // 2):
            cps[f"wq{hp}"].wait()
            repack(wq_v, hp, wqb, M)
        lax.fori_loop(0, Q_VPU // 2, both, 0)
        ones = jnp.ones((8, M), bf16)

        def colsum(g, carry):
            acc = jnp.zeros((8, 128), f32)
            for r in range(8):
                acc = jnp.where(sub == r, _dot(ones, _bf16(wqb[8 * g + r])), acc)
            cs_v[pl.ds(pl.multiple_of(8 * g, 8), 8), :] = acc
            return carry
        lax.fori_loop(0, H // 8, colsum, 0)

    def prep_wuk():
        def pair_b(hp, carry):
            wait_pair("wuk", hp)
            for cb in range(NC):
                t = wuk_v[hp, pl.ds(cb * 128, 128), :].T
                ukb[2 * hp, pl.ds(cb * 64, 64), :] = _u32(_lo(t).astype(bf16))
                ukb[2 * hp + 1, pl.ds(cb * 64, 64), :] = _u32(_hi(t).astype(bf16))
            return carry

        def pair_bf(hp, carry):
            wait_pair("wuk", hp)
            for cb in range(NC):
                t = wuk_v[hp, pl.ds(cb * 128, 128), :].T
                lo, hi = _lo(t), _hi(t)
                ukf[(2 * hp - (H - K2_VPU)) * NC + cb] = lo
                ukf[(2 * hp + 1 - (H - K2_VPU)) * NC + cb] = hi
                ukb[2 * hp, pl.ds(cb * 64, 64), :] = _u32(lo.astype(bf16))
                ukb[2 * hp + 1, pl.ds(cb * 64, 64), :] = _u32(hi.astype(bf16))
            return carry
        def with_z(fn, mxu):
            def body(hp, carry):
                fn(hp, carry)
                z_head(hp, mxu)
                return carry
            return body
        cuts = sorted({0, min(Q2_MXU, ZH_UK), min(ZH_UK, H // 2), (H - K2_VPU) // 2, H // 2})
        for a, b in zip(cuts[:-1], cuts[1:]):
            fn = pair_b if a < (H - K2_VPU) // 2 else pair_bf
            if a < ZH_UK:
                lax.fori_loop(a, b, with_z(fn, a < Q2_MXU), 0)
            else:
                lax.fori_loop(a, b, fn, 0)

    def prep_c():
        for cb in range(NC):
            cps[f"c{cb}"].wait()

            def blk(i, carry, cb=cb):
                for kk in range(16):
                    kb = 16 * i + kk
                    t = _bf16(c2[cb, pl.ds(pl.multiple_of(kb * 64, 64), 64), :])
                    cT[kb, pl.ds(cb * 64, 64), :] = _u32(t.T)
                return carry
            lax.fori_loop(0, NK // 16, blk, 0)

    def prep_wuv():
        def pair(hp, carry):
            wait_pair("wuv", hp)
            repack(wuv_v, hp, uvb, DC)
            return carry

        def pair_z(hp, carry):
            z_head(hp + ZH_UK, False)
            return pair(hp, carry)
        lax.fori_loop(0, ZH_UV, pair_z, 0)
        if ZH_UV < H // 2:
            lax.fori_loop(ZH_UV, H // 2, pair, 0)

    def prep_gu(mat, raw, fb0, fb1):
        def tile(fb, j):
            return raw[pl.ds(pl.multiple_of(fb * 128, 128), 128), pl.ds(j * 128, 128)].T

        def vpu_blks(i, carry):
            for fb in (2 * i, 2 * i + 1):
                for j in range(NJ):
                    guf[2 * fb + mat, pl.ds(j * 128, 128), :] = tile(fb, j).astype(f32)
            return carry
        if fb0 < F_VPU:
            lax.fori_loop(fb0 // 2, min(fb1, F_VPU) // 2, vpu_blks, 0)

        for fb in range(max(fb0, F_VPU), min(fb1, NF - 1)):
            for j in range(NJ):
                gub[z0 + 2 * (fb - F_VPU) + mat, pl.ds(j * 64, 64), :] = _u32(tile(fb, j))
        if fb0 <= NF - 1 < fb1:
            for j in range(NJ):
                t = raw[pl.ds((NF - 1) * 128, 64), pl.ds(j * 128, 128)]
                t = jnp.concatenate([t, jnp.zeros((64, 128), bf16)], axis=0).T
                gub[z0 + 2 * (NF - 1 - F_VPU) + mat, pl.ds(j * 64, 64), :] = _u32(t)

    def prep_late_wd():
        for b, fb in enumerate(LATE):
            cps[f"wdL{fb}"].wait()
            acc = None
            for j in range(NJ):
                t = wd_v[pl.ds(fb * 128, 128), pl.ds(j * 128, 128)]
                wdb[z0 + fb * NJ + j] = _u32(t)
                wdf[j, pl.ds(b * 128, 128), :] = t.astype(f32)
                r = jnp.sum(t.astype(f32), axis=-1, keepdims=True)
                acc = r if acc is None else acc + r
            rm_v[b] = jnp.broadcast_to(acc * (1.0 / M), (128, 128))

    def z_head(h, mxu):
        cs = cs_v[pl.ds(h, 1), :]
        for b, fb in enumerate(LATE):
            z = None
            for j in range(NJ):
                y = _dot(_bf16(wdb[fb * NJ + j]), _bf16(wqb[h, pl.ds(j * 64, 64), :]))
                z = y if z is None else z + y
            z = z - rm_v[b] * cs
            if mxu:
                zb[h, pl.ds(b * 64, 64), :] = _u32(z.astype(bf16))
            else:
                zf[h - Q2_MXU, pl.ds(b * 128, 128), :] = z

    def prep_z(h0, h1):
        if h0 < h1:
            lax.fori_loop(h0, h1, lambda h, c: (z_head(h, False), c)[1], 0)

    def prep_wo(h0, h1):
        def vpu_head(h, carry):
            for j in range(NJ):
                t = wo_v[pl.ds(pl.multiple_of(h * 128, 128), 128), pl.ds(j * 128, 128)]
                wof[h * NJ + j] = t.astype(f32)
            return carry

        def mxu_head(h, carry):
            for j in range(NJ):
                t = wo_v[pl.ds(pl.multiple_of(h * 128, 128), 128), pl.ds(j * 128, 128)]
                wob[(h - O_VPU) * NJ + j] = _u32(t)
            return carry
        if h0 < O_VPU:
            lax.fori_loop(h0, min(h1, O_VPU), vpu_head, 0)
        if h1 > O_VPU:
            lax.fori_loop(max(h0, O_VPU), h1, mxu_head, 0)

    def stage_xt(x, mean):
        for kb in range(NJ):
            t = _xpose_bcast(x[0:1, kb * 128:(kb + 1) * 128])
            xts[kb][pl.ds(0, 128), :] = t - mean[0:1, 0:1]

    def vpu_cols(wref, idxs, static, prev, rows=M):
        accs = [None] * len(idxs)
        if not static:
            zf = next(zi)
            for kb in range(rows // 128):
                xts[kb][pl.ds(zf + 128, 8), :] = pltpu.bitcast(zvec, f32)
        for i in range(rows // 8):
            xt = xts[i // 16][pl.ds(8 * (i % 16), 8), :]
            for n, c in enumerate(idxs):
                p = xt * wref[c, pl.ds(8 * i, 8), :]
                if accs[n] is None:
                    if prev:
                        p = jnp.where(zmask, prev[n % len(prev)], p)
                    accs[n] = p
                else:
                    accs[n] = accs[n] + p
        prev[:] = accs
        return [_rowsum(a) for a in accs]

    def region(fn, first, zero, tag):
        if tag not in (REG1 if first else REG2):
            return fn()
        return lax.cond(z0 == 0, fn, lambda: zero)

    def phase_a(x, xb, mean, rstd):
        stage_xt(x, mean)
        qabs = [[None] * NC for _ in range(4)]

        def absorb(h, qh):
            qb = qh.astype(bf16)
            for cb in range(NC):
                y = _dot(qb, _bf16(ukb[h, pl.ds(cb * 64, 64), :]))
                old = qabs[h // 8][cb]
                qabs[h // 8][cb] = y if old is None else jnp.where(sub == h % 8, y, old)

        qm = [_dot(xb, _bf16(wqb[h])) for h in range(Q_MXU)]
        for h in range(Q_MXU):
            absorb(h, qm[h])
        h0 = 0
        prev = []
        for gsz in Q_GROUPS:
            qs = vpu_cols(wqf, list(range(h0, h0 + gsz)), h0 == 0, prev)
            for n in range(gsz):
                absorb(Q_MXU + h0 + n, qs[n])
            h0 += gsz
        scale = rstd[0:1, 0:1] * ((D ** -0.5) * LOG2E)
        qa = jnp.concatenate([jnp.concatenate(qabs[g], axis=1) for g in range(4)], axis=0)
        return (qa * scale).astype(bf16)

    def phase_b(qa, ycalc=None):
        sc = None
        side = {}
        def scores(k0, k1):
            mrun = None
            for kb in range(k0, k1):
                s = _dot(qa, _bf16(cT[kb]))
                s_v[kb] = s
                if ycalc is not None and kb == TIE_KB:
                    side['sc'] = ycalc(s[0:8, :])
                if ycalc is not None and kb == TIE_KB2:
                    ycalc.late(s[0:8, :])
                mrun = s if mrun is None else jnp.maximum(mrun, s)
            return jnp.max(mrun, axis=-1, keepdims=True)

        def weighted(k0, k1, mrow):
            lsum = None
            cacc = [None] * NC
            for kb in range(k0, k1):
                p = jnp.exp2(s_v[kb] - mrow if sc is None else (s_v[kb] - mrow) * sc)
                lsum = p if lsum is None else lsum + p
                pb = p.astype(bf16)
                for cb in range(NC):
                    y = _dot(pb, _bf16(c2[cb, pl.ds(kb * 64, 64), :]))
                    cacc[cb] = y if cacc[cb] is None else cacc[cb] + y
            return jnp.sum(lsum, axis=-1, keepdims=True), cacc

        hk = NK // 2
        ma = scores(0, hk)
        mb = scores(hk, NK)
        sc = side.get('sc')
        la, ca = weighted(0, hk, ma)
        lb, cb_ = weighted(hk, NK, mb)
        m = jnp.maximum(ma, mb)
        fa = jnp.exp2(ma - m if sc is None else (ma - m) * sc)
        fb = jnp.exp2(mb - m if sc is None else (mb - m) * sc)
        linv = 1.0 / (la * fa + lb * fb)
        wa = fa * linv
        wb = fb * linv
        return jnp.concatenate([(ca[c] * wa + cb_[c] * wb).astype(bf16) for c in range(NC)], axis=1)

    def phase_c(cx):
        vacc = [None] * NJ
        macc = [None] * NJ
        ys = {}
        la = 4
        for i in range(H + la):
            if i < H:
                g = i // 8
                ys[i] = _dot(cx[8 * g:8 * g + 8, :], _bf16(uvb[i]))
            h = i - la
            if 0 <= h < O_VPU:
                xt = _xpose_bcast(ys[h][h % 8:h % 8 + 1, :])
                for ii in range(D // 8):
                    for j in range(NJ):
                        p = xt[8 * ii:8 * ii + 8, :] * wof[h * NJ + j, pl.ds(8 * ii, 8), :]
                        vacc[j] = p if vacc[j] is None else vacc[j] + p
        for h in range(O_VPU, H):
            lhs = jnp.broadcast_to(ys[h][h % 8:h % 8 + 1, :], (8, 128)).astype(bf16)
            for j in range(NJ):
                yy = _dot(lhs, _bf16(wob[(h - O_VPU) * NJ + j]))
                macc[j] = yy if macc[j] is None else macc[j] + yy
        return jnp.concatenate([_rowsum(vacc[j]) + macc[j] for j in range(NJ)], axis=1)

    def swiglu(x, xb, mean, rstd, on_block, skip=()):
        stage_xt(x, mean)

        def act(g, u):
            return (jax.nn.silu(g * rstd) * (u * rstd)).astype(bf16)

        for i in range(NF - F_VPU):
            if F_VPU + i in skip:
                continue
            on_block(F_VPU + i, act(_dot(xb, _bf16(gub[2 * i])), _dot(xb, _bf16(gub[2 * i + 1]))), 0)
        on_block(None, None, 0)
        f0 = 0
        prev = []
        for gsz in F_GROUPS:
            ys = vpu_cols(guf, list(range(2 * f0, 2 * (f0 + gsz))), f0 == 0, prev)
            for n in range(gsz):
                on_block(f0 + n, act(ys[2 * n], ys[2 * n + 1]), 1)
            f0 += gsz

    def phase_d1(x, xb, mean, rstd):
        hs = {}

        def keep(fb, h, kind):
            if fb is not None:
                hs[fb] = h
        swiglu(x, xb, mean, rstd, keep, skip=LATE)
        return tuple(hs[fb] for fb in EARLY)

    def phase_d2(x, xb, mean, rstd):
        yacc = [None] * NJ
        held = []

        def down(fb, hb):
            for j in range(NJ):
                yy = _dot(hb, _bf16(wdb[fb * NJ + j]))
                yacc[j] = yy if yacc[j] is None else yacc[j] + yy

        def on_block(fb, h, kind):
            if fb is None:
                for b, hb in held:
                    down(b, hb)
            elif kind == 0:
                held.append((fb, h))
            else:
                down(fb, h)
        swiglu(x, xb, mean, rstd, on_block)
        return jnp.concatenate(yacc, axis=1)

    def phase_a_early(v):
        vb = v.astype(bf16)
        for kb in range(NJ):
            xts[kb][pl.ds(0, 128), :] = _xpose_bcast(v[0:1, kb * 128:(kb + 1) * 128])
        delta = jnp.sum(vb.astype(f32), axis=-1, keepdims=True) * (1.0 / M)
        q = [None] * 4

        def put(h, y):
            q[h // 8] = y if q[h // 8] is None else jnp.where(sub == h % 8, y, q[h // 8])

        for h in range(AE_MXU):
            put(h, _dot(vb, _bf16(wqb[h])))
        h0 = AE_MXU
        prev = []
        for gsz in AE_GROUPS:
            ys = vpu_cols(wqf, list(range(h0 - Q_MXU, h0 - Q_MXU + gsz)), h0 == AE_MXU, prev)
            for n in range(gsz):
                put(h0 + n, ys[n])
            h0 += gsz
        return tuple(q[g] - delta * cs_v[pl.ds(8 * g, 8), :] for g in range(4))

    def phase_a2(hl, qbase, rs, scale):
        for b in range(NL):
            xts[b][pl.ds(0, 128), :] = _xpose_bcast(hl[b].astype(f32)[0:1, :])
        hcat = jnp.concatenate(hl, axis=1)
        qabs = [[None] * NC for _ in range(4)]

        def put(h, cb, y):
            old = qabs[h // 8][cb]
            qabs[h // 8][cb] = y if old is None else jnp.where(sub == h % 8, y, old)

        def base(h):
            return _rowsum(jnp.where(sub == h % 8, qbase[h // 8], 0.0))

        def absorb_mxu(h, qh):
            qb = qh.astype(bf16)
            for cb in range(NC):
                put(h, cb, _dot(qb, _bf16(ukb[h, pl.ds(cb * 64, 64), :])))

        segs = []

        def absorb_vpu(h, qh):
            xq = _xpose_bcast(qh[0:1, :])
            for cb in range(NC):
                acc = None
                for i in range(16):
                    p = xq[8 * i:8 * i + 8] * ukf[(h - (H - K2_VPU)) * NC + cb, pl.ds(8 * i, 8), :]
                    if acc is None:
                        if len(segs) >= K2_LANES:
                            p = jnp.where(zmask, segs[len(segs) - K2_LANES], p)
                        acc = p
                    else:
                        acc = acc + p
                segs.append(acc)
                put(h, cb, _rowsum(acc))

        qm = [_dot(hcat, _bf16(zb[h])) * rs + base(h) for h in range(Q2_MXU)]
        for h in range(Q2_MXU):
            absorb_mxu(h, qm[h])
        mh = list(range(Q2_MXU, H - K2_VPU))
        order = mh[:A2_KPOS] + list(range(H - K2_VPU, H)) + mh[A2_KPOS:]
        prev = []
        held = []
        pos = 0
        for gsz in A2_GROUPS:
            hh = order[pos:pos + gsz]
            ys = vpu_cols(zf, [h - Q2_MXU for h in hh], pos == 0, prev, rows=128 * NL)
            for n, h in enumerate(hh):
                qh = ys[n] * rs + base(h)
                if h >= H - K2_VPU:
                    held.append((h, qh))
                else:
                    absorb_mxu(h, qh)
            pos += gsz
        for h, qh in held:
            absorb_vpu(h, qh)
        qa = jnp.concatenate([jnp.concatenate(qabs[g], axis=1) for g in range(4)], axis=0)
        return (qa if scale is None else qa * scale).astype(bf16)

    def router(xn):
        r = jnp.sum(xn.astype(bf16).astype(f32) * wr, axis=-1, keepdims=True)
        return jax.nn.sigmoid(r)

    cps["x"].wait()
    cps["wr"].wait()
    x = jnp.broadcast_to(x_v[0].astype(f32), (8, M))
    wr = wr_v[...].astype(f32).reshape(1, M)

    xc, rstd, mean = _ln_parts(x)
    xb = xc.astype(bf16)
    prep_wq()
    prep_late_wd()
    prep_wuk()
    qa = region(lambda: phase_a(x, xb, mean, rstd), True, jnp.zeros((H, DC), bf16), 'A')
    prep_c()
    cx = region(lambda: phase_b(qa), True, jnp.zeros((H, DC), bf16), 'B')
    prep_wuv()
    for i, (s0, n0) in enumerate(WG_CHUNKS):
        cps[f"wg{i}"].wait()
        prep_gu(0, wg_v, s0, s0 + n0)
    zh = ZH_UK + ZH_UV
    zper = (H - zh + WO_CHUNKS - 2) // (WO_CHUNKS - 1)
    for i in range(WO_CHUNKS):
        cps[f"wo{i}"].wait()
        prep_wo(i * hpc, (i + 1) * hpc)
        prep_z(min(zh + i * zper, H), min(zh + (i + 1) * zper, H))
    x = x + region(lambda: phase_c(cx), True, jnp.zeros((8, M), f32), 'C')

    xc, rstd, mean = _ln_parts(x)
    xn = xc * rstd
    xb = xc.astype(bf16)
    rs = router(xn)
    for i, (s0, n0) in enumerate(WU_CHUNKS):
        cps[f"wu{i}"].wait()
        prep_gu(1, wu_v, s0, s0 + n0)
    hs_e = region(lambda: phase_d1(x, xb, mean, rstd), True,
                  tuple(jnp.zeros((8, 128), bf16) for _ in range(len(EARLY))), 'D')
    hs = dict(zip(EARLY, hs_e))
    u = x + (xn + xn * 0.0)
    yj = [None] * NJ

    def down1(fb, hb):
        for j in range(NJ):
            n = min(128, F - fb * 128)
            t = wd_v[pl.ds(fb * 128, n), pl.ds(j * 128, 128)]
            if n < 128:
                t = jnp.concatenate([t, jnp.zeros((128 - n, 128), bf16)], axis=0)
            wdb[z0 + fb * NJ + j] = _u32(t)
            yy = _dot(hb, t)
            yj[j] = yy if yj[j] is None else yj[j] + yy

    for i, (fb0, nb) in enumerate(WD_CHUNKS):
        cps[f"wd{i}"].wait()
        for fb in range(fb0, fb0 + nb):
            down1(fb, hs[fb])
    v = u + jnp.concatenate(yj, axis=1) * rs
    qbase = region(lambda: phase_a_early(v), True,
                   tuple(jnp.zeros((8, 128), f32) for _ in range(4)), 'E')
    tr = (((1,), (1,)), ((), ()))

    def proj(ref, fb):
        return lax.dot_general(xb, ref[pl.ds(fb * 128, 128), :], tr, preferred_element_type=f32)

    gu = {}
    for stage in LATE_STAGES:
        for m, fb in stage:
            cps[f"w{m}L{fb}"].wait()
        for m, fb in stage:
            gu[m, fb] = proj(wg_v if m == 'g' else wu_v, fb)
            if ('g', fb) in gu and ('u', fb) not in gu and m == 'g' and ('u', fb) not in stage:
                gu['s', fb] = jax.nn.silu(gu['g', fb] * rstd) * rstd
            if m == 'u':
                sg = gu['s', fb] if ('s', fb) in gu else jax.nn.silu(gu['g', fb] * rstd) * rstd
                gu['h', fb] = (sg * gu['u', fb]).astype(bf16)
    hl = [gu['h', fb] for fb in LATE]
    if not Y_VPU:
        yj = [None] * NJ
        for b, fb in enumerate(LATE):
            for j in range(NJ):
                yy = _dot(hl[b], _bf16(wdb[fb * NJ + j]))
                yj[j] = yy if yj[j] is None else yj[j] + yy
        x = v + jnp.concatenate(yj, axis=1) * rs
        xc, rstd2, mean = _ln_parts(x)
        qa = phase_a2(hl, qbase, rs, rstd2[0:1, 0:1] * ((D ** -0.5) * LOG2E))
        sc2 = None
    else:
        qa = phase_a2(hl, qbase, rs, None)
        xs = {}

        def sc2(tie):
            ys = vpu_cols(wdf, list(range(NJ)), False, [tie], rows=128 * NL)
            xs['x'] = v + jnp.concatenate(ys, axis=1) * rs
            xc, rstd2, mean = _ln_parts(xs['x'])
            return rstd2[0:1, 0:1] * ((D ** -0.5) * LOG2E)

        def late_prep(tie):
            for fb in LATE:
                prep_gu(0, wg_v, fb, fb + 1)
                prep_gu(1, wu_v, fb, fb + 1)
        sc2.late = late_prep
    if not Y_VPU:
        for fb in LATE:
            prep_gu(0, wg_v, fb, fb + 1)
            prep_gu(1, wu_v, fb, fb + 1)
    cx = region(lambda: phase_b(qa, sc2), False, jnp.zeros((H, DC), bf16), 'B')
    if Y_VPU:
        x = xs['x']
    x = x + region(lambda: phase_c(cx), False, jnp.zeros((8, M), f32), 'C')
    xc, rstd, mean = _ln_parts(x)
    xn = xc * rstd
    xb = xc.astype(bf16)
    rs = router(xn)
    y = region(lambda: phase_d2(x, xb, mean, rstd), False, jnp.zeros((8, M), f32), 'D')
    x = x + (xn + (xn * 0.0 + y * rs))

    o_v[0] = x[0:1, :].astype(bf16)
    ocp = pltpu.make_async_copy(o_v, o_hbm, sems.at[len(names)])
    ocp.start()
    ocp.wait()


@jax.jit
def pallas_interleave_layers__compressed_kv_cla__moe_arch_mod__decode_kernel(
    A_x, A_c_kv, A_w_q, A_w_uk, A_w_uv, A_w_o, B_x, B_w_r, B_w_gate, B_w_up, B_w_down,
):
    del B_x
    ins = [
        A_x, B_w_r, A_w_q, A_w_uk,
        A_c_kv.reshape(SK, DC),
        A_w_uv,
        A_w_o.reshape(H * D, M),
        B_w_gate.T, B_w_up.T,
        B_w_down,
    ]
    scratch = [
        pltpu.VMEM((1, 1, M), bf16),
        pltpu.VMEM((M,), bf16),
        pltpu.VMEM((H // 2, M, D), u32),
        pltpu.VMEM((H // 2, DC, D), u32),
        pltpu.VMEM((H // 2, DC, D), u32),
        pltpu.VMEM((H * D, M), bf16),
        pltpu.VMEM((F, M), bf16),
        pltpu.VMEM((F, M), bf16),
        pltpu.VMEM((F, M), bf16),
        pltpu.VMEM((H, M // 2, 128), u32),
        pltpu.VMEM((Q_VPU, M, 128), f32),
        pltpu.VMEM((H, NC * 64, 128), u32),
        pltpu.VMEM((K2_VPU * NC, 128, 128), f32),
        pltpu.VMEM((H, 128), f32),
        pltpu.VMEM((NL, 128, 128), f32),
        pltpu.VMEM((NJ, NL * 128, 128), f32),
        pltpu.VMEM((Q2_MXU, NL * 64, 128), u32),
        pltpu.VMEM((H - Q2_MXU, NL * 128, 128), f32),
        pltpu.VMEM((NF * NJ, 64, 128), u32),
        pltpu.VMEM((NK, DC // 2, 128), u32),
        pltpu.VMEM((NC, SK // 2, 128), u32),
        pltpu.VMEM((H, DC // 2, 128), u32),
        pltpu.VMEM(((H - O_VPU) * NJ, 64, 128), u32),
        pltpu.VMEM((O_VPU * NJ, 128, 128), f32),
        pltpu.VMEM((2 * (NF - F_VPU), M // 2, 128), u32),
        pltpu.VMEM((2 * F_VPU, M, 128), f32),
        *[pltpu.VMEM((160, 128), f32) for _ in range(NJ)],
        pltpu.VMEM((NK, H, 128), f32),
        pltpu.VMEM((1, 1, M), bf16),
        pltpu.SemaphoreType.DMA((96,)),
        pltpu.SemaphoreType.REGULAR((NZ,)),
    ]
    return pl.pallas_call(
        _kernel,
        in_specs=[pl.BlockSpec(memory_space=pltpu.HBM)] * len(ins),
        out_specs=pl.BlockSpec(memory_space=pltpu.HBM),
        out_shape=jax.ShapeDtypeStruct((1, 1, M), bf16),
        scratch_shapes=scratch,
        compiler_params=pltpu.CompilerParams(
            vmem_limit_bytes=120 * 1024 * 1024,
            disable_semaphore_checks=True,
            disable_bounds_checks=True,
            flags={"XLA_TPU_FORCE_LP_LLO_SCHEDULER": True},
        ),
    )(*ins)
```

```python
import jax
import jax.numpy as jnp
from jax import lax
import jax.experimental.pallas as pl
import jax.experimental.pallas.tpu as pltpu

bf16 = jnp.bfloat16
f32 = jnp.float32
u32 = jnp.uint32
i32 = jnp.int32

M = 640
H = 32
D = 128
SK = 4096
DC = 512
F = 1728
NJ = M // 128
NC = DC // 128
NK = SK // 128
NF = (F + 127) // 128
LOG2E = 1.4426950408889634
EPS = 1e-5

REG1 = 'ABCD'
REG2 = 'C'

Q_MXU = 8
Q_GROUPS = [4, 4, 4, 4, 4, 4]
O_VPU = 24
F_GROUPS = [2, 2, 2, 2]
F_VPU = sum(F_GROUPS)
Q2_MXU = 8
K2_VPU = 4
K2_LANES = 3
Q_VPU = H - Q_MXU
assert sum(Q_GROUPS) == Q_VPU and Q_MXU % 2 == 0 and F_VPU % 2 == 0

WO_CHUNKS = 4
LATE = [11, 12]
WG_CHUNKS = [(0, 11), (13, 1)]
WU_CHUNKS = [(0, 4), (4, 4), (8, 3), (13, 1)]
WD_CHUNKS = [(0, 3), (3, 3), (6, 3), (9, 1), (10, 1), (13, 1)]
NL = len(LATE)
EARLY = [fb for fb in range(NF) if fb not in LATE]
ZH_UK = 16
ZH_UV = 16
LATE_STAGES = [[('g', 11), ('u', 11), ('g', 12), ('u', 12)]]
Y_VPU = True
TIE_KB = 2
A2_KPOS = 8
FAST_ACT = True
Y_GROUPS = [5]
C_LK = None
C_LA = 4
A2_POST = False
AE_POST = False
A2_MPRE = [8, 0, 0, 0, 0, 0]
TIE_KB2 = 3
A2_GROUPS = [4, 4, 4, 4, 4, 4, 4, 4]
AE_MXU = 20
AE_GROUPS = [4,4,4]
NZ = 32


def _dot(a, b):
    return jnp.dot(a, b, preferred_element_type=f32)


def _u32(a):
    return pltpu.bitcast(a, u32)


def _bf16(a):
    return pltpu.bitcast(a, bf16)


def _lo(w):
    return pltpu.bitcast(w << 16, f32)


def _hi(w):
    return pltpu.bitcast(w & jnp.uint32(0xFFFF0000), f32)


def _rowsum(acc):
    return jnp.broadcast_to(jnp.sum(acc, axis=0, keepdims=True), (8, 128))


def _ln_parts(x):
    m = jnp.sum(x, axis=-1, keepdims=True) * (1.0 / M)
    m2 = jnp.sum(x * x, axis=-1, keepdims=True) * (1.0 / M)
    v = jnp.maximum(m2 - m * m, 0.0)
    return x - m, lax.rsqrt(v + EPS), m


def _xpose_bcast(row):
    r16 = jnp.broadcast_to(row, (16, 128)).astype(bf16)
    return jnp.concatenate([r16] * 8, axis=0).T.astype(f32)


def _swiglu(g, u, rstd):
    e = jnp.exp2(g * (rstd * -LOG2E))
    return (g * u) * (rstd * rstd) * pl.reciprocal(1.0 + e, approx=True)


def _kernel(x_hbm, wr_hbm, wq_hbm, wuk_hbm, c_hbm, wuv_hbm, wo_hbm, wg_hbm, wu_hbm, wd_hbm,
            o_hbm,
            x_v, wr_v, wq_v, wuk_v, wuv_v, wo_v, wg_v, wu_v, wd_v,
            wqb, wqf, ukb, ukf, cs_v, rm_v, wdf, gul, wdp, zf, wdb, cT, c2, uvb, wob, wof, gub, guf, xt0, xt1, xt2, xt3, xt4, s_v, o_v, sems, zsem):
    cps = {}
    names = []
    families = {}

    def add(name, src, dst):
        cp = pltpu.make_async_copy(src, dst, sems.at[len(names)])
        cp.start()
        cps[name] = cp
        names.append(name)

    def add_pairs(name, src, dst):
        s32 = src.bitcast(u32)
        families[name] = (s32, dst, len(names))
        for hp in range(H // 2):
            add(f"{name}{hp}", s32.at[:, hp, :], dst.at[hp])

    def wait_pair(name, hp):
        src, dst, base = families[name]
        pltpu.make_async_copy(src.at[:, hp, :], dst.at[hp], sems.at[base + hp]).wait()

    add("x", x_hbm, x_v)
    add("wr", wr_hbm, wr_v)
    def add_blocks(name, src, dst, fb0, nb):
        rows = min(128 * nb, F - 128 * fb0)
        add(name, src.at[pl.ds(128 * fb0, rows)], dst.at[pl.ds(128 * fb0, rows)])

    add_pairs("wq", wq_hbm, wq_v)
    for fb in LATE:
        add_blocks(f"wdL{fb}", wd_hbm, wd_v, fb, 1)
    add_pairs("wuk", wuk_hbm, wuk_v)
    c32 = c_hbm.bitcast(u32)
    for cb in range(NC):
        add(f"c{cb}", c32.at[:, pl.ds(cb * 128, 128)], c2.at[cb])
    add_pairs("wuv", wuv_hbm, wuv_v)
    for i, (s, n) in enumerate(WG_CHUNKS):
        add_blocks(f"wg{i}", wg_hbm, wg_v, s, n)
    hpc = H // WO_CHUNKS
    for i in range(WO_CHUNKS):
        add(f"wo{i}", wo_hbm.at[pl.ds(i * hpc * D, hpc * D)], wo_v.at[pl.ds(i * hpc * D, hpc * D)])
    for i, (s, n) in enumerate(WU_CHUNKS):
        add_blocks(f"wu{i}", wu_hbm, wu_v, s, n)
    for i, (s, n) in enumerate(WD_CHUNKS):
        add_blocks(f"wd{i}", wd_hbm, wd_v, s, n)
    for b, fb in enumerate(LATE):
        add(f"wgL{fb}", wg_hbm.bitcast(u32).at[pl.ds(64 * fb, 64)], gul.at[2 * b])
        add(f"wuL{fb}", wu_hbm.bitcast(u32).at[pl.ds(64 * fb, 64)], gul.at[2 * b + 1])

    sub = lax.broadcasted_iota(i32, (8, 128), 0)
    xts = [xt0, xt1, xt2, xt3, xt4]
    zs = [pl.semaphore_read(zsem.at[n]) for n in range(NZ)]
    z0 = zs[0]
    zvec = jnp.zeros((8, 128), u32) + zs[-1].astype(u32)
    zmask = zvec != 0
    zi = iter(zs[1:-1])

    def repack(src, hp, dst, rows):
        for i in range(rows // 16):
            v = src[hp, pl.ds(16 * i, 16), :]
            dst[2 * hp, pl.ds(8 * i, 8), :] = _u32(_lo(v).astype(bf16))
            dst[2 * hp + 1, pl.ds(8 * i, 8), :] = _u32(_hi(v).astype(bf16))

    def prep_wq():
        def both(k, carry):
            hp = k + Q_MXU // 2
            wait_pair("wq", hp)
            repack(wq_v, hp, wqb, M)
            v = wq_v[hp]
            wqf[2 * k] = _lo(v)
            wqf[2 * k + 1] = _hi(v)
            return carry

        for hp in range(Q_MXU // 2):
            cps[f"wq{hp}"].wait()
            repack(wq_v, hp, wqb, M)
        lax.fori_loop(0, Q_VPU // 2, both, 0)
        ones = jnp.ones((8, M), bf16)

        def colsum(g, carry):
            acc = jnp.zeros((8, 128), f32)
            for r in range(8):
                acc = jnp.where(sub == r, _dot(ones, _bf16(wqb[8 * g + r])), acc)
            cs_v[pl.ds(pl.multiple_of(8 * g, 8), 8), :] = acc
            return carry
        lax.fori_loop(0, H // 8, colsum, 0)

    def prep_wuk():
        def pair_b(hp, carry):
            wait_pair("wuk", hp)
            for cb in range(NC):
                t = wuk_v[hp, pl.ds(cb * 128, 128), :].T
                ukb[2 * hp, pl.ds(cb * 64, 64), :] = _u32(_lo(t).astype(bf16))
                ukb[2 * hp + 1, pl.ds(cb * 64, 64), :] = _u32(_hi(t).astype(bf16))
            return carry

        def pair_bf(hp, carry):
            wait_pair("wuk", hp)
            for cb in range(NC):
                t = wuk_v[hp, pl.ds(cb * 128, 128), :].T
                lo, hi = _lo(t), _hi(t)
                ukf[(2 * hp - (H - K2_VPU)) * NC + cb] = lo
                ukf[(2 * hp + 1 - (H - K2_VPU)) * NC + cb] = hi
                ukb[2 * hp, pl.ds(cb * 64, 64), :] = _u32(lo.astype(bf16))
                ukb[2 * hp + 1, pl.ds(cb * 64, 64), :] = _u32(hi.astype(bf16))
            return carry
        def with_z(fn):
            def body(hp, carry):
                fn(hp, carry)
                z_head(hp)
                return carry
            return body
        cuts = sorted({0, min(ZH_UK, H // 2), (H - K2_VPU) // 2, H // 2})
        for a, b in zip(cuts[:-1], cuts[1:]):
            fn = pair_b if a < (H - K2_VPU) // 2 else pair_bf
            if a < ZH_UK:
                lax.fori_loop(a, b, with_z(fn), 0)
            else:
                lax.fori_loop(a, b, fn, 0)

    def prep_c():
        for cb in range(NC):
            cps[f"c{cb}"].wait()

            def blk(i, carry, cb=cb):
                for kk in range(16):
                    kb = 16 * i + kk
                    t = _bf16(c2[cb, pl.ds(pl.multiple_of(kb * 64, 64), 64), :])
                    cT[kb, pl.ds(cb * 64, 64), :] = _u32(t.T)
                return carry
            lax.fori_loop(0, NK // 16, blk, 0)

    def prep_wuv():
        def pair(hp, carry):
            wait_pair("wuv", hp)
            repack(wuv_v, hp, uvb, DC)
            return carry

        def pair_z(hp, carry):
            z_head(hp + ZH_UK)
            return pair(hp, carry)
        lax.fori_loop(0, ZH_UV, pair_z, 0)
        if ZH_UV < H // 2:
            lax.fori_loop(ZH_UV, H // 2, pair, 0)

    def prep_gu(mat, raw, fb0, fb1):
        def tile(fb, j):
            return raw[pl.ds(pl.multiple_of(fb * 128, 128), 128), pl.ds(j * 128, 128)].T

        def vpu_blks(i, carry):
            for fb in (2 * i, 2 * i + 1):
                for j in range(NJ):
                    guf[2 * fb + mat, pl.ds(j * 128, 128), :] = tile(fb, j).astype(f32)
            return carry
        if fb0 < F_VPU:
            lax.fori_loop(fb0 // 2, min(fb1, F_VPU) // 2, vpu_blks, 0)

        for fb in range(max(fb0, F_VPU), min(fb1, NF - 1)):
            for j in range(NJ):
                gub[z0 + 2 * (fb - F_VPU) + mat, pl.ds(j * 64, 64), :] = _u32(tile(fb, j))
        if fb0 <= NF - 1 < fb1:
            for j in range(NJ):
                t = raw[pl.ds((NF - 1) * 128, 64), pl.ds(j * 128, 128)]
                t = jnp.concatenate([t, jnp.zeros((64, 128), bf16)], axis=0).T
                gub[z0 + 2 * (NF - 1 - F_VPU) + mat, pl.ds(j * 64, 64), :] = _u32(t)

    def prep_late_wd():
        for b, fb in enumerate(LATE):
            cps[f"wdL{fb}"].wait()
            acc = None
            for j in range(NJ):
                w = _u32(wd_v[pl.ds(fb * 128, 128), pl.ds(j * 128, 128)])
                wdb[z0 + fb * NJ + j] = w
                t = jnp.concatenate([_lo(w), _hi(w)], axis=0)
                wdf[j, pl.ds(b * 128, 128), :] = t
                wdp[b * NJ + j] = _u32(t.astype(bf16))
                r = jnp.sum(t, axis=-1, keepdims=True)
                acc = r if acc is None else acc + r
            rm_v[b] = jnp.broadcast_to(acc * (1.0 / M), (128, 128))

    def z_head(h):
        cs = cs_v[pl.ds(h, 1), :]
        for b, fb in enumerate(LATE):
            z = None
            for j in range(NJ):
                y = _dot(_bf16(wdp[b * NJ + j]), _bf16(wqb[h, pl.ds(j * 64, 64), :]))
                z = y if z is None else z + y
            zf[h, pl.ds(b * 128, 128), :] = z - rm_v[b] * cs

    def prep_z(h0, h1):
        if h0 < h1:
            lax.fori_loop(h0, h1, lambda h, c: (z_head(h), c)[1], 0)

    def prep_wo(h0, h1):
        def vpu_head(h, carry):
            for j in range(NJ):
                t = wo_v[pl.ds(pl.multiple_of(h * 128, 128), 128), pl.ds(j * 128, 128)]
                wof[h * NJ + j] = t.astype(f32)
            return carry

        def mxu_head(h, carry):
            for j in range(NJ):
                t = wo_v[pl.ds(pl.multiple_of(h * 128, 128), 128), pl.ds(j * 128, 128)]
                wob[(h - O_VPU) * NJ + j] = _u32(t)
            return carry
        if h0 < O_VPU:
            lax.fori_loop(h0, min(h1, O_VPU), vpu_head, 0)
        if h1 > O_VPU:
            lax.fori_loop(max(h0, O_VPU), h1, mxu_head, 0)

    def stage_xt(x, mean):
        for kb in range(NJ):
            t = _xpose_bcast(x[0:1, kb * 128:(kb + 1) * 128])
            xts[kb][pl.ds(0, 128), :] = t - mean[0:1, 0:1]

    def vpu_cols(wref, idxs, static, prev, rows=M, post=False):
        accs = [None] * len(idxs)
        if not static:
            zf = next(zi)
            for kb in range(rows // 128):
                xts[kb][pl.ds(zf + 128, 8), :] = pltpu.bitcast(zvec, f32)
        for i in range(rows // 8):
            xt = xts[i // 16][pl.ds(8 * (i % 16), 8), :]
            for n, c in enumerate(idxs):
                p = xt * wref[c, pl.ds(8 * i, 8), :]
                if accs[n] is None:
                    if prev:
                        p = jnp.where(zmask, prev[n % len(prev)], p)
                    accs[n] = p
                else:
                    accs[n] = accs[n] + p
        ys = [_rowsum(a) for a in accs]
        prev[:] = ys if post else accs
        return ys

    def region(fn, first, zero, tag):
        if tag not in (REG1 if first else REG2):
            return fn()
        return lax.cond(z0 == 0, fn, lambda: zero)

    def phase_a(x, xb, mean, rstd):
        stage_xt(x, mean)
        qabs = [[None] * NC for _ in range(4)]

        def absorb(h, qh):
            qb = qh.astype(bf16)
            for cb in range(NC):
                y = _dot(qb, _bf16(ukb[h, pl.ds(cb * 64, 64), :]))
                old = qabs[h // 8][cb]
                qabs[h // 8][cb] = y if old is None else jnp.where(sub == h % 8, y, old)

        qm = [_dot(xb, _bf16(wqb[h])) for h in range(Q_MXU)]
        for h in range(Q_MXU):
            absorb(h, qm[h])
        h0 = 0
        prev = []
        for gsz in Q_GROUPS:
            qs = vpu_cols(wqf, list(range(h0, h0 + gsz)), h0 == 0, prev)
            for n in range(gsz):
                absorb(Q_MXU + h0 + n, qs[n])
            h0 += gsz
        scale = rstd[0:1, 0:1] * ((D ** -0.5) * LOG2E)
        qa = jnp.concatenate([jnp.concatenate(qabs[g], axis=1) for g in range(4)], axis=0)
        return (qa * scale).astype(bf16)

    def phase_b(qa, ycalc=None):
        sc = None
        side = {}
        def scores(k0, k1):
            mrun = None
            for kb in range(k0, k1):
                s = _dot(qa, _bf16(cT[kb]))
                s_v[kb] = s
                if ycalc is not None and kb == TIE_KB:
                    side['sc'] = ycalc(s[0:8, :])
                if ycalc is not None and kb == TIE_KB2:
                    ycalc.late(s[0:8, :])
                mrun = s if mrun is None else jnp.maximum(mrun, s)
            return jnp.max(mrun, axis=-1, keepdims=True)

        def weighted(k0, k1, mrow):
            lsum = None
            cacc = [None] * NC
            for kb in range(k0, k1):
                p = jnp.exp2(s_v[kb] - mrow if sc is None else (s_v[kb] - mrow) * sc)
                lsum = p if lsum is None else lsum + p
                pb = p.astype(bf16)
                for cb in range(NC):
                    y = _dot(pb, _bf16(c2[cb, pl.ds(kb * 64, 64), :]))
                    cacc[cb] = y if cacc[cb] is None else cacc[cb] + y
            return jnp.sum(lsum, axis=-1, keepdims=True), cacc

        hk = NK // 2
        ma = scores(0, hk)
        mb = scores(hk, NK)
        sc = side.get('sc')
        la, ca = weighted(0, hk, ma)
        lb, cb_ = weighted(hk, NK, mb)
        m = jnp.maximum(ma, mb)
        fa = jnp.exp2(ma - m if sc is None else (ma - m) * sc)
        fb = jnp.exp2(mb - m if sc is None else (mb - m) * sc)
        linv = 1.0 / (la * fa + lb * fb)
        wa = fa * linv
        wb = fb * linv
        return jnp.concatenate([(ca[c] * wa + cb_[c] * wb).astype(bf16) for c in range(NC)], axis=1)

    def phase_c(cx):
        vacc = [None] * NJ
        macc = [None] * NJ
        ys = {}
        la = C_LA
        for i in range(H + la):
            if i < H:
                g = i // 8
                ys[i] = _dot(cx[8 * g:8 * g + 8, :], _bf16(uvb[i]))
            h = i - la
            if 0 <= h < O_VPU:
                xt = _xpose_bcast(ys[h][h % 8:h % 8 + 1, :])
                if C_LK is None:
                    for ii in range(D // 8):
                        for j in range(NJ):
                            p = xt[8 * ii:8 * ii + 8, :] * wof[h * NJ + j, pl.ds(8 * ii, 8), :]
                            vacc[j] = p if vacc[j] is None else vacc[j] + p
                else:
                    tie = None
                    for j in range(NJ):
                        for ii in range(D // 8):
                            p = xt[8 * ii:8 * ii + 8, :] * wof[h * NJ + j, pl.ds(8 * ii, 8), :]
                            if j == 0 and ii == 0 and h > 0:
                                p = jnp.where(zmask, vacc[NJ - 1], p)
                            if j == NJ - 1 and ii == 0:
                                p = jnp.where(zmask, tie, p)
                            vacc[j] = p if vacc[j] is None else vacc[j] + p
                            if j == 0 and ii == C_LK:
                                tie = vacc[0]
        for h in range(O_VPU, H):
            lhs = jnp.broadcast_to(ys[h][h % 8:h % 8 + 1, :], (8, 128)).astype(bf16)
            for j in range(NJ):
                yy = _dot(lhs, _bf16(wob[(h - O_VPU) * NJ + j]))
                macc[j] = yy if macc[j] is None else macc[j] + yy
        return jnp.concatenate([_rowsum(vacc[j]) + macc[j] for j in range(NJ)], axis=1)

    def swiglu(x, xb, mean, rstd, on_block, skip=()):
        stage_xt(x, mean)

        def act(g, u):
            if FAST_ACT:
                return _swiglu(g, u, rstd).astype(bf16)
            return (jax.nn.silu(g * rstd) * (u * rstd)).astype(bf16)

        for i in range(NF - F_VPU):
            if F_VPU + i in skip:
                continue
            on_block(F_VPU + i, act(_dot(xb, _bf16(gub[2 * i])), _dot(xb, _bf16(gub[2 * i + 1]))), 0)
        on_block(None, None, 0)
        f0 = 0
        prev = []
        for gsz in F_GROUPS:
            ys = vpu_cols(guf, list(range(2 * f0, 2 * (f0 + gsz))), f0 == 0, prev)
            for n in range(gsz):
                on_block(f0 + n, act(ys[2 * n], ys[2 * n + 1]), 1)
            f0 += gsz

    def phase_d1(x, xb, mean, rstd):
        hs = {}

        def keep(fb, h, kind):
            if fb is not None:
                hs[fb] = h
        swiglu(x, xb, mean, rstd, keep, skip=LATE)
        return tuple(hs[fb] for fb in EARLY)

    def phase_d2(x, xb, mean, rstd):
        yacc = [None] * NJ
        held = []

        def down(fb, hb):
            for j in range(NJ):
                yy = _dot(hb, _bf16(wdb[fb * NJ + j]))
                yacc[j] = yy if yacc[j] is None else yacc[j] + yy

        def on_block(fb, h, kind):
            if fb is None:
                for b, hb in held:
                    down(b, hb)
            elif kind == 0:
                held.append((fb, h))
            else:
                down(fb, h)
        swiglu(x, xb, mean, rstd, on_block)
        return jnp.concatenate(yacc, axis=1)

    def phase_a_early(v):
        vb = v.astype(bf16)
        for kb in range(NJ):
            xts[kb][pl.ds(0, 128), :] = _xpose_bcast(v[0:1, kb * 128:(kb + 1) * 128])
        delta = jnp.sum(vb.astype(f32), axis=-1, keepdims=True) * (1.0 / M)
        q = [None] * 4

        def put(h, y):
            q[h // 8] = y if q[h // 8] is None else jnp.where(sub == h % 8, y, q[h // 8])

        for h in range(AE_MXU):
            put(h, _dot(vb, _bf16(wqb[h])))
        h0 = AE_MXU
        prev = []
        for gsz in AE_GROUPS:
            ys = vpu_cols(wqf, list(range(h0 - Q_MXU, h0 - Q_MXU + gsz)), h0 == AE_MXU, prev, post=AE_POST)
            for n in range(gsz):
                put(h0 + n, ys[n])
            h0 += gsz
        return tuple(q[g] - delta * cs_v[pl.ds(8 * g, 8), :] for g in range(4))

    def late_hidden(xb, rstd):
        xf = xb.astype(f32)
        for b in range(NL):
            gu = []
            for m in range(2):
                lo, hi = None, None
                for j in range(NJ):
                    w = gul[2 * b + m, :, pl.ds(j * 128, 128)]
                    xj = xf[0:1, j * 128:(j + 1) * 128]
                    pl_, ph_ = _lo(w) * xj, _hi(w) * xj
                    lo = pl_ if lo is None else lo + pl_
                    hi = ph_ if hi is None else hi + ph_
                s_ = jnp.sum(jnp.concatenate([lo, hi], axis=0), axis=-1, keepdims=True)
                gu.append(jnp.broadcast_to(s_, (128, 128)))
            xts[b][pl.ds(0, 128), :] = _swiglu(gu[0], gu[1], rstd[0:1, 0:1])

    def phase_a2(qbase, rs):
        qabs = [[None] * NC for _ in range(4)]

        def put(h, cb, y):
            old = qabs[h // 8][cb]
            qabs[h // 8][cb] = y if old is None else jnp.where(sub == h % 8, y, old)

        def base(h):
            return _rowsum(jnp.where(sub == h % 8, qbase[h // 8], 0.0))

        def absorb_mxu(h, qh):
            qb = qh.astype(bf16)
            for cb in range(NC):
                put(h, cb, _dot(qb, _bf16(ukb[h, pl.ds(cb * 64, 64), :])))

        segs = []

        def absorb_vpu(h, qh):
            xq = _xpose_bcast(qh[0:1, :])
            for cb in range(NC):
                acc = None
                for i in range(16):
                    p = xq[8 * i:8 * i + 8] * ukf[(h - (H - K2_VPU)) * NC + cb, pl.ds(8 * i, 8), :]
                    if acc is None:
                        if len(segs) >= K2_LANES:
                            p = jnp.where(zmask, segs[len(segs) - K2_LANES], p)
                        acc = p
                    else:
                        acc = acc + p
                segs.append(acc)
                put(h, cb, _rowsum(acc))

        mh = list(range(H - K2_VPU))
        order = mh[:A2_KPOS] + list(range(H - K2_VPU, H)) + mh[A2_KPOS:]
        prev = []
        held = []
        pos = 0
        for gi, gsz in enumerate(A2_GROUPS):
            hh = order[pos:pos + gsz]
            ys = vpu_cols(zf, hh, pos == 0, prev, rows=128 * NL, post=A2_POST)
            for n, h in enumerate(hh):
                qh = ys[n] * rs + base(h)
                if h >= H - K2_VPU:
                    held.append((h, qh))
                else:
                    absorb_mxu(h, qh)
            pos += gsz
        for h, qh in held:
            absorb_vpu(h, qh)
        qa = jnp.concatenate([jnp.concatenate(qabs[g], axis=1) for g in range(4)], axis=0)
        return qa.astype(bf16)

    def router(xn):
        r = jnp.sum(xn.astype(bf16).astype(f32) * wr, axis=-1, keepdims=True)
        return jax.nn.sigmoid(r)

    cps["x"].wait()
    cps["wr"].wait()
    x = jnp.broadcast_to(x_v[0].astype(f32), (8, M))
    wr = wr_v[...].astype(f32).reshape(1, M)

    xc, rstd, mean = _ln_parts(x)
    xb = xc.astype(bf16)
    prep_wq()
    prep_late_wd()
    prep_wuk()
    qa = region(lambda: phase_a(x, xb, mean, rstd), True, jnp.zeros((H, DC), bf16), 'A')
    prep_c()
    cx = region(lambda: phase_b(qa), True, jnp.zeros((H, DC), bf16), 'B')
    prep_wuv()
    for i, (s0, n0) in enumerate(WG_CHUNKS):
        cps[f"wg{i}"].wait()
        prep_gu(0, wg_v, s0, s0 + n0)
    zh = ZH_UK + ZH_UV
    zper = (H - zh + WO_CHUNKS - 2) // (WO_CHUNKS - 1)
    for i in range(WO_CHUNKS):
        cps[f"wo{i}"].wait()
        prep_wo(i * hpc, (i + 1) * hpc)
        prep_z(min(zh + i * zper, H), min(zh + (i + 1) * zper, H))
    x = x + region(lambda: phase_c(cx), True, jnp.zeros((8, M), f32), 'C')

    xc, rstd, mean = _ln_parts(x)
    xn = xc * rstd
    xb = xc.astype(bf16)
    rs = router(xn)
    for i, (s0, n0) in enumerate(WU_CHUNKS):
        cps[f"wu{i}"].wait()
        prep_gu(1, wu_v, s0, s0 + n0)
    hs_e = region(lambda: phase_d1(x, xb, mean, rstd), True,
                  tuple(jnp.zeros((8, 128), bf16) for _ in range(len(EARLY))), 'D')
    hs = dict(zip(EARLY, hs_e))
    u = x + (xn + xn * 0.0)
    yj = [None] * NJ

    def down1(fb, hb):
        for j in range(NJ):
            n = min(128, F - fb * 128)
            t = wd_v[pl.ds(fb * 128, n), pl.ds(j * 128, 128)]
            if n < 128:
                t = jnp.concatenate([t, jnp.zeros((128 - n, 128), bf16)], axis=0)
            wdb[z0 + fb * NJ + j] = _u32(t)
            yy = _dot(hb, t)
            yj[j] = yy if yj[j] is None else yj[j] + yy

    for i, (fb0, nb) in enumerate(WD_CHUNKS):
        cps[f"wd{i}"].wait()
        for fb in range(fb0, fb0 + nb):
            down1(fb, hs[fb])
    v = u + jnp.concatenate(yj, axis=1) * rs
    qbase = region(lambda: phase_a_early(v), True,
                   tuple(jnp.zeros((8, 128), f32) for _ in range(4)), 'E')
    for fb in LATE:
        cps[f"wgL{fb}"].wait()
        cps[f"wuL{fb}"].wait()
    late_hidden(xb, rstd)
    if True:
        qa = phase_a2(qbase, rs)
        xs = {}

        def sc2(tie):
            ys, j0, pv = [], 0, [tie]
            for gsz in Y_GROUPS:
                ys += vpu_cols(wdf, list(range(j0, j0 + gsz)), False, pv, rows=128 * NL)
                j0 += gsz
            xs['x'] = v + jnp.concatenate(ys, axis=1) * rs
            xc, rstd2, mean = _ln_parts(xs['x'])
            return rstd2[0:1, 0:1] * ((D ** -0.5) * LOG2E)

        def late_prep(tie):
            for b, fb in enumerate(LATE):
                for m in range(2):
                    for j in range(NJ):
                        t = _bf16(gul[2 * b + m, :, pl.ds(j * 128, 128)])
                        gub[z0 + 2 * (fb - F_VPU) + m, pl.ds(j * 64, 64), :] = _u32(t.T)
        sc2.late = late_prep
    cx = region(lambda: phase_b(qa, sc2), False, jnp.zeros((H, DC), bf16), 'B')
    if Y_VPU:
        x = xs['x']
    x = x + region(lambda: phase_c(cx), False, jnp.zeros((8, M), f32), 'C')
    xc, rstd, mean = _ln_parts(x)
    xn = xc * rstd
    xb = xc.astype(bf16)
    rs = router(xn)
    y = region(lambda: phase_d2(x, xb, mean, rstd), False, jnp.zeros((8, M), f32), 'D')
    x = x + (xn + (xn * 0.0 + y * rs))

    o_v[0] = x[0:1, :].astype(bf16)
    ocp = pltpu.make_async_copy(o_v, o_hbm, sems.at[len(names)])
    ocp.start()
    ocp.wait()


@jax.jit
def pallas_interleave_layers__compressed_kv_cla__moe_arch_mod__decode_kernel(
    A_x, A_c_kv, A_w_q, A_w_uk, A_w_uv, A_w_o, B_x, B_w_r, B_w_gate, B_w_up, B_w_down,
):
    del B_x
    ins = [
        A_x, B_w_r, A_w_q, A_w_uk,
        A_c_kv.reshape(SK, DC),
        A_w_uv,
        A_w_o.reshape(H * D, M),
        B_w_gate.T, B_w_up.T,
        B_w_down,
    ]
    scratch = [
        pltpu.VMEM((1, 1, M), bf16),
        pltpu.VMEM((M,), bf16),
        pltpu.VMEM((H // 2, M, D), u32),
        pltpu.VMEM((H // 2, DC, D), u32),
        pltpu.VMEM((H // 2, DC, D), u32),
        pltpu.VMEM((H * D, M), bf16),
        pltpu.VMEM((F, M), bf16),
        pltpu.VMEM((F, M), bf16),
        pltpu.VMEM((F, M), bf16),
        pltpu.VMEM((H, M // 2, 128), u32),
        pltpu.VMEM((Q_VPU, M, 128), f32),
        pltpu.VMEM((H, NC * 64, 128), u32),
        pltpu.VMEM((K2_VPU * NC, 128, 128), f32),
        pltpu.VMEM((H, 128), f32),
        pltpu.VMEM((NL, 128, 128), f32),
        pltpu.VMEM((NJ, NL * 128, 128), f32),
        pltpu.VMEM((2 * NL, 64, M), u32),
        pltpu.VMEM((NL * NJ, 64, 128), u32),
        pltpu.VMEM((H, NL * 128, 128), f32),
        pltpu.VMEM((NF * NJ, 64, 128), u32),
        pltpu.VMEM((NK, DC // 2, 128), u32),
        pltpu.VMEM((NC, SK // 2, 128), u32),
        pltpu.VMEM((H, DC // 2, 128), u32),
        pltpu.VMEM(((H - O_VPU) * NJ, 64, 128), u32),
        pltpu.VMEM((O_VPU * NJ, 128, 128), f32),
        pltpu.VMEM((2 * (NF - F_VPU), M // 2, 128), u32),
        pltpu.VMEM((2 * F_VPU, M, 128), f32),
        *[pltpu.VMEM((160, 128), f32) for _ in range(NJ)],
        pltpu.VMEM((NK, H, 128), f32),
        pltpu.VMEM((1, 1, M), bf16),
        pltpu.SemaphoreType.DMA((96,)),
        pltpu.SemaphoreType.REGULAR((NZ,)),
    ]
    return pl.pallas_call(
        _kernel,
        in_specs=[pl.BlockSpec(memory_space=pltpu.HBM)] * len(ins),
        out_specs=pl.BlockSpec(memory_space=pltpu.HBM),
        out_shape=jax.ShapeDtypeStruct((1, 1, M), bf16),
        scratch_shapes=scratch,
        compiler_params=pltpu.CompilerParams(
            vmem_limit_bytes=120 * 1024 * 1024,
            disable_semaphore_checks=True,
            disable_bounds_checks=True,
            flags={"XLA_TPU_FORCE_LP_LLO_SCHEDULER": True},
        ),
    )(*ins)
```

```python
import jax
import jax.numpy as jnp
from jax import lax
import jax.experimental.pallas as pl
import jax.experimental.pallas.tpu as pltpu

bf16 = jnp.bfloat16
f32 = jnp.float32
u32 = jnp.uint32
i32 = jnp.int32

M = 640
H = 32
D = 128
SK = 4096
DC = 512
F = 1728
NJ = M // 128
NC = DC // 128
NK = SK // 128
NF = (F + 127) // 128
LOG2E = 1.4426950408889634
EPS = 1e-5

REG1 = 'ABCD'
REG2 = 'C'

Q_MXU = 8
Q_GROUPS = [4, 4, 4, 4, 4, 4]
O_VPU = 21
F_GROUPS = [2, 2, 2, 2]
F_VPU = sum(F_GROUPS)
Q2_MXU = 8
K2_VPU = 8
K2_LANES = 3
Q_VPU = H - Q_MXU
assert sum(Q_GROUPS) == Q_VPU and Q_MXU % 2 == 0 and F_VPU % 2 == 0

WO_CHUNKS = 4
LATE = [12,13]
WG_CHUNKS = [(0,12)]
WU_CHUNKS = [(0,4),(4,4),(8,4)]
WD_CHUNKS = [(0,3),(3,3),(6,3),(9,1),(10,1),(11,1)]
NL = len(LATE)
LR = [min(128, F - 128 * fb) for fb in LATE]
LO = [sum(LR[:b]) for b in range(NL)]
KL = sum(LR)
assert all(r == 128 for r in LR[:-1])
AE_LATE = 8
EARLY = [fb for fb in range(NF) if fb not in LATE]
ZH_UK = 16
ZH_UV = 16
LATE_STAGES = [[('g', 11), ('u', 11), ('g', 12), ('u', 12)]]
Y_VPU = True
TIE_KB = 2
A2_KPOS = 8
FAST_ACT = True
D_JOINT = True
MERGE_IN_C = False
FOLD_D = True
FOLD_RS = True
A2_LPOS = 16
Y_GROUPS = [5]
C_LK = 6
C_LA = 4
A2_POST = False
AE_POST = False
A2_MPRE = [8, 0, 0, 0, 0, 0]
TIE_KB2 = 3
A2_GROUPS = [4, 4, 4, 4, 4, 4, 4, 4]
AE_MXU = 24
AE_GROUPS = [4,4]
NZ = 32


def _dot(a, b):
    return jnp.dot(a, b, preferred_element_type=f32)


def _u32(a):
    return pltpu.bitcast(a, u32)


def _bf16(a):
    return pltpu.bitcast(a, bf16)


def _lo(w):
    return pltpu.bitcast(w << 16, f32)


def _hi(w):
    return pltpu.bitcast(w & jnp.uint32(0xFFFF0000), f32)


def _rowsum(acc):
    return jnp.broadcast_to(jnp.sum(acc, axis=0, keepdims=True), (8, 128))


def _rowsum4(a):
    sub = lax.broadcasted_iota(i32, (8, 128), 0)
    m1 = (sub & 1) == 0
    m2 = (sub & 2) == 0
    s01 = jnp.where(m1, a[0], a[1]) + pltpu.roll(jnp.where(m1, a[1], a[0]), 7, 0)
    s23 = jnp.where(m1, a[2], a[3]) + pltpu.roll(jnp.where(m1, a[3], a[2]), 7, 0)
    s = jnp.where(m2, s01, s23) + pltpu.roll(jnp.where(m2, s23, s01), 6, 0)
    return s + pltpu.roll(s, 4, 0)


def _ln_parts(x):
    m = jnp.sum(x, axis=-1, keepdims=True) * (1.0 / M)
    m2 = jnp.sum(x * x, axis=-1, keepdims=True) * (1.0 / M)
    v = jnp.maximum(m2 - m * m, 0.0)
    return x - m, lax.rsqrt(v + EPS), m


def _xpose_bcast(row):
    r16 = jnp.broadcast_to(row, (16, 128)).astype(bf16)
    return jnp.concatenate([r16] * 8, axis=0).T.astype(f32)


def _swiglu(g, u, rstd, post=None):
    e = jnp.exp2(g * (rstd * -LOG2E))
    c = rstd * rstd if post is None else rstd * rstd * post
    return (g * u) * c * pl.reciprocal(1.0 + e, approx=True)


def _kernel(x_hbm, wr_hbm, wq_hbm, wuk_hbm, c_hbm, wuv_hbm, wo_hbm, wg_hbm, wu_hbm, wd_hbm,
            o_hbm,
            x_v, wr_v, wq_v, wuk_v, wuv_v, wo_v, wg_v, wu_v, wd_v,
            wqb, wqf, ukb, ukf, cs_v, rm_v, wdf, gul, wdp, zf, wdb, cT, c2, uvb, wob, wof, gub, guf, xt0, xt1, xt2, xt3, xt4, s_v, o_v, sems, zsem):
    cps = {}
    names = []
    families = {}

    def add(name, src, dst):
        cp = pltpu.make_async_copy(src, dst, sems.at[len(names)])
        cp.start()
        cps[name] = cp
        names.append(name)

    def add_pairs(name, src, dst):
        s32 = src.bitcast(u32)
        families[name] = (s32, dst, len(names))
        for hp in range(H // 2):
            add(f"{name}{hp}", s32.at[:, hp, :], dst.at[hp])

    def wait_pair(name, hp):
        src, dst, base = families[name]
        pltpu.make_async_copy(src.at[:, hp, :], dst.at[hp], sems.at[base + hp]).wait()

    add("x", x_hbm, x_v)
    add("wr", wr_hbm, wr_v)
    def add_blocks(name, src, dst, fb0, nb):
        rows = min(128 * nb, F - 128 * fb0)
        add(name, src.at[pl.ds(128 * fb0, rows)], dst.at[pl.ds(128 * fb0, rows)])

    add_pairs("wq", wq_hbm, wq_v)
    for fb in LATE:
        add_blocks(f"wdL{fb}", wd_hbm, wd_v, fb, 1)
    add_pairs("wuk", wuk_hbm, wuk_v)
    c32 = c_hbm.bitcast(u32)
    for cb in range(NC):
        add(f"c{cb}", c32.at[:, pl.ds(cb * 128, 128)], c2.at[cb])
    add_pairs("wuv", wuv_hbm, wuv_v)
    for i, (s, n) in enumerate(WG_CHUNKS):
        add_blocks(f"wg{i}", wg_hbm, wg_v, s, n)
    hpc = H // WO_CHUNKS
    for i in range(WO_CHUNKS):
        add(f"wo{i}", wo_hbm.at[pl.ds(i * hpc * D, hpc * D)], wo_v.at[pl.ds(i * hpc * D, hpc * D)])
    for i, (s, n) in enumerate(WU_CHUNKS):
        add_blocks(f"wu{i}", wu_hbm, wu_v, s, n)
    for i, (s, n) in enumerate(WD_CHUNKS):
        add_blocks(f"wd{i}", wd_hbm, wd_v, s, n)
    for b, fb in enumerate(LATE):
        n = LR[b] // 2
        add(f"wgL{fb}", wg_hbm.bitcast(u32).at[pl.ds(64 * fb, n)], gul.at[2 * b, pl.ds(0, n)])
        add(f"wuL{fb}", wu_hbm.bitcast(u32).at[pl.ds(64 * fb, n)], gul.at[2 * b + 1, pl.ds(0, n)])

    sub = lax.broadcasted_iota(i32, (8, 128), 0)
    xts = [xt0, xt1, xt2, xt3, xt4]
    zs = [pl.semaphore_read(zsem.at[n]) for n in range(NZ)]
    z0 = zs[0]
    zvec = jnp.zeros((8, 128), u32) + zs[-1].astype(u32)
    zmask = zvec != 0
    zi = iter(zs[1:-1])

    def repack(src, hp, dst, rows):
        for i in range(rows // 16):
            v = src[hp, pl.ds(16 * i, 16), :]
            dst[2 * hp, pl.ds(8 * i, 8), :] = _u32(_lo(v).astype(bf16))
            dst[2 * hp + 1, pl.ds(8 * i, 8), :] = _u32(_hi(v).astype(bf16))

    def prep_wq():
        def both(k, carry):
            hp = k + Q_MXU // 2
            wait_pair("wq", hp)
            repack(wq_v, hp, wqb, M)
            v = wq_v[hp]
            wqf[2 * k] = _lo(v)
            wqf[2 * k + 1] = _hi(v)
            return carry

        for hp in range(Q_MXU // 2):
            cps[f"wq{hp}"].wait()
            repack(wq_v, hp, wqb, M)
        lax.fori_loop(0, Q_VPU // 2, both, 0)
        ones = jnp.ones((8, M), bf16)

        def colsum(g, carry):
            acc = jnp.zeros((8, 128), f32)
            for r in range(8):
                acc = jnp.where(sub == r, _dot(ones, _bf16(wqb[8 * g + r])), acc)
            cs_v[pl.ds(pl.multiple_of(8 * g, 8), 8), :] = acc
            return carry
        lax.fori_loop(0, H // 8, colsum, 0)

    def prep_wuk():
        def pair_b(hp, carry):
            wait_pair("wuk", hp)
            for cb in range(NC):
                t = wuk_v[hp, pl.ds(cb * 128, 128), :].T
                ukb[2 * hp, pl.ds(cb * 64, 64), :] = _u32(_lo(t).astype(bf16))
                ukb[2 * hp + 1, pl.ds(cb * 64, 64), :] = _u32(_hi(t).astype(bf16))
            return carry

        def pair_bf(hp, carry):
            wait_pair("wuk", hp)
            for cb in range(NC):
                t = wuk_v[hp, pl.ds(cb * 128, 128), :].T
                lo, hi = _lo(t), _hi(t)
                ukf[(2 * hp - (H - K2_VPU)) * NC + cb] = lo
                ukf[(2 * hp + 1 - (H - K2_VPU)) * NC + cb] = hi
                ukb[2 * hp, pl.ds(cb * 64, 64), :] = _u32(lo.astype(bf16))
                ukb[2 * hp + 1, pl.ds(cb * 64, 64), :] = _u32(hi.astype(bf16))
            return carry
        def with_z(fn):
            def body(hp, carry):
                fn(hp, carry)
                z_head(hp)
                return carry
            return body
        cuts = sorted({0, min(ZH_UK, H // 2), (H - K2_VPU) // 2, H // 2})
        for a, b in zip(cuts[:-1], cuts[1:]):
            fn = pair_b if a < (H - K2_VPU) // 2 else pair_bf
            if a < ZH_UK:
                lax.fori_loop(a, b, with_z(fn), 0)
            else:
                lax.fori_loop(a, b, fn, 0)

    def prep_c():
        for cb in range(NC):
            cps[f"c{cb}"].wait()

            def blk(i, carry, cb=cb):
                for kk in range(16):
                    kb = 16 * i + kk
                    t = _bf16(c2[cb, pl.ds(pl.multiple_of(kb * 64, 64), 64), :])
                    cT[kb, pl.ds(cb * 64, 64), :] = _u32(t.T)
                return carry
            lax.fori_loop(0, NK // 16, blk, 0)

    def prep_wuv():
        def pair(hp, carry):
            wait_pair("wuv", hp)
            repack(wuv_v, hp, uvb, DC)
            return carry

        def pair_z(hp, carry):
            z_head(hp + ZH_UK)
            return pair(hp, carry)
        lax.fori_loop(0, ZH_UV, pair_z, 0)
        if ZH_UV < H // 2:
            lax.fori_loop(ZH_UV, H // 2, pair, 0)

    def prep_gu(mat, raw, fb0, fb1):
        def tile(fb, j):
            return raw[pl.ds(pl.multiple_of(fb * 128, 128), 128), pl.ds(j * 128, 128)].T

        def vpu_blks(i, carry):
            for fb in (2 * i, 2 * i + 1):
                for j in range(NJ):
                    guf[2 * fb + mat, pl.ds(j * 128, 128), :] = tile(fb, j).astype(f32)
            return carry
        if fb0 < F_VPU:
            lax.fori_loop(fb0 // 2, min(fb1, F_VPU) // 2, vpu_blks, 0)

        for fb in range(max(fb0, F_VPU), min(fb1, NF - 1)):
            for j in range(NJ):
                gub[z0 + 2 * (fb - F_VPU) + mat, pl.ds(j * 64, 64), :] = _u32(tile(fb, j))
        if fb0 <= NF - 1 < fb1:
            for j in range(NJ):
                t = raw[pl.ds((NF - 1) * 128, 64), pl.ds(j * 128, 128)]
                t = jnp.concatenate([t, jnp.zeros((64, 128), bf16)], axis=0).T
                gub[z0 + 2 * (NF - 1 - F_VPU) + mat, pl.ds(j * 64, 64), :] = _u32(t)

    def prep_late_wd():
        for b, fb in enumerate(LATE):
            cps[f"wdL{fb}"].wait()
            r = LR[b]
            acc = None
            for j in range(NJ):
                tb = wd_v[pl.ds(fb * 128, r), pl.ds(j * 128, 128)]
                w = _u32(tb)
                if r < 128:
                    tb = jnp.concatenate([tb, jnp.zeros((128 - r, 128), bf16)], axis=0)
                wdb[z0 + fb * NJ + j] = _u32(tb)
                t = jnp.concatenate([_lo(w), _hi(w)], axis=0)
                wdf[j, pl.ds(LO[b], r), :] = t
                wdp[j, pl.ds(LO[b] // 2, r // 2), :] = _u32(t.astype(bf16))
                rsum = jnp.sum(t, axis=-1, keepdims=True)
                acc = rsum if acc is None else acc + rsum
            rm_v[pl.ds(LO[b], r), :] = jnp.broadcast_to(acc * (1.0 / M), (r, 128))

    def z_head(h):
        cs = cs_v[pl.ds(h, 1), :]
        z = None
        for j in range(NJ):
            y = _dot(_bf16(wdp[j]), _bf16(wqb[h, pl.ds(j * 64, 64), :]))
            z = y if z is None else z + y
        zf[h] = z - rm_v[...] * cs

    def prep_z(h0, h1):
        if h0 < h1:
            lax.fori_loop(h0, h1, lambda h, c: (z_head(h), c)[1], 0)

    def prep_wo(h0, h1):
        def vpu_head(h, carry):
            for j in range(NJ):
                t = wo_v[pl.ds(pl.multiple_of(h * 128, 128), 128), pl.ds(j * 128, 128)]
                wof[h * NJ + j] = t.astype(f32)
            return carry

        def mxu_head(h, carry):
            for j in range(NJ):
                t = wo_v[pl.ds(pl.multiple_of(h * 128, 128), 128), pl.ds(j * 128, 128)]
                wob[(h - O_VPU) * NJ + j] = _u32(t)
            return carry
        if h0 < O_VPU:
            lax.fori_loop(h0, min(h1, O_VPU), vpu_head, 0)
        if h1 > O_VPU:
            lax.fori_loop(max(h0, O_VPU), h1, mxu_head, 0)

    def stage_xt(x, mean):
        for kb in range(NJ):
            t = _xpose_bcast(x[0:1, kb * 128:(kb + 1) * 128])
            xts[kb][pl.ds(0, 128), :] = t - mean[0:1, 0:1]

    def vpu_cols(wref, idxs, static, prev, rows=M, post=False, joint=False):
        accs = [None] * len(idxs)
        if not static:
            zf = next(zi)
            for kb in range((rows + 127) // 128):
                xts[kb][pl.ds(zf + 128, 8), :] = pltpu.bitcast(zvec, f32)
        for i in range(rows // 8):
            xt = xts[i // 16][pl.ds(8 * (i % 16), 8), :]
            for n, c in enumerate(idxs):
                p = xt * wref[c, pl.ds(8 * i, 8), :]
                if accs[n] is None:
                    if prev:
                        p = jnp.where(zmask, prev[n % len(prev)], p)
                    accs[n] = p
                else:
                    accs[n] = accs[n] + p
        if joint:
            prev[:] = accs
            return _rowsum4(accs)
        ys = [_rowsum(a) for a in accs]
        prev[:] = ys if post else accs
        return ys

    def region(fn, first, zero, tag):
        if tag not in (REG1 if first else REG2):
            return fn()
        return lax.cond(z0 == 0, fn, lambda: zero)

    def phase_a(x, xb, mean, rstd):
        stage_xt(x, mean)
        qabs = [[None] * NC for _ in range(4)]

        def absorb(h, qh):
            qb = qh.astype(bf16)
            for cb in range(NC):
                y = _dot(qb, _bf16(ukb[h, pl.ds(cb * 64, 64), :]))
                old = qabs[h // 8][cb]
                qabs[h // 8][cb] = y if old is None else jnp.where(sub == h % 8, y, old)

        qm = [_dot(xb, _bf16(wqb[h])) for h in range(Q_MXU)]
        for h in range(Q_MXU):
            absorb(h, qm[h])
        h0 = 0
        prev = []
        for gsz in Q_GROUPS:
            qs = vpu_cols(wqf, list(range(h0, h0 + gsz)), h0 == 0, prev)
            for n in range(gsz):
                absorb(Q_MXU + h0 + n, qs[n])
            h0 += gsz
        scale = rstd[0:1, 0:1] * ((D ** -0.5) * LOG2E)
        qa = jnp.concatenate([jnp.concatenate(qabs[g], axis=1) for g in range(4)], axis=0)
        return (qa * scale).astype(bf16)

    def phase_b(qa, ycalc=None, lazy=False):
        sc = None
        side = {}
        def scores(k0, k1):
            mrun = None
            for kb in range(k0, k1):
                s = _dot(qa, _bf16(cT[kb]))
                s_v[kb] = s
                if ycalc is not None and kb == TIE_KB:
                    side['sc'] = ycalc(s[0:8, :])
                if ycalc is not None and kb == TIE_KB2:
                    ycalc.late(s[0:8, :])
                mrun = s if mrun is None else jnp.maximum(mrun, s)
            return jnp.max(mrun, axis=-1, keepdims=True)

        def weighted(k0, k1, mrow):
            lsum = None
            cacc = [None] * NC
            for kb in range(k0, k1):
                p = jnp.exp2(s_v[kb] - mrow if sc is None else (s_v[kb] - mrow) * sc)
                lsum = p if lsum is None else lsum + p
                pb = p.astype(bf16)
                for cb in range(NC):
                    y = _dot(pb, _bf16(c2[cb, pl.ds(kb * 64, 64), :]))
                    cacc[cb] = y if cacc[cb] is None else cacc[cb] + y
            return jnp.sum(lsum, axis=-1, keepdims=True), cacc

        hk = NK // 2
        ma = scores(0, hk)
        mb = scores(hk, NK)
        sc = side.get('sc')
        la, ca = weighted(0, hk, ma)
        lb, cb_ = weighted(hk, NK, mb)
        m = jnp.maximum(ma, mb)
        fa = jnp.exp2(ma - m if sc is None else (ma - m) * sc)
        fb = jnp.exp2(mb - m if sc is None else (mb - m) * sc)
        linv = 1.0 / (la * fa + lb * fb)
        wa = fa * linv
        wb = fb * linv
        def merged():
            return jnp.concatenate([(ca[c] * wa + cb_[c] * wb).astype(bf16) for c in range(NC)], axis=1)
        return merged if lazy else merged()

    def phase_c(cx):
        vacc = [None] * NJ
        macc = [None] * NJ
        ys = {}
        la = C_LA
        for i in range(H + la):
            if i < H:
                g = i // 8
                ys[i] = _dot(cx[8 * g:8 * g + 8, :], _bf16(uvb[i]))
            h = i - la
            if 0 <= h < O_VPU:
                xt = _xpose_bcast(ys[h][h % 8:h % 8 + 1, :])
                if C_LK is None:
                    for ii in range(D // 8):
                        for j in range(NJ):
                            p = xt[8 * ii:8 * ii + 8, :] * wof[h * NJ + j, pl.ds(8 * ii, 8), :]
                            vacc[j] = p if vacc[j] is None else vacc[j] + p
                else:
                    tie = None
                    for j in range(NJ):
                        for ii in range(D // 8):
                            p = xt[8 * ii:8 * ii + 8, :] * wof[h * NJ + j, pl.ds(8 * ii, 8), :]
                            if j == 0 and ii == 0 and h > 0:
                                p = jnp.where(zmask, vacc[NJ - 1], p)
                            if j == NJ - 1 and ii == 0:
                                p = jnp.where(zmask, tie, p)
                            vacc[j] = p if vacc[j] is None else vacc[j] + p
                            if j == 0 and ii == C_LK:
                                tie = vacc[0]
        for h in range(O_VPU, H):
            lhs = jnp.broadcast_to(ys[h][h % 8:h % 8 + 1, :], (8, 128)).astype(bf16)
            for j in range(NJ):
                yy = _dot(lhs, _bf16(wob[(h - O_VPU) * NJ + j]))
                macc[j] = yy if macc[j] is None else macc[j] + yy
        return jnp.concatenate([_rowsum(vacc[j]) + macc[j] for j in range(NJ)], axis=1)

    def swiglu(x, xb, mean, rstd, on_block, skip=(), post=None, row0_only=False):
        stage_xt(x, mean)

        def act(g, u):
            if FAST_ACT:
                return _swiglu(g, u, rstd, post).astype(bf16)
            return (jax.nn.silu(g * rstd) * (u * rstd)).astype(bf16)

        for i in range(NF - F_VPU):
            if F_VPU + i in skip:
                continue
            on_block(F_VPU + i, act(_dot(xb, _bf16(gub[2 * i])), _dot(xb, _bf16(gub[2 * i + 1]))), 0)
        on_block(None, None, 0)
        f0 = 0
        prev = []
        for gsz in F_GROUPS:
            if row0_only and gsz == 2 and D_JOINT:
                r = vpu_cols(guf, [2 * f0, 2 * f0 + 2, 2 * f0 + 1, 2 * f0 + 3], f0 == 0, prev, joint=True)
                hh = _swiglu(r, pltpu.roll(r, 6, 0), rstd, post)
                on_block(f0, hh.astype(bf16), 1)
                on_block(f0 + 1, pltpu.roll(hh, 7, 0).astype(bf16), 1)
                f0 += gsz
                continue
            ys = vpu_cols(guf, list(range(2 * f0, 2 * (f0 + gsz))), f0 == 0, prev)
            for n in range(gsz):
                on_block(f0 + n, act(ys[2 * n], ys[2 * n + 1]), 1)
            f0 += gsz

    def phase_d1(x, xb, mean, rstd):
        hs = {}

        def keep(fb, h, kind):
            if fb is not None:
                hs[fb] = h
        swiglu(x, xb, mean, rstd, keep, skip=LATE)
        return tuple(hs[fb] for fb in EARLY)

    def phase_d2(x, xb, mean, rstd, rs):
        yacc = [None] * NJ
        held = []

        def down(fb, hb):
            for j in range(NJ):
                yy = _dot(hb, _bf16(wdb[fb * NJ + j]))
                yacc[j] = yy if yacc[j] is None else yacc[j] + yy

        def on_block(fb, h, kind):
            if fb is None:
                for b, hb in held:
                    down(b, hb)
            elif kind == 0:
                held.append((fb, h))
            else:
                down(fb, h)
        swiglu(x, xb, mean, rstd, on_block, post=rs if FOLD_D else None, row0_only=True)
        return jnp.concatenate(yacc, axis=1)

    def phase_a_early(v):
        vb = v.astype(bf16)
        for kb in range(NJ):
            xts[kb][pl.ds(0, 128), :] = _xpose_bcast(v[0:1, kb * 128:(kb + 1) * 128])
        delta = jnp.sum(vb.astype(f32), axis=-1, keepdims=True) * (1.0 / M)
        q = [None] * 4

        def put(h, y):
            q[h // 8] = y if q[h // 8] is None else jnp.where(sub == h % 8, y, q[h // 8])

        for h in range(AE_LATE, AE_MXU):
            put(h, _dot(vb, _bf16(wqb[h])))
        h0 = AE_MXU
        prev = []
        for gsz in AE_GROUPS:
            ys = vpu_cols(wqf, list(range(h0 - Q_MXU, h0 - Q_MXU + gsz)), h0 == AE_MXU, prev, post=AE_POST)
            for n in range(gsz):
                put(h0 + n, ys[n])
            h0 += gsz
        for g in range(4):
            if q[g] is None:
                q[g] = jnp.zeros((8, 128), f32)
        return tuple(q[g] - delta * cs_v[pl.ds(8 * g, 8), :] for g in range(4)) + (vb,)

    def late_hidden(xb, rstd, rs):
        xf = xb.astype(f32)
        for b in range(NL):
            r = LR[b]
            gu = []
            for m in range(2):
                lo, hi = None, None
                for j in range(NJ):
                    w = gul[2 * b + m, pl.ds(0, r // 2), pl.ds(j * 128, 128)]
                    xj = xf[0:1, j * 128:(j + 1) * 128]
                    pl_, ph_ = _lo(w) * xj, _hi(w) * xj
                    lo = pl_ if lo is None else lo + pl_
                    hi = ph_ if hi is None else hi + ph_
                s_ = jnp.sum(jnp.concatenate([lo, hi], axis=0), axis=-1, keepdims=True)
                gu.append(jnp.broadcast_to(s_, (r, 128)))
            xts[b][pl.ds(0, r), :] = _swiglu(gu[0], gu[1], rstd[0:1, 0:1], rs[0:1, 0:1] if FOLD_RS else None)

    def phase_a2(qbase, rs, vb):
        qabs = [[None] * NC for _ in range(4)]

        def put(h, cb, y):
            old = qabs[h // 8][cb]
            qabs[h // 8][cb] = y if old is None else jnp.where(sub == h % 8, y, old)

        late = {h: _dot(vb, _bf16(wqb[h])) for h in range(AE_LATE)}

        def base(h):
            b = _rowsum(jnp.where(sub == h % 8, qbase[h // 8], 0.0))
            return b + late[h] if h < AE_LATE else b

        def absorb_mxu(h, qh):
            for cb in range(NC):
                put(h, cb, _dot(qh, _bf16(ukb[h, pl.ds(cb * 64, 64), :])))

        segs = []

        def absorb_vpu(h, qh):
            xq = _xpose_bcast(qh[0:1, :])
            for cb in range(NC):
                acc = None
                for i in range(16):
                    p = xq[8 * i:8 * i + 8] * ukf[(h - (H - K2_VPU)) * NC + cb, pl.ds(8 * i, 8), :]
                    if acc is None:
                        if len(segs) >= K2_LANES:
                            p = jnp.where(zmask, segs[len(segs) - K2_LANES], p)
                        acc = p
                    else:
                        acc = acc + p
                segs.append(acc)
                put(h, cb, _rowsum(acc))

        mh = list(range(AE_LATE, H - K2_VPU))
        mh = mh[:A2_LPOS] + list(range(AE_LATE)) + mh[A2_LPOS:]
        order = mh[:A2_KPOS] + list(range(H - K2_VPU, H)) + mh[A2_KPOS:]
        prev = []
        held = []
        pos = 0
        for gi, gsz in enumerate(A2_GROUPS):
            hh = order[pos:pos + gsz]
            assert gsz == 4 and hh == list(range(hh[0], hh[0] + 4)) and hh[0] % 4 == 0
            qg = vpu_cols(zf, hh, pos == 0, prev, rows=KL, joint=True)
            qg = (qg if FOLD_RS else qg * rs) + qbase[hh[0] // 8]
            if hh[0] < AE_LATE:
                for h in hh:
                    qg = qg + jnp.where(sub == h % 8, late[h], 0.0)
            if hh[0] >= H - K2_VPU:
                held += [(h, jnp.broadcast_to(qg[h % 8:h % 8 + 1, :], (8, 128))) for h in hh]
            else:
                qb = qg.astype(bf16)
                for h in hh:
                    absorb_mxu(h, qb)
            pos += gsz
        for h, qh in held:
            absorb_vpu(h, qh)
        qa = jnp.concatenate([jnp.concatenate(qabs[g], axis=1) for g in range(4)], axis=0)
        return qa.astype(bf16)

    def router(xn):
        r = jnp.sum(xn.astype(bf16).astype(f32) * wr, axis=-1, keepdims=True)
        return jax.nn.sigmoid(r)

    cps["x"].wait()
    cps["wr"].wait()
    x = jnp.broadcast_to(x_v[0].astype(f32), (8, M))
    wr = wr_v[...].astype(f32).reshape(1, M)

    xc, rstd, mean = _ln_parts(x)
    xb = xc.astype(bf16)
    prep_wq()
    prep_late_wd()
    prep_wuk()
    qa = region(lambda: phase_a(x, xb, mean, rstd), True, jnp.zeros((H, DC), bf16), 'A')
    prep_c()
    cx = region(lambda: phase_b(qa), True, jnp.zeros((H, DC), bf16), 'B')
    prep_wuv()
    for i, (s0, n0) in enumerate(WG_CHUNKS):
        cps[f"wg{i}"].wait()
        prep_gu(0, wg_v, s0, s0 + n0)
    zh = ZH_UK + ZH_UV
    zper = (H - zh + WO_CHUNKS - 2) // (WO_CHUNKS - 1)
    for i in range(WO_CHUNKS):
        cps[f"wo{i}"].wait()
        prep_wo(i * hpc, (i + 1) * hpc)
        prep_z(min(zh + i * zper, H), min(zh + (i + 1) * zper, H))
    x = x + region(lambda: phase_c(cx), True, jnp.zeros((8, M), f32), 'C')

    xc, rstd, mean = _ln_parts(x)
    xn = xc * rstd
    xb = xc.astype(bf16)
    rs = router(xn)
    for i, (s0, n0) in enumerate(WU_CHUNKS):
        cps[f"wu{i}"].wait()
        prep_gu(1, wu_v, s0, s0 + n0)
    hs_e = region(lambda: phase_d1(x, xb, mean, rstd), True,
                  tuple(jnp.zeros((8, 128), bf16) for _ in range(len(EARLY))), 'D')
    hs = dict(zip(EARLY, hs_e))
    u = x + (xn + xn * 0.0)
    yj = [None] * NJ

    def down1(fb, hb):
        for j in range(NJ):
            n = min(128, F - fb * 128)
            t = wd_v[pl.ds(fb * 128, n), pl.ds(j * 128, 128)]
            if n < 128:
                t = jnp.concatenate([t, jnp.zeros((128 - n, 128), bf16)], axis=0)
            wdb[z0 + fb * NJ + j] = _u32(t)
            yy = _dot(hb, t)
            yj[j] = yy if yj[j] is None else yj[j] + yy

    for i, (fb0, nb) in enumerate(WD_CHUNKS):
        cps[f"wd{i}"].wait()
        for fb in range(fb0, fb0 + nb):
            down1(fb, hs[fb])
    v = u + jnp.concatenate(yj, axis=1) * rs
    *qbase, vb = region(lambda: phase_a_early(v), True,
                        tuple(jnp.zeros((8, 128), f32) for _ in range(4)) + (jnp.zeros((8, M), bf16),), 'E')
    for fb in LATE:
        cps[f"wgL{fb}"].wait()
        cps[f"wuL{fb}"].wait()
    late_hidden(xb, rstd, rs)
    if True:
        qa = phase_a2(qbase, rs, vb)
        xs = {}

        def sc2(tie):
            ys, j0, pv = [], 0, [tie]
            for gsz in Y_GROUPS:
                ys += vpu_cols(wdf, list(range(j0, j0 + gsz)), False, pv, rows=KL)
                j0 += gsz
            yl = jnp.concatenate(ys, axis=1)
            xs['x'] = v + (yl if FOLD_RS else yl * rs)
            xc, rstd2, mean = _ln_parts(xs['x'])
            return rstd2[0:1, 0:1] * ((D ** -0.5) * LOG2E)

        def late_prep(tie):
            for b, fb in enumerate(LATE):
                for m in range(2):
                    for j in range(NJ):
                        t = _bf16(gul[2 * b + m, pl.ds(0, LR[b] // 2), pl.ds(j * 128, 128)])
                        if LR[b] < 128:
                            t = jnp.concatenate([t, jnp.zeros((128 - LR[b], 128), bf16)], axis=0)
                        gub[z0 + 2 * (fb - F_VPU) + m, pl.ds(j * 64, 64), :] = _u32(t.T)
        sc2.late = late_prep
    if MERGE_IN_C:
        cxf = phase_b(qa, sc2, True)
    else:
        cx = region(lambda: phase_b(qa, sc2), False, jnp.zeros((H, DC), bf16), 'B')
    if Y_VPU:
        x = xs['x']
    x = x + region(lambda: phase_c(cxf() if MERGE_IN_C else cx), False, jnp.zeros((8, M), f32), 'C')
    xc, rstd, mean = _ln_parts(x)
    xn = xc * rstd
    xb = xc.astype(bf16)
    rs = router(xn)
    y = region(lambda: phase_d2(x, xb, mean, rstd, rs), False, jnp.zeros((8, M), f32), 'D')
    x = (x + (xn + xn * 0.0)) + (y if FOLD_D else y * rs)

    o_v[0] = x[0:1, :].astype(bf16)
    ocp = pltpu.make_async_copy(o_v, o_hbm, sems.at[len(names)])
    ocp.start()
    ocp.wait()


@jax.jit
def pallas_interleave_layers__compressed_kv_cla__moe_arch_mod__decode_kernel(
    A_x, A_c_kv, A_w_q, A_w_uk, A_w_uv, A_w_o, B_x, B_w_r, B_w_gate, B_w_up, B_w_down,
):
    del B_x
    ins = [
        A_x, B_w_r, A_w_q, A_w_uk,
        A_c_kv.reshape(SK, DC),
        A_w_uv,
        A_w_o.reshape(H * D, M),
        B_w_gate.T, B_w_up.T,
        B_w_down,
    ]
    scratch = [
        pltpu.VMEM((1, 1, M), bf16),
        pltpu.VMEM((M,), bf16),
        pltpu.VMEM((H // 2, M, D), u32),
        pltpu.VMEM((H // 2, DC, D), u32),
        pltpu.VMEM((H // 2, DC, D), u32),
        pltpu.VMEM((H * D, M), bf16),
        pltpu.VMEM((F, M), bf16),
        pltpu.VMEM((F, M), bf16),
        pltpu.VMEM((F, M), bf16),
        pltpu.VMEM((H, M // 2, 128), u32),
        pltpu.VMEM((Q_VPU, M, 128), f32),
        pltpu.VMEM((H, NC * 64, 128), u32),
        pltpu.VMEM((K2_VPU * NC, 128, 128), f32),
        pltpu.VMEM((H, 128), f32),
        pltpu.VMEM((KL, 128), f32),
        pltpu.VMEM((NJ, KL, 128), f32),
        pltpu.VMEM((2 * NL, 64, M), u32),
        pltpu.VMEM((NJ, KL // 2, 128), u32),
        pltpu.VMEM((H, KL, 128), f32),
        pltpu.VMEM((NF * NJ, 64, 128), u32),
        pltpu.VMEM((NK, DC // 2, 128), u32),
        pltpu.VMEM((NC, SK // 2, 128), u32),
        pltpu.VMEM((H, DC // 2, 128), u32),
        pltpu.VMEM(((H - O_VPU) * NJ, 64, 128), u32),
        pltpu.VMEM((O_VPU * NJ, 128, 128), f32),
        pltpu.VMEM((2 * (NF - F_VPU), M // 2, 128), u32),
        pltpu.VMEM((2 * F_VPU, M, 128), f32),
        *[pltpu.VMEM((160, 128), f32) for _ in range(NJ)],
        pltpu.VMEM((NK, H, 128), f32),
        pltpu.VMEM((1, 1, M), bf16),
        pltpu.SemaphoreType.DMA((96,)),
        pltpu.SemaphoreType.REGULAR((NZ,)),
    ]
    return pl.pallas_call(
        _kernel,
        in_specs=[pl.BlockSpec(memory_space=pltpu.HBM)] * len(ins),
        out_specs=pl.BlockSpec(memory_space=pltpu.HBM),
        out_shape=jax.ShapeDtypeStruct((1, 1, M), bf16),
        scratch_shapes=scratch,
        compiler_params=pltpu.CompilerParams(
            vmem_limit_bytes=120 * 1024 * 1024,
            disable_semaphore_checks=True,
            disable_bounds_checks=True,
            flags={"XLA_TPU_FORCE_LP_LLO_SCHEDULER": True},
        ),
    )(*ins)
```

```python
import jax
import jax.numpy as jnp
from jax import lax
import jax.experimental.pallas as pl
import jax.experimental.pallas.tpu as pltpu

bf16 = jnp.bfloat16
f32 = jnp.float32
u32 = jnp.uint32
i32 = jnp.int32

M = 640
H = 32
D = 128
SK = 4096
DC = 512
F = 1728
NJ = M // 128
NC = DC // 128
NK = SK // 128
NF = (F + 127) // 128
LOG2E = 1.4426950408889634
EPS = 1e-5

REG1 = 'ABCD'
REG2 = 'C'

Q_MXU = 8
Q_GROUPS = [4, 4, 4, 4, 4, 4]
Q_VPU = H - Q_MXU
O_VPU = 21
O_LINK = 6
F_GROUPS = [2, 2, 2, 2]
F_VPU = sum(F_GROUPS)
E_LATE = 8
E_MXU = 24
E_GROUPS = [4, 4]
K2_VPU = 8
K2_LANES = 3
A2_ORDER = [8, 12, 24, 28, 16, 0, 4, 20]
A2_DELAY = 3
D2_DELAY = 5
TIE_Y = 2
TIE_PREP = 3
assert sum(Q_GROUPS) == Q_VPU and Q_MXU % 2 == 0 and F_VPU % 2 == 0 and K2_VPU % 2 == 0
assert sorted(A2_ORDER) == list(range(0, H, 4)) and E_LATE % 4 == 0 and K2_VPU % 4 == 0

WO_CHUNKS = 4
LATE = [12, 13]
WG_CHUNKS = [(0, 12)]
WU_CHUNKS = [(0, 4), (4, 4), (8, 4)]
WD_CHUNKS = [(0, 3), (3, 3), (6, 3), (9, 1), (10, 1), (11, 1)]
NL = len(LATE)
LR = [min(128, F - 128 * fb) for fb in LATE]
LO = [sum(LR[:b]) for b in range(NL)]
KL = sum(LR)
EARLY = [fb for fb in range(NF) if fb not in LATE]
assert all(r == 128 for r in LR[:-1]) and min(LATE) >= F_VPU and NL <= NJ
NZ = 32


def _dot(a, b):
    return jnp.dot(a, b, preferred_element_type=f32)


def _u32(a):
    return pltpu.bitcast(a, u32)


def _bf16(a):
    return pltpu.bitcast(a, bf16)


def _lo(w):
    return pltpu.bitcast(w << 16, f32)


def _hi(w):
    return pltpu.bitcast(w & jnp.uint32(0xFFFF0000), f32)


def _rowsum(acc):
    return jnp.broadcast_to(jnp.sum(acc, axis=0, keepdims=True), (8, 128))


def _rowsum4(a):
    sub = lax.broadcasted_iota(i32, (8, 128), 0)
    m1 = (sub & 1) == 0
    m2 = (sub & 2) == 0
    s01 = jnp.where(m1, a[0], a[1]) + pltpu.roll(jnp.where(m1, a[1], a[0]), 7, 0)
    s23 = jnp.where(m1, a[2], a[3]) + pltpu.roll(jnp.where(m1, a[3], a[2]), 7, 0)
    s = jnp.where(m2, s01, s23) + pltpu.roll(jnp.where(m2, s23, s01), 6, 0)
    return s + pltpu.roll(s, 4, 0)


def _ln_parts(x):
    m = jnp.sum(x, axis=-1, keepdims=True) * (1.0 / M)
    m2 = jnp.sum(x * x, axis=-1, keepdims=True) * (1.0 / M)
    v = jnp.maximum(m2 - m * m, 0.0)
    return x - m, lax.rsqrt(v + EPS), m


def _xpose_bcast(row):
    r16 = jnp.broadcast_to(row, (16, 128)).astype(bf16)
    return jnp.concatenate([r16] * 8, axis=0).T.astype(f32)


def _swiglu(g, u, rstd, post=None):
    e = jnp.exp2(g * (rstd * -LOG2E))
    c = rstd * rstd if post is None else rstd * rstd * post
    return (g * u) * c * pl.reciprocal(1.0 + e, approx=True)


def _kernel(x_hbm, wr_hbm, wq_hbm, wuk_hbm, c_hbm, wuv_hbm, wo_hbm, wg_hbm, wu_hbm, wd_hbm,
            o_hbm,
            x_v, wr_v, wq_v, wuk_v, wuv_v, wo_v, wg_v, wu_v, wd_v,
            wqb, wqf, ukb, ukf, cs_v, rm_v, wdf, gul, wdp, zf, wdb, cT, c2, uvb, wob, wof, gub, guf,
            xt0, xt1, xt2, xt3, xt4, s_v, o_v, sems, zsem):
    cps = {}
    names = []
    families = {}

    def add(name, src, dst):
        cp = pltpu.make_async_copy(src, dst, sems.at[len(names)])
        cp.start()
        cps[name] = cp
        names.append(name)

    def add_pairs(name, src, dst):
        s32 = src.bitcast(u32)
        families[name] = (s32, dst, len(names))
        for hp in range(H // 2):
            add(f"{name}{hp}", s32.at[:, hp, :], dst.at[hp])

    def wait_pair(name, hp):
        src, dst, base = families[name]
        pltpu.make_async_copy(src.at[:, hp, :], dst.at[hp], sems.at[base + hp]).wait()

    add("x", x_hbm, x_v)
    add("wr", wr_hbm, wr_v)

    def add_blocks(name, src, dst, fb0, nb):
        rows = min(128 * nb, F - 128 * fb0)
        add(name, src.at[pl.ds(128 * fb0, rows)], dst.at[pl.ds(128 * fb0, rows)])

    add_pairs("wq", wq_hbm, wq_v)
    for fb in LATE:
        add_blocks(f"wdL{fb}", wd_hbm, wd_v, fb, 1)
    add_pairs("wuk", wuk_hbm, wuk_v)
    c32 = c_hbm.bitcast(u32)
    for cb in range(NC):
        add(f"c{cb}", c32.at[:, pl.ds(cb * 128, 128)], c2.at[cb])
    add_pairs("wuv", wuv_hbm, wuv_v)
    for i, (s, n) in enumerate(WG_CHUNKS):
        add_blocks(f"wg{i}", wg_hbm, wg_v, s, n)
    hpc = H // WO_CHUNKS
    for i in range(WO_CHUNKS):
        add(f"wo{i}", wo_hbm.at[pl.ds(i * hpc * D, hpc * D)], wo_v.at[pl.ds(i * hpc * D, hpc * D)])
    for i, (s, n) in enumerate(WU_CHUNKS):
        add_blocks(f"wu{i}", wu_hbm, wu_v, s, n)
    for i, (s, n) in enumerate(WD_CHUNKS):
        add_blocks(f"wd{i}", wd_hbm, wd_v, s, n)
    for b, fb in enumerate(LATE):
        n = LR[b] // 2
        add(f"wgL{fb}", wg_hbm.bitcast(u32).at[pl.ds(64 * fb, n)], gul.at[2 * b, pl.ds(0, n)])
        add(f"wuL{fb}", wu_hbm.bitcast(u32).at[pl.ds(64 * fb, n)], gul.at[2 * b + 1, pl.ds(0, n)])

    sub = lax.broadcasted_iota(i32, (8, 128), 0)
    xts = [xt0, xt1, xt2, xt3, xt4]
    zs = [pl.semaphore_read(zsem.at[n]) for n in range(NZ)]
    z0 = zs[0]
    zvec = jnp.zeros((8, 128), u32) + zs[-1].astype(u32)
    zmask = zvec != 0
    zi = iter(zs[1:-1])

    def repack(src, hp, dst, rows):
        for i in range(rows // 16):
            v = src[hp, pl.ds(16 * i, 16), :]
            dst[2 * hp, pl.ds(8 * i, 8), :] = _u32(_lo(v).astype(bf16))
            dst[2 * hp + 1, pl.ds(8 * i, 8), :] = _u32(_hi(v).astype(bf16))

    def prep_wq():
        def both(k, carry):
            hp = k + Q_MXU // 2
            wait_pair("wq", hp)
            repack(wq_v, hp, wqb, M)
            v = wq_v[hp]
            wqf[2 * k] = _lo(v)
            wqf[2 * k + 1] = _hi(v)
            return carry

        for hp in range(Q_MXU // 2):
            cps[f"wq{hp}"].wait()
            repack(wq_v, hp, wqb, M)
        lax.fori_loop(0, Q_VPU // 2, both, 0)
        ones = jnp.ones((8, M), bf16)

        def colsum(g, carry):
            acc = jnp.zeros((8, 128), f32)
            for r in range(8):
                acc = jnp.where(sub == r, _dot(ones, _bf16(wqb[8 * g + r])), acc)
            cs_v[pl.ds(pl.multiple_of(8 * g, 8), 8), :] = acc
            return carry
        lax.fori_loop(0, H // 8, colsum, 0)

    def prep_wuk():
        def pair_b(hp, carry):
            wait_pair("wuk", hp)
            for cb in range(NC):
                t = wuk_v[hp, pl.ds(cb * 128, 128), :].T
                ukb[2 * hp, pl.ds(cb * 64, 64), :] = _u32(_lo(t).astype(bf16))
                ukb[2 * hp + 1, pl.ds(cb * 64, 64), :] = _u32(_hi(t).astype(bf16))
            return carry

        def pair_bf(hp, carry):
            wait_pair("wuk", hp)
            for cb in range(NC):
                t = wuk_v[hp, pl.ds(cb * 128, 128), :].T
                lo, hi = _lo(t), _hi(t)
                ukf[(2 * hp - (H - K2_VPU)) * NC + cb] = lo
                ukf[(2 * hp + 1 - (H - K2_VPU)) * NC + cb] = hi
                ukb[2 * hp, pl.ds(cb * 64, 64), :] = _u32(lo.astype(bf16))
                ukb[2 * hp + 1, pl.ds(cb * 64, 64), :] = _u32(hi.astype(bf16))
            return carry

        def with_z(fn):
            def body(hp, carry):
                fn(hp, carry)
                z_head(hp)
                return carry
            return body
        lax.fori_loop(0, (H - K2_VPU) // 2, with_z(pair_b), 0)
        lax.fori_loop((H - K2_VPU) // 2, H // 2, with_z(pair_bf), 0)

    def prep_c():
        for cb in range(NC):
            cps[f"c{cb}"].wait()

            def blk(i, carry, cb=cb):
                for kk in range(16):
                    kb = 16 * i + kk
                    t = _bf16(c2[cb, pl.ds(pl.multiple_of(kb * 64, 64), 64), :])
                    cT[kb, pl.ds(cb * 64, 64), :] = _u32(t.T)
                return carry
            lax.fori_loop(0, NK // 16, blk, 0)

    def prep_wuv():
        def pair(hp, carry):
            z_head(hp + H // 2)
            wait_pair("wuv", hp)
            repack(wuv_v, hp, uvb, DC)
            return carry
        lax.fori_loop(0, H // 2, pair, 0)

    def prep_gu(mat, raw, fb0, fb1):
        def tile(fb, j):
            return raw[pl.ds(pl.multiple_of(fb * 128, 128), 128), pl.ds(j * 128, 128)].T

        def vpu_blks(i, carry):
            for fb in (2 * i, 2 * i + 1):
                for j in range(NJ):
                    guf[2 * fb + mat, pl.ds(j * 128, 128), :] = tile(fb, j).astype(f32)
            return carry
        if fb0 < F_VPU:
            lax.fori_loop(fb0 // 2, min(fb1, F_VPU) // 2, vpu_blks, 0)

        for fb in range(max(fb0, F_VPU), fb1):
            for j in range(NJ):
                gub[z0 + 2 * (fb - F_VPU) + mat, pl.ds(j * 64, 64), :] = _u32(tile(fb, j))

    def prep_late_wd():
        for b, fb in enumerate(LATE):
            cps[f"wdL{fb}"].wait()
            r = LR[b]
            acc = None
            for j in range(NJ):
                tb = wd_v[pl.ds(fb * 128, r), pl.ds(j * 128, 128)]
                w = _u32(tb)
                if r < 128:
                    tb = jnp.concatenate([tb, jnp.zeros((128 - r, 128), bf16)], axis=0)
                wdb[z0 + fb * NJ + j] = _u32(tb)
                t = jnp.concatenate([_lo(w), _hi(w)], axis=0)
                wdf[j, pl.ds(LO[b], r), :] = t
                wdp[j, pl.ds(LO[b] // 2, r // 2), :] = _u32(t.astype(bf16))
                rsum = jnp.sum(t, axis=-1, keepdims=True)
                acc = rsum if acc is None else acc + rsum
            rm_v[pl.ds(LO[b], r), :] = jnp.broadcast_to(acc * (1.0 / M), (r, 128))

    def z_head(h):
        cs = cs_v[pl.ds(h, 1), :]
        z = None
        for j in range(NJ):
            y = _dot(_bf16(wdp[j]), _bf16(wqb[h, pl.ds(j * 64, 64), :]))
            z = y if z is None else z + y
        zf[h] = z - rm_v[...] * cs

    def prep_wo(h0, h1):
        def vpu_head(h, carry):
            for j in range(NJ):
                t = wo_v[pl.ds(pl.multiple_of(h * 128, 128), 128), pl.ds(j * 128, 128)]
                wof[h * NJ + j] = t.astype(f32)
            return carry

        def mxu_head(h, carry):
            for j in range(NJ):
                t = wo_v[pl.ds(pl.multiple_of(h * 128, 128), 128), pl.ds(j * 128, 128)]
                wob[(h - O_VPU) * NJ + j] = _u32(t)
            return carry
        if h0 < O_VPU:
            lax.fori_loop(h0, min(h1, O_VPU), vpu_head, 0)
        if h1 > O_VPU:
            lax.fori_loop(max(h0, O_VPU), h1, mxu_head, 0)

    def stage_xt(x, mean):
        for kb in range(NJ):
            t = _xpose_bcast(x[0:1, kb * 128:(kb + 1) * 128])
            xts[kb][pl.ds(0, 128), :] = t - mean[0:1, 0:1]

    def vpu_cols(wref, idxs, static, prev, rows=M, joint=False, delay=0):
        accs = [None] * len(idxs)
        if prev and delay:
            t = prev[-1]
            for _ in range(delay):
                t = t + pltpu.bitcast(zvec, f32)
            prev[:] = [t]
        if not static:
            zf = next(zi)
            for kb in range((rows + 127) // 128):
                xts[kb][pl.ds(zf + 128, 8), :] = pltpu.bitcast(zvec, f32)
        for i in range(rows // 8):
            xt = xts[i // 16][pl.ds(8 * (i % 16), 8), :]
            for n, c in enumerate(idxs):
                p = xt * wref[c, pl.ds(8 * i, 8), :]
                if accs[n] is None:
                    if prev:
                        p = jnp.where(zmask, prev[n % len(prev)], p)
                    accs[n] = p
                else:
                    accs[n] = accs[n] + p
        if joint:
            prev[:] = accs
            return _rowsum4(accs)
        prev[:] = accs
        return [_rowsum(a) for a in accs]

    def region(fn, first, zero, tag):
        if tag not in (REG1 if first else REG2):
            return fn()
        return lax.cond(z0 == 0, fn, lambda: zero)

    def phase_a(x, xb, mean, rstd):
        stage_xt(x, mean)
        qabs = [[None] * NC for _ in range(4)]

        def absorb(h, qh):
            qb = qh.astype(bf16)
            for cb in range(NC):
                y = _dot(qb, _bf16(ukb[h, pl.ds(cb * 64, 64), :]))
                old = qabs[h // 8][cb]
                qabs[h // 8][cb] = y if old is None else jnp.where(sub == h % 8, y, old)

        qm = [_dot(xb, _bf16(wqb[h])) for h in range(Q_MXU)]
        for h in range(Q_MXU):
            absorb(h, qm[h])
        h0 = 0
        prev = []
        for gsz in Q_GROUPS:
            qs = vpu_cols(wqf, list(range(h0, h0 + gsz)), h0 == 0, prev)
            for n in range(gsz):
                absorb(Q_MXU + h0 + n, qs[n])
            h0 += gsz
        scale = rstd[0:1, 0:1] * ((D ** -0.5) * LOG2E)
        qa = jnp.concatenate([jnp.concatenate(qabs[g], axis=1) for g in range(4)], axis=0)
        return (qa * scale).astype(bf16)

    def phase_b(qa, scale_fn=None, side_fn=None):
        sc = None
        side = {}
        def scores(k0, k1):
            mrun = None
            for kb in range(k0, k1):
                s = _dot(qa, _bf16(cT[kb]))
                s_v[kb] = s
                if scale_fn is not None and kb == TIE_Y:
                    side['sc'] = scale_fn(s[0:8, :])
                if side_fn is not None and kb == TIE_PREP:
                    side_fn()
                mrun = s if mrun is None else jnp.maximum(mrun, s)
            return jnp.max(mrun, axis=-1, keepdims=True)

        def weighted(k0, k1, mrow):
            lsum = None
            cacc = [None] * NC
            for kb in range(k0, k1):
                p = jnp.exp2(s_v[kb] - mrow if sc is None else (s_v[kb] - mrow) * sc)
                lsum = p if lsum is None else lsum + p
                pb = p.astype(bf16)
                for cb in range(NC):
                    y = _dot(pb, _bf16(c2[cb, pl.ds(kb * 64, 64), :]))
                    cacc[cb] = y if cacc[cb] is None else cacc[cb] + y
            return jnp.sum(lsum, axis=-1, keepdims=True), cacc

        hk = NK // 2
        ma = scores(0, hk)
        mb = scores(hk, NK)
        sc = side.get('sc')
        la, ca = weighted(0, hk, ma)
        lb, cb_ = weighted(hk, NK, mb)
        m = jnp.maximum(ma, mb)
        fa = jnp.exp2(ma - m if sc is None else (ma - m) * sc)
        fb = jnp.exp2(mb - m if sc is None else (mb - m) * sc)
        linv = 1.0 / (la * fa + lb * fb)
        wa = fa * linv
        wb = fb * linv
        return jnp.concatenate([(ca[c] * wa + cb_[c] * wb).astype(bf16) for c in range(NC)], axis=1)

    def phase_c(cx):
        vacc = [None] * NJ
        macc = [None] * NJ
        ys = {}
        la = 4
        for i in range(H + la):
            if i < H:
                g = i // 8
                ys[i] = _dot(cx[8 * g:8 * g + 8, :], _bf16(uvb[i]))
            h = i - la
            if 0 <= h < O_VPU:
                xt = _xpose_bcast(ys[h][h % 8:h % 8 + 1, :])
                tie = None
                for j in range(NJ):
                    for ii in range(D // 8):
                        p = xt[8 * ii:8 * ii + 8, :] * wof[h * NJ + j, pl.ds(8 * ii, 8), :]
                        if j == 0 and ii == 0 and h > 0:
                            p = jnp.where(zmask, vacc[NJ - 1], p)
                        if j == NJ - 1 and ii == 0:
                            p = jnp.where(zmask, tie, p)
                        vacc[j] = p if vacc[j] is None else vacc[j] + p
                        if j == 0 and ii == O_LINK:
                            tie = vacc[0]
        for h in range(O_VPU, H):
            lhs = jnp.broadcast_to(ys[h][h % 8:h % 8 + 1, :], (8, 128)).astype(bf16)
            for j in range(NJ):
                yy = _dot(lhs, _bf16(wob[(h - O_VPU) * NJ + j]))
                macc[j] = yy if macc[j] is None else macc[j] + yy
        return jnp.concatenate([_rowsum(vacc[j]) + macc[j] for j in range(NJ)], axis=1)

    def swiglu(x, xb, mean, rstd, on_block, skip=(), rs=None):
        stage_xt(x, mean)

        post = None if rs is None else rs

        def act(g, u):
            return _swiglu(g, u, rstd, post).astype(bf16)

        for i in range(NF - F_VPU):
            if F_VPU + i in skip:
                continue
            on_block(F_VPU + i, act(_dot(xb, _bf16(gub[2 * i])), _dot(xb, _bf16(gub[2 * i + 1]))), 0)
        on_block(None, None, 0)
        f0 = 0
        prev = []
        for gsz in F_GROUPS:
            if rs is not None and gsz == 2:
                r = vpu_cols(guf, [2 * f0, 2 * f0 + 2, 2 * f0 + 1, 2 * f0 + 3], f0 == 0, prev, joint=True, delay=D2_DELAY)
                hh = _swiglu(r, pltpu.roll(r, 6, 0), rstd, post)
                on_block(f0, hh.astype(bf16), 1)
                on_block(f0 + 1, pltpu.roll(hh, 7, 0).astype(bf16), 1)
                f0 += gsz
                continue
            ys = vpu_cols(guf, list(range(2 * f0, 2 * (f0 + gsz))), f0 == 0, prev)
            for n in range(gsz):
                on_block(f0 + n, act(ys[2 * n], ys[2 * n + 1]), 1)
            f0 += gsz

    def phase_d1(x, xb, mean, rstd):
        hs = {}

        def keep(fb, h, kind):
            if fb is not None:
                hs[fb] = h
        swiglu(x, xb, mean, rstd, keep, skip=LATE)
        return tuple(hs[fb] for fb in EARLY)

    def phase_d2(x, xb, mean, rstd, rs):
        yacc = [None] * NJ
        held = []

        def down(fb, hb):
            for j in range(NJ):
                yy = _dot(hb, _bf16(wdb[fb * NJ + j]))
                yacc[j] = yy if yacc[j] is None else yacc[j] + yy

        def on_block(fb, h, kind):
            if fb is None:
                for b, hb in held:
                    down(b, hb)
            elif kind == 0:
                held.append((fb, h))
            else:
                down(fb, h)
        swiglu(x, xb, mean, rstd, on_block, rs=rs)
        return jnp.concatenate(yacc, axis=1)

    def phase_a_early(v):
        vb = v.astype(bf16)
        for kb in range(NJ):
            xts[kb][pl.ds(0, 128), :] = _xpose_bcast(v[0:1, kb * 128:(kb + 1) * 128])
        delta = jnp.sum(vb.astype(f32), axis=-1, keepdims=True) * (1.0 / M)
        q = [None] * 4

        def put(h, y):
            q[h // 8] = y if q[h // 8] is None else jnp.where(sub == h % 8, y, q[h // 8])

        for h in range(E_LATE, E_MXU):
            put(h, _dot(vb, _bf16(wqb[h])))
        h0 = E_MXU
        prev = []
        for gsz in E_GROUPS:
            ys = vpu_cols(wqf, list(range(h0 - Q_MXU, h0 - Q_MXU + gsz)), h0 == E_MXU, prev)
            for n in range(gsz):
                put(h0 + n, ys[n])
            h0 += gsz
        for g in range(4):
            if q[g] is None:
                q[g] = jnp.zeros((8, 128), f32)
        return tuple(q[g] - delta * cs_v[pl.ds(8 * g, 8), :] for g in range(4)) + (vb,)

    def late_hidden(xb, rstd, rs):
        xf = xb.astype(f32)
        for b in range(NL):
            r = LR[b]
            gu = []
            for m in range(2):
                lo, hi = None, None
                for j in range(NJ):
                    w = gul[2 * b + m, pl.ds(0, r // 2), pl.ds(j * 128, 128)]
                    xj = xf[0:1, j * 128:(j + 1) * 128]
                    pl_, ph_ = _lo(w) * xj, _hi(w) * xj
                    lo = pl_ if lo is None else lo + pl_
                    hi = ph_ if hi is None else hi + ph_
                s_ = jnp.sum(jnp.concatenate([lo, hi], axis=0), axis=-1, keepdims=True)
                gu.append(jnp.broadcast_to(s_, (r, 128)))
            xts[b][pl.ds(0, r), :] = _swiglu(gu[0], gu[1], rstd[0:1, 0:1], rs[0:1, 0:1])

    def phase_a2(qbase, vb):
        qabs = [[None] * NC for _ in range(4)]

        def put(h, cb, y):
            old = qabs[h // 8][cb]
            qabs[h // 8][cb] = y if old is None else jnp.where(sub == h % 8, y, old)

        late = {h: _dot(vb, _bf16(wqb[h])) for h in range(E_LATE)}

        def absorb_mxu(h, qh):
            for cb in range(NC):
                put(h, cb, _dot(qh, _bf16(ukb[h, pl.ds(cb * 64, 64), :])))

        segs = []

        def absorb_vpu(h, qh):
            xq = _xpose_bcast(qh[0:1, :])
            for cb in range(NC):
                acc = None
                for i in range(16):
                    p = xq[8 * i:8 * i + 8] * ukf[(h - (H - K2_VPU)) * NC + cb, pl.ds(8 * i, 8), :]
                    if acc is None:
                        if len(segs) >= K2_LANES:
                            p = jnp.where(zmask, segs[len(segs) - K2_LANES], p)
                        acc = p
                    else:
                        acc = acc + p
                segs.append(acc)
                put(h, cb, _rowsum(acc))

        prev = []
        held = []
        for pos, h0 in enumerate(A2_ORDER):
            hh = list(range(h0, h0 + 4))
            qg = vpu_cols(zf, hh, pos == 0, prev, rows=KL, joint=True, delay=A2_DELAY) + qbase[h0 // 8]
            if h0 < E_LATE:
                for h in hh:
                    qg = qg + jnp.where(sub == h % 8, late[h], 0.0)
            if h0 >= H - K2_VPU:
                held += [(h, jnp.broadcast_to(qg[h % 8:h % 8 + 1, :], (8, 128))) for h in hh]
            else:
                qb = qg.astype(bf16)
                for h in hh:
                    absorb_mxu(h, qb)
        for h, qh in held:
            absorb_vpu(h, qh)
        qa = jnp.concatenate([jnp.concatenate(qabs[g], axis=1) for g in range(4)], axis=0)
        return qa.astype(bf16)

    def router(xn):
        r = jnp.sum(xn.astype(bf16).astype(f32) * wr, axis=-1, keepdims=True)
        return jax.nn.sigmoid(r)

    cps["x"].wait()
    cps["wr"].wait()
    x = jnp.broadcast_to(x_v[0].astype(f32), (8, M))
    wr = wr_v[...].astype(f32).reshape(1, M)

    xc, rstd, mean = _ln_parts(x)
    xb = xc.astype(bf16)
    prep_wq()
    prep_late_wd()
    prep_wuk()
    qa = region(lambda: phase_a(x, xb, mean, rstd), True, jnp.zeros((H, DC), bf16), 'A')
    prep_c()
    cx = region(lambda: phase_b(qa), True, jnp.zeros((H, DC), bf16), 'B')
    prep_wuv()
    for i, (s0, n0) in enumerate(WG_CHUNKS):
        cps[f"wg{i}"].wait()
        prep_gu(0, wg_v, s0, s0 + n0)
    for i in range(WO_CHUNKS):
        cps[f"wo{i}"].wait()
        prep_wo(i * hpc, (i + 1) * hpc)
    x = x + region(lambda: phase_c(cx), True, jnp.zeros((8, M), f32), 'C')

    xc, rstd, mean = _ln_parts(x)
    xn = xc * rstd
    xb = xc.astype(bf16)
    rs = router(xn)
    for i, (s0, n0) in enumerate(WU_CHUNKS):
        cps[f"wu{i}"].wait()
        prep_gu(1, wu_v, s0, s0 + n0)
    hs_e = region(lambda: phase_d1(x, xb, mean, rstd), True,
                  tuple(jnp.zeros((8, 128), bf16) for _ in range(len(EARLY))), 'D')
    hs = dict(zip(EARLY, hs_e))
    u = x + (xn + xn * 0.0)
    yj = [None] * NJ

    def down1(fb, hb):
        for j in range(NJ):
            n = min(128, F - fb * 128)
            t = wd_v[pl.ds(fb * 128, n), pl.ds(j * 128, 128)]
            if n < 128:
                t = jnp.concatenate([t, jnp.zeros((128 - n, 128), bf16)], axis=0)
            wdb[z0 + fb * NJ + j] = _u32(t)
            yy = _dot(hb, t)
            yj[j] = yy if yj[j] is None else yj[j] + yy

    for i, (fb0, nb) in enumerate(WD_CHUNKS):
        cps[f"wd{i}"].wait()
        for fb in range(fb0, fb0 + nb):
            down1(fb, hs[fb])
    v = u + jnp.concatenate(yj, axis=1) * rs
    *qbase, vb = region(lambda: phase_a_early(v), True,
                        tuple(jnp.zeros((8, 128), f32) for _ in range(4)) + (jnp.zeros((8, M), bf16),), 'E')
    for fb in LATE:
        cps[f"wgL{fb}"].wait()
        cps[f"wuL{fb}"].wait()
    late_hidden(xb, rstd, rs)
    qa = phase_a2(qbase, vb)
    carried = {}

    def finish_layer1(tie):
        yl = vpu_cols(wdf, list(range(NJ)), False, [tie], rows=KL)
        carried['x'] = v + jnp.concatenate(yl, axis=1)
        _, rstd2, _ = _ln_parts(carried['x'])
        return rstd2[0:1, 0:1] * ((D ** -0.5) * LOG2E)

    def prep_late_gu():
        for b, fb in enumerate(LATE):
            for m in range(2):
                for j in range(NJ):
                    t = _bf16(gul[2 * b + m, pl.ds(0, LR[b] // 2), pl.ds(j * 128, 128)])
                    if LR[b] < 128:
                        t = jnp.concatenate([t, jnp.zeros((128 - LR[b], 128), bf16)], axis=0)
                    gub[z0 + 2 * (fb - F_VPU) + m, pl.ds(j * 64, 64), :] = _u32(t.T)

    cx = region(lambda: phase_b(qa, finish_layer1, prep_late_gu), False, jnp.zeros((H, DC), bf16), 'B')
    x = carried['x']
    x = x + region(lambda: phase_c(cx), False, jnp.zeros((8, M), f32), 'C')
    xc, rstd, mean = _ln_parts(x)
    xn = xc * rstd
    xb = xc.astype(bf16)
    rs = router(xn)
    y = region(lambda: phase_d2(x, xb, mean, rstd, rs), False, jnp.zeros((8, M), f32), 'D')
    x = (x + (xn + xn * 0.0)) + y

    o_v[0] = x[0:1, :].astype(bf16)
    ocp = pltpu.make_async_copy(o_v, o_hbm, sems.at[len(names)])
    ocp.start()
    ocp.wait()


@jax.jit
def pallas_interleave_layers__compressed_kv_cla__moe_arch_mod__decode_kernel(
    A_x, A_c_kv, A_w_q, A_w_uk, A_w_uv, A_w_o, B_x, B_w_r, B_w_gate, B_w_up, B_w_down,
):
    del B_x
    ins = [
        A_x, B_w_r, A_w_q, A_w_uk,
        A_c_kv.reshape(SK, DC),
        A_w_uv,
        A_w_o.reshape(H * D, M),
        B_w_gate.T, B_w_up.T,
        B_w_down,
    ]
    scratch = [
        pltpu.VMEM((1, 1, M), bf16),
        pltpu.VMEM((M,), bf16),
        pltpu.VMEM((H // 2, M, D), u32),
        pltpu.VMEM((H // 2, DC, D), u32),
        pltpu.VMEM((H // 2, DC, D), u32),
        pltpu.VMEM((H * D, M), bf16),
        pltpu.VMEM((F, M), bf16),
        pltpu.VMEM((F, M), bf16),
        pltpu.VMEM((F, M), bf16),
        pltpu.VMEM((H, M // 2, 128), u32),
        pltpu.VMEM((Q_VPU, M, 128), f32),
        pltpu.VMEM((H, NC * 64, 128), u32),
        pltpu.VMEM((K2_VPU * NC, 128, 128), f32),
        pltpu.VMEM((H, 128), f32),
        pltpu.VMEM((KL, 128), f32),
        pltpu.VMEM((NJ, KL, 128), f32),
        pltpu.VMEM((2 * NL, 64, M), u32),
        pltpu.VMEM((NJ, KL // 2, 128), u32),
        pltpu.VMEM((H, KL, 128), f32),
        pltpu.VMEM((NF * NJ, 64, 128), u32),
        pltpu.VMEM((NK, DC // 2, 128), u32),
        pltpu.VMEM((NC, SK // 2, 128), u32),
        pltpu.VMEM((H, DC // 2, 128), u32),
        pltpu.VMEM(((H - O_VPU) * NJ, 64, 128), u32),
        pltpu.VMEM((O_VPU * NJ, 128, 128), f32),
        pltpu.VMEM((2 * (NF - F_VPU), M // 2, 128), u32),
        pltpu.VMEM((2 * F_VPU, M, 128), f32),
        *[pltpu.VMEM((160, 128), f32) for _ in range(NJ)],
        pltpu.VMEM((NK, H, 128), f32),
        pltpu.VMEM((1, 1, M), bf16),
        pltpu.SemaphoreType.DMA((96,)),
        pltpu.SemaphoreType.REGULAR((NZ,)),
    ]
    return pl.pallas_call(
        _kernel,
        in_specs=[pl.BlockSpec(memory_space=pltpu.HBM)] * len(ins),
        out_specs=pl.BlockSpec(memory_space=pltpu.HBM),
        out_shape=jax.ShapeDtypeStruct((1, 1, M), bf16),
        scratch_shapes=scratch,
        compiler_params=pltpu.CompilerParams(
            vmem_limit_bytes=120 * 1024 * 1024,
            disable_semaphore_checks=True,
            disable_bounds_checks=True,
            flags={"XLA_TPU_FORCE_LP_LLO_SCHEDULER": True},
        ),
    )(*ins)
```
